```python
import jax
import jax.numpy as jnp

def _softmax(x, axis=-1):
    return jax.nn.softmax(x, axis=axis)

def _gelu(x):
    return jax.nn.gelu(x, approximate=True)

def _silu(x):
    return jax.nn.silu(x)

def _sigmoid(x):
    return jax.nn.sigmoid(x)

def _layernorm(x, axis=-1, eps=1e-05):
    m = jnp.mean(x, axis=axis, keepdims=True)
    v = jnp.var(x, axis=axis, keepdims=True)
    return (x - m) / jnp.sqrt(v + eps)

def _scatter_add(tgt, idx, src, axis=0):
    return tgt.at[idx].add(src)

def _segment_sum(src, seg, n):
    return jax.ops.segment_sum(src, seg, n)

class _Rng:

    def __init__(self, key):
        self._k = key

    def _next(self):
        self._k, sub = jax.random.split(self._k)
        return sub

    def normal(self, shape):
        return jax.random.normal(self._next(), shape, dtype=jnp.bfloat16)

    def randint(self, lo, hi, shape):
        return jax.random.randint(self._next(), shape, lo, hi, dtype=jnp.int32)

    def uniform(self, shape, lo=0.0, hi=1.0):
        return jax.random.uniform(self._next(), shape, jnp.bfloat16, lo, hi)

    def permutation(self, n):
        return jax.random.permutation(self._next(), n)
kernel_name = 'concat_heads__memory_aug_recurrent_mem_tr__spectral_gfnet__prompt'

def setup_inputs():
    _rng = _Rng(jax.random.key(int.from_bytes(__import__("os").urandom(4), "little")))
    _w = lambda a: (lambda t: t.astype(jnp.bfloat16) if jnp.issubdtype(t.dtype, jnp.floating) else t)(jnp.asarray(a))

    def _A_setup():
        B, S, Dm = (1, 2048, 1024)
        H, Dh = (32, 128)
        M, seg = (8, 32)
        seg = min(seg, S)
        S = S // seg * seg
        return {'x': _w((lambda *s: _rng.normal(s) * 0.05)(B, S, Dm)), 'mem0': _w((lambda *s: _rng.normal(s) * 0.05)(B, M, Dm)), 'Wq': _w((lambda *s: _rng.normal(s) * 0.05)(Dm, H, Dh) * Dm ** (-0.5)), 'Wk': _w((lambda *s: _rng.normal(s) * 0.05)(Dm, H, Dh) * Dm ** (-0.5)), 'Wv': _w((lambda *s: _rng.normal(s) * 0.05)(Dm, H, Dh) * Dm ** (-0.5)), 'Wo': _w((lambda *s: _rng.normal(s) * 0.05)(H, Dh, Dm) * (H * Dh) ** (-0.5)), 'seg_len': seg}
    _A_in = _A_setup()

    def _B_setup():
        B, S, D = (1, 2048, 1024)
        Df = D // 2 + 1
        return {'x': _w((lambda *s: _rng.normal(s) * 0.05)(B, S, D)), 'w_r': _w((lambda *s: _rng.normal(s) * 0.05)(S, Df) * 0.02), 'w_i': _w((lambda *s: _rng.normal(s) * 0.05)(S, Df) * 0.02)}
    _B_in = _B_setup()
    return {'A_x': _A_in['x'], 'A_mem0': _A_in['mem0'], 'A_Wq': _A_in['Wq'], 'A_Wk': _A_in['Wk'], 'A_Wv': _A_in['Wv'], 'A_Wo': _A_in['Wo'], 'A_seg_len': _A_in['seg_len'], 'B_x': _B_in['x'], 'B_w_r': _B_in['w_r'], 'B_w_i': _B_in['w_i']}

def reference(A_x, A_mem0, A_Wq, A_Wk, A_Wv, A_Wo, A_seg_len, B_x, B_w_r, B_w_i):

    def _A_ref(x, mem0, Wq, Wk, Wv, Wo, seg_len):
        B, S, Dm = x.shape
        H, Dh = (Wq.shape[1], Wq.shape[2])
        M = mem0.shape[1]
        scale = Dh ** (-0.5)
        n_seg = S // seg_len
        L = M + seg_len
        idx = jnp.arange(L)
        mask = (idx[:, None] < M) | (idx[:, None] >= idx[None, :])
        mem = mem0
        outs = []
        for s in range(n_seg):
            xs = x[:, s * seg_len:(s + 1) * seg_len, :].copy()
            h = jnp.concatenate([mem, xs], axis=1)
            q = jnp.einsum('btd,dhe->bhte', h, Wq)
            k = jnp.einsum('btd,dhe->bhte', h, Wk)
            v = jnp.einsum('btd,dhe->bhte', h, Wv)
            scores = jnp.einsum('bhqe,bhke->bhqk', q, k) * scale
            scores = jnp.where(mask[None, None], scores, -1000000000.0)
            p = _softmax(scores, axis=-1)
            o = jnp.einsum('bhqk,bhke->bhqe', p, v)
            o = jnp.einsum('bhte,hed->btd', o, Wo)
            mem = o[:, :M, :].copy()
            outs.append(o[:, M:, :])
        return jnp.concatenate(outs, axis=1)

    def _B_ref(x, w_r, w_i):
        B, S, D = x.shape
        X = (lambda x, axes=(-2, -1): jnp.fft.rfft2(x.astype(jnp.float32), axes=axes))(x, axes=(-2, -1))
        W = w_r + 1j * w_i
        X = X * W
        y = (lambda x, s, axes=(-2, -1): jnp.fft.irfft2(x, s=s, axes=axes).astype(jnp.bfloat16))(X, (S, D), axes=(-2, -1))
        return y
    a = _A_ref(A_x, A_mem0, A_Wq, A_Wk, A_Wv, A_Wo, A_seg_len)
    b = _B_ref(B_x, B_w_r, B_w_i)
    return jnp.concatenate([a, b], axis=-1)
```

```python
import functools

import jax
import jax.numpy as jnp
import numpy as np
from jax import lax
from jax.experimental import pallas as pl
from jax.experimental.pallas import tpu as pltpu

F32 = jnp.float32
BF16 = jnp.bfloat16
U32 = jnp.uint32

G = 8
T = 8
SEG = 32
MEM = 8
DM = 1024
NH = 32
DH = 128
XR = G * SEG
MR = G * MEM
HR = XR + MR
LOG2E = 1.4426950408889634
QSCALE = float(DH ** -0.5 * LOG2E)
MASKED = float(-1e9 * LOG2E)
TOL = 2.0 ** -10
NT = (((1,), (1,)), ((), ()))
KROWS = 528
ROW_OFF = {0: 0, 4: 64, 1: 128, 7: 192, 2: 256, 6: 320, 3: 384, 5: 448}


def _constants():
    beta = np.arange(128)[None, :]
    m = np.arange(64)[:, None]
    d = np.zeros((4, 256, 256))
    for blk, r in enumerate((0, 4)):
        th = 2 * np.pi * (8 * m + r) * beta / 1024
        d[0, 64 * blk:64 * blk + 64, 128 * blk:128 * blk + 128] = np.cos(th)
        d[0, 128 + 64 * blk:192 + 64 * blk, 128 * blk:128 * blk + 128] = -np.sin(th)
    d[0, 128, 0:128] = np.cos(np.pi * np.arange(128))
    for r, sg in ((1, -1.0), (2, -1.0), (3, 1.0)):
        for blk, (res, cj) in enumerate(((r, 1.0), (8 - r, -1.0))):
            th = 2 * np.pi * (8 * m + res) * beta / 1024
            re, im = slice(64 * blk, 64 * blk + 64), slice(128 + 64 * blk, 192 + 64 * blk)
            d[r, re, 0:128] = np.cos(th)
            d[r, im, 0:128] = -np.sin(th)
            d[r, re, 128:256] = sg * cj * np.sin(th)
            d[r, im, 128:256] = sg * cj * np.cos(th)
    d *= 2.0 ** -10
    b = np.arange(128)[:, None]
    kb = np.arange(128)[None, :]
    s = np.zeros((16, 256, 256))
    for a in range(16):
        th = 2 * np.pi * ((kb * (16 * b + a)) % 2048) / 2048
        s[a, :128, :128] = np.cos(th)
        s[a, 128:, :128] = np.sin(th)
        s[a, :128, 128:] = -np.sin(th)
        s[a, 128:, 128:] = np.cos(th)
    mask = np.zeros((2, 128, 128), np.float32)
    for i, ns in enumerate((3, 2)):
        idx = np.arange(128)
        isx = idx < SEG * ns
        pad = idx >= (SEG + MEM) * ns
        seg = np.where(isx, idx // SEG, (idx - SEG * ns) // MEM)
        same = (seg[:, None] == seg[None, :]) & ~pad[None, :]
        future = isx[:, None] & isx[None, :] & (idx[None, :] > idx[:, None])
        mk = np.where(same, np.where(future, MASKED, 0.0), -np.inf)
        mask[i] = np.where(pad[:, None], 0.0, mk)
    return d.astype(BF16), s.astype(BF16), mask


def _lo(w):
    return lax.bitcast_convert_type(w << 16, F32)


def _hi(w):
    return lax.bitcast_convert_type(w & np.uint32(0xFFFF0000), F32)


def _bf16_bits(y):
    return lax.bitcast_convert_type(y.astype(BF16).astype(F32), U32)


def _r4(x, sg):
    (ar, ai), (br, bi), (cr, ci), (dr, di) = x
    s0r, s0i, d0r, d0i = ar + cr, ai + ci, ar - cr, ai - ci
    s1r, s1i, d1r, d1i = br + dr, bi + di, br - dr, bi - di
    p = (d0r - d1i, d0i + d1r)
    q = (d0r + d1i, d0i - d1r)
    y1, y3 = (p, q) if sg > 0 else (q, p)
    return [(s0r + s1r, s0i + s1i), y1, (s0r - s1r, s0i - s1i), y3]


def _tw(z, e, sg):
    r, i = z
    if e == 0:
        return z
    if e == 4:
        return (-i, r) if sg > 0 else (i, -r)
    h = float(np.sqrt(0.5))
    if e == 2:
        return ((r - i) * h, (r + i) * h) if sg > 0 else ((r + i) * h, (i - r) * h)
    if e == 6:
        return ((r + i) * -h, (r - i) * h) if sg > 0 else ((i - r) * h, (r + i) * -h)
    c = float(np.cos(2 * np.pi * e / 16))
    s = float(sg * np.sin(2 * np.pi * e / 16))
    return (r * c - i * s, r * s + i * c)


def _fft16(x, sg):
    t = [_r4([x[4 * a1 + a0] for a1 in range(4)], sg) for a0 in range(4)]
    out = [None] * 16
    for k0 in range(4):
        u = _r4([_tw(t[a0][k0], a0 * k0, sg) for a0 in range(4)], sg)
        for k1 in range(4):
            out[k0 + 4 * k1] = u[k1]
    return out


def _kernel(ax_hbm, wq_hbm, wk_hbm, wv_hbm, wo_hbm, bx_hbm, wr_hbm, wi_hbm, s_hbm,
            mem0_ref, wrn_ref, win_ref, d_ref, mask_ref,
            out_hbm,
            ax, wqkv, wo, xw, wr, wi, sm, yb, vb, kret, vret, h, qt, kt, vt, ob,
            mstart, mend, ostage, sem_b, sem_w, sem_m, sem_o):
    def cp_bx(c):
        return pltpu.make_async_copy(bx_hbm.bitcast(U32).at[:, c, :], xw.at[c], sem_b.at[0, c])

    def cp_s(c):
        sl = pl.ds(2 * c, 2)
        return pltpu.make_async_copy(s_hbm.at[sl], sm.at[sl], sem_b.at[1, c])

    def cp_by(c):
        return pltpu.make_async_copy(
            xw.at[c], out_hbm.bitcast(U32).at[:, c, pl.ds(DM, DM)], sem_b.at[2, c])

    def cp_w(j, p):
        src = (wq_hbm, wk_hbm, wv_hbm)[j]
        return pltpu.make_async_copy(src.bitcast(U32).at[:, :, p, :],
                                     wqkv.at[p, :, :, pl.ds(DH * j, DH)], sem_w.at[j, p])

    def cp_ao(t, g):
        return pltpu.make_async_copy(
            ostage.at[t, pl.ds(2 * g, 2)],
            out_hbm.at[pl.ds(2 * (T * g + t), 2), :, pl.ds(0, DM)], sem_o.at[t])

    def cp_f(j, k):
        src, dst = ((wr_hbm, wr), (wi_hbm, wi))[j]
        return pltpu.make_async_copy(
            src.at[pl.ds(0, 512), pl.ds(128 * k, 128)].bitcast(U32), dst.at[k], sem_m.at[j])

    cp_ax = pltpu.make_async_copy(ax_hbm, ax, sem_m.at[2])
    cp_wo = pltpu.make_async_copy(wo_hbm, wo, sem_m.at[3])

    for c in range(8):
        cp_bx(c).start()
        cp_s(c).start()
    for k in range(16):
        cp_f(0, k).start()
        cp_f(1, k).start()
    cp_ax.start()
    for p in range(NH // 2):
        cp_w(1, p).start()
        cp_w(2, p).start()
    cp_wo.start()
    for p in range(NH // 2):
        cp_w(0, p).start()

    rt = float(np.sqrt(0.5))
    row8 = lax.broadcasted_iota(jnp.int32, (8, 128), 0)

    def b_forward(c, carry):
        cp_bx(c).wait()
        cp_s(c).wait()
        w = xw[c]
        for half, xf in enumerate((_lo(w), _hi(w))):
            x = [xf[:, 128 * al:128 * (al + 1)] for al in range(8)]
            s = [x[i] + x[i + 4] for i in range(4)]
            d = [x[i] - x[i + 4] for i in range(4)]
            e, o = s[0] + s[2], s[1] + s[3]
            p, q = (d[1] - d[3]) * rt, (d[1] + d[3]) * rt
            u = [(e + o, e - o), (d[0] + p, d[2] + q), (s[0] - s[2], s[1] - s[3]),
                 (d[0] - p, d[2] - q)]
            tt = [lax.dot_general(d_ref[k], jnp.concatenate(u[k], axis=1).astype(BF16), NT,
                                  preferred_element_type=F32) for k in range(4)]
            dc, ny = tt[0][0:8], tt[0][128:136]
            re = [jnp.where(row8 == 0, dc * 0.5, dc), tt[0][8:128]]
            im = [jnp.where(row8 == 0, 0.0, ny), tt[0][136:256]]
            for k in range(1, 4):
                re.append(tt[k][0:128])
                im.append(tt[k][128:256])
            re += [jnp.where(row8 == 0, ny * 0.5, 0.0), jnp.zeros((8, 128), F32)]
            im.append(jnp.zeros((16, 128), F32))
            lhs = jnp.concatenate([jnp.concatenate(re, axis=0), jnp.concatenate(im, axis=0)],
                                  axis=1).astype(BF16)
            a = 2 * c + half
            yb[a] = jnp.dot(lhs, sm[a], preferred_element_type=F32)
        return carry

    lax.fori_loop(0, 8, b_forward, 0)
    pltpu.make_async_copy(wr, wr, sem_m.at[0]).wait()
    pltpu.make_async_copy(wi, wi, sem_m.at[1]).wait()

    def filt(row, wre, wim):
        y = [(yb[a, pl.ds(row, 8), 0:128], yb[a, pl.ds(row, 8), 128:256]) for a in range(16)]
        z = _fft16(y, -1)
        z = [(z[k][0] * wre(k) - z[k][1] * wim(k), z[k][0] * wim(k) + z[k][1] * wre(k))
             for k in range(16)]
        return _fft16(z, 1)

    def b_filter(i, carry):
        mg, j = i // 4, i % 4
        for half, un in enumerate((_lo, _hi)):
            off = [ROW_OFF[2 * jj + half] for jj in range(4)]
            base = jnp.where(j < 2, jnp.where(j == 0, off[0], off[1]),
                             jnp.where(j == 2, off[2], off[3])) + 16 * mg
            base = pl.multiple_of(base, 16)
            res = []
            for r8 in range(2):
                sl = pl.ds(64 * mg + 32 * r8 + j, 8, stride=4)
                res.append(filt(pl.multiple_of(base + 8 * r8, 8),
                                lambda k: un(wr[k, sl, :]),
                                lambda k: un(wi[k, sl, :])))
            for a in range(16):
                for ri in range(2):
                    vb[a, pl.ds(base, 16), 128 * ri:128 * (ri + 1)] = jnp.concatenate(
                        [res[0][a][ri], res[1][a][ri]], axis=0).astype(BF16)
        return carry

    lax.fori_loop(0, 16, b_filter, 0)
    res = filt(512, lambda k: wrn_ref[0:1, 128 * k:128 * (k + 1)].astype(F32),
               lambda k: win_ref[0:1, 128 * k:128 * (k + 1)].astype(F32))
    for a in range(16):
        for ri in range(2):
            vb[a, 512:KROWS, 128 * ri:128 * (ri + 1)] = jnp.concatenate(
                [res[a][ri], jnp.zeros((8, 128), F32)], axis=0).astype(BF16)
        vb[a, KROWS:640, :] = jnp.zeros((640 - KROWS, 256), BF16)

    lane0 = lax.broadcasted_iota(jnp.int32, (128, 128), 1) == 0

    def b_inverse(c, carry):
        lhs = [[] for _ in range(4)]
        for half in range(2):
            a = 2 * c + half
            z = lax.dot_general(sm[a], vb[a, 0:512, :], NT, preferred_element_type=F32)
            ny = lax.dot_general(sm[a, 0:128, :], vb[a, 512:640, :], NT,
                                 preferred_element_type=F32)
            for k in range(4):
                zr, zi = z[0:128, 128 * k:128 * (k + 1)], z[128:256, 128 * k:128 * (k + 1)]
                if k == 0:
                    zi = jnp.where(lane0, ny, zi)
                lhs[k].append(jnp.concatenate([zr, zi], axis=1).astype(BF16))
        g = [jnp.dot(jnp.concatenate(lhs[k], axis=0), d_ref[k], preferred_element_type=F32)
             for k in range(4)]
        (g0, g4), (g1r, g1i), (g2r, g2i), (g3r, g3i) = [(v[:, :128], v[:, 128:]) for v in g]
        e, o = g0 + g4, g0 - g4
        s = [e + g2r, o + g2i, e - g2r, o - g2i]
        p, q = (g1r - g3r) * rt, (g1i - g3i) * rt
        d = [g1r + g3r, q + p, g1i + g3i, q - p]
        y = [s[i] + d[i] for i in range(4)] + [s[i] - d[i] for i in range(4)]
        for al in range(8):
            bits = _bf16_bits(y[al])
            xw[c, :, 128 * al:128 * (al + 1)] = (bits[0:128] >> 16) | bits[128:256]
        cp_by(c).start()
        return carry

    lax.fori_loop(0, 8, b_inverse, 0)

    def unzip(p, lo, hi):
        for i0 in range(0, 64, 8):
            w = wqkv[p, i0:i0 + 8, :, DH * lo:DH * hi]
            wqkv[p, i0:i0 + 8, 0:8, DH * lo:DH * hi] = pltpu.bitcast(_lo(w).astype(BF16), U32)
            wqkv[p, i0:i0 + 8, 8:16, DH * lo:DH * hi] = pltpu.bitcast(_hi(w).astype(BF16), U32)

    def wmat(p, e, lo, hi):
        w = wqkv[p, :, 8 * e:8 * e + 8, DH * lo:DH * hi]
        return pltpu.bitcast(w, BF16).reshape(DM, DH * (hi - lo))

    XS = ((0, 96), (96, 192), (192, 256))
    MS = ((0, 24), (24, 48), (48, 64))

    def load_x(t):
        h[0:XR, :] = ax[:, t].reshape(XR, DM)

    cp_ax.wait()
    load_x(T - 1)
    cp_w(1, 0).wait()
    cp_w(2, 0).wait()
    unzip(0, 1, 3)

    def kv_last(p, nxt):
        if nxt:
            cp_w(1, p + 1).wait()
            cp_w(2, p + 1).wait()
        for e in range(2):
            r = jnp.dot(h[0:XR, :], wmat(p, e, 1, 3), preferred_element_type=F32).astype(BF16)
            kret[2 * p + e] = r[:, 0:DH]
            vret[2 * p + e] = r[:, DH:2 * DH]
        if nxt:
            unzip(p + 1, 1, 3)

    lax.fori_loop(0, NH // 2 - 1, lambda p, c: (kv_last(p, True), c)[1], 0)
    kv_last(NH // 2 - 1, False)

    xbar = jnp.sum(ax[:, T - 2].astype(F32), axis=1) * (1.0 / (SEG + MEM))
    xbar = jnp.concatenate([xbar, jnp.zeros((8, DM), F32)], axis=0).astype(BF16)

    def guess(p, carry):
        wv2 = jnp.concatenate([wmat(p, 0, 2, 3), wmat(p, 1, 2, 3)], axis=1)
        o = jnp.dot(xbar, wv2, preferred_element_type=F32).astype(BF16)
        ob[2 * p, 0:16, :] = o[:, 0:DH]
        ob[2 * p + 1, 0:16, :] = o[:, DH:2 * DH]
        return carry

    lax.fori_loop(0, NH // 2, guess, 0, unroll=2)
    cp_wo.wait()

    def out_proj(r0, r1, n):
        o = jnp.concatenate([ob[hh, r0:r1, :] for hh in range(NH)], axis=1)
        return jnp.dot(o, wo[:, pl.ds(pl.multiple_of(256 * n, 256), 256)],
                       preferred_element_type=F32)

    def guess_out(n, carry):
        m = out_proj(0, 16, n)
        rows = [jnp.broadcast_to(m[g:g + 1], (MEM, 256)) for g in range(G)]
        h[XR:HR, pl.ds(pl.multiple_of(256 * n, 256), 256)] = jnp.concatenate(
            rows, axis=0).astype(BF16)
        return carry

    lax.fori_loop(0, 4, guess_out, 0)

    def tile(v, g, with_x):
        m0 = XR if with_x else 0
        parts = [v[XS[g][0]:XS[g][1]]] if with_x else []
        parts.append(v[m0 + MS[g][0]:m0 + MS[g][1]])
        if g < 2:
            parts.append(jnp.zeros((8, DH), F32))
        return jnp.concatenate(parts, axis=0).astype(BF16)

    def step(mode, t):
        q_x, kv_x = mode != "pred", mode == "mid"
        nx = [hi - lo for lo, hi in XS]
        nm = (32, 32, 16)

        def put(ref, e, v, with_x):
            for g in range(3):
                r0 = 0 if with_x else nx[g]
                ref[e, g, r0:nx[g] + nm[g], :] = tile(v, g, with_x)

        def rows(with_x):
            return h[...] if with_x else h[XR:HR, :]

        def proj_qk(p, e):
            if q_x == kv_x:
                r = jnp.dot(rows(q_x), wmat(p, e, 0, 2), preferred_element_type=F32)
                q, k = r[:, 0:DH], r[:, DH:2 * DH]
            else:
                q = jnp.dot(rows(q_x), wmat(p, e, 0, 1), preferred_element_type=F32)
                k = jnp.dot(rows(kv_x), wmat(p, e, 1, 2), preferred_element_type=F32)
            put(qt, e, q * QSCALE, q_x)
            put(kt, e, k, kv_x)

        def proj_v(p, e):
            put(vt, e, jnp.dot(rows(kv_x), wmat(p, e, 2, 3), preferred_element_type=F32), kv_x)

        def get(ref, ret, hh, e, g):
            if kv_x:
                return ref[e, g]
            return jnp.concatenate([ret[hh, XS[g][0]:XS[g][1], :], ref[e, g, nx[g]:128, :]],
                                   axis=0)

        def scores(hh, e):
            out = []
            for g in range(3):
                r0 = 0 if q_x else nx[g]
                s = lax.dot_general(qt[e, g, r0:nx[g] + nm[g], :], get(kt, kret, hh, e, g), NT,
                                    preferred_element_type=F32)
                fill = mask_ref[g // 2, r0:nx[g] + nm[g], :]
                s = jnp.where(fill == 0.0, s, fill)
                pr = jnp.exp2(s - jnp.max(s, axis=1, keepdims=True))
                out.append((pr.astype(BF16), jnp.sum(pr, axis=1, keepdims=True)))
            return out

        def values(hh, e, sc):
            xs, ms = [], []
            for g in range(3):
                pr, den = sc[g]
                o = jnp.dot(pr, get(vt, vret, hh, e, g), preferred_element_type=F32) / den
                m0 = nx[g] if q_x else 0
                if q_x:
                    xs.append(o[0:m0])
                ms.append(o[m0:m0 + MS[g][1] - MS[g][0]])
            ob[hh, (0 if q_x else XR):HR, :] = jnp.concatenate(xs + ms, axis=0).astype(BF16)

        def pair(p, nxt):
            sc = scores(2 * p, 0)
            proj_qk(p, 1)
            values(2 * p, 0, sc)
            proj_v(p, 1)
            sc = scores(2 * p + 1, 1)
            if nxt:
                proj_qk(p + 1, 0)
            values(2 * p + 1, 1, sc)
            if nxt:
                proj_v(p + 1, 0)

        def pair_loop(p, carry):
            if mode == "pred":
                cp_w(0, p + 1).wait()
                unzip(p + 1, 0, 1)
            pair(p, True)
            return carry

        if mode == "pred":
            cp_w(0, 0).wait()
            unzip(0, 0, 1)
        proj_qk(0, 0)
        proj_v(0, 0)
        lax.fori_loop(0, NH // 2 - 1, pair_loop, 0)
        pair(NH // 2 - 1, False)

        def out_loop(n, carry):
            cols = pl.ds(pl.multiple_of(256 * n, 256), 256)
            r = out_proj(0 if q_x else XR, HR, n)
            if q_x:
                ostage[t, :, :, cols] = r[0:XR].astype(BF16).reshape(2 * G, 16, 256)
                r = r[XR:HR]
            if mode == "mid":
                h[XR:HR, cols] = r.astype(BF16)
            else:
                mend[:, cols] = r
            return carry

        lax.fori_loop(0, 4, out_loop, 0)

    kt[:, 2, 80:128, :] = jnp.zeros((2, 48, DH), BF16)
    vt[:, 2, 80:128, :] = jnp.zeros((2, 48, DH), BF16)

    step("pred", 0)

    def one_pass(carry):
        it, _ = carry
        mstart[...] = mend[0:MR - MEM, :]
        h[XR:HR, :] = jnp.concatenate(
            [mem0_ref[...].astype(F32), mend[0:MR - MEM, :]], axis=0).astype(BF16)

        def mid(t, c):
            load_x(t)
            step("mid", t)
            for g in range(G):
                cp_ao(t, g).start()
            return c

        lax.fori_loop(0, T - 1, mid, 0)
        load_x(T - 1)
        step("last", T - 1)
        for g in range(G):
            cp_ao(T - 1, g).start()
        real = mend[0:MR - MEM, :]
        lim = jnp.max(jnp.abs(real), axis=1, keepdims=True) * TOL
        good = jnp.abs(real - mstart[...]) <= lim
        bad = jnp.max(jnp.where(good, 0.0, 1.0))
        for t in range(T):
            pltpu.make_async_copy(ostage.at[t], ostage.at[t], sem_o.at[t]).wait()
        return it + 1, bad

    lax.while_loop(lambda c: jnp.logical_and(c[0] < G, c[1] > 0.0), one_pass,
                   (jnp.int32(0), jnp.float32(1.0)))
    for c in range(8):
        cp_by(c).wait()


@functools.partial(jax.jit, static_argnames=("A_seg_len",))
def pallas_concat_heads__memory_aug_recurrent_mem_tr__spectral_gfnet__prompt_kernel(
    A_x, A_mem0, A_Wq, A_Wk, A_Wv, A_Wo, A_seg_len, B_x, B_w_r, B_w_i,
):
    assert A_seg_len == SEG and A_x.shape == (1, G * T * SEG, DM) and A_Wq.shape == (DM, NH, DH)
    assert A_mem0.shape == (1, MEM, DM) and B_x.shape == (1, 2048, 1024)
    dmat, smat, mask = _constants()
    wr_t, wi_t = B_w_r.T, B_w_i.T
    hbm = pl.BlockSpec(memory_space=pl.ANY)
    nyq = pl.BlockSpec((16, 2048), lambda i: (32, 0))

    def full(shape):
        return pl.BlockSpec(shape, lambda i: (0,) * len(shape))

    out = pl.pallas_call(
        _kernel,
        grid=(1,),
        in_specs=[hbm] * 9 + [full((MEM, DM)), nyq, nyq, full(dmat.shape), full(mask.shape)],
        out_specs=hbm,
        out_shape=jax.ShapeDtypeStruct((128, 16, 2 * DM), BF16),
        scratch_shapes=[
            pltpu.VMEM((G, T, SEG, DM), BF16),
            pltpu.VMEM((NH // 2, 64, 16, 3 * DH), U32),
            pltpu.VMEM((NH * DH, DM), BF16),
            pltpu.VMEM((8, 128, 1024), U32),
            pltpu.VMEM((16, 256, 128), U32),
            pltpu.VMEM((16, 256, 128), U32),
            pltpu.VMEM((16, 256, 256), BF16),
            pltpu.VMEM((16, KROWS, 256), F32),
            pltpu.VMEM((16, 640, 256), BF16),
            pltpu.VMEM((NH, XR, DH), BF16),
            pltpu.VMEM((NH, XR, DH), BF16),
            pltpu.VMEM((HR, DM), BF16),
            pltpu.VMEM((2, 3, 128, DH), BF16),
            pltpu.VMEM((2, 3, 128, DH), BF16),
            pltpu.VMEM((2, 3, 128, DH), BF16),
            pltpu.VMEM((NH, HR, DH), BF16),
            pltpu.VMEM((MR - MEM, DM), F32),
            pltpu.VMEM((MR, DM), F32),
            pltpu.VMEM((T, 2 * G, 16, DM), BF16),
            pltpu.SemaphoreType.DMA((3, 8)),
            pltpu.SemaphoreType.DMA((3, NH // 2)),
            pltpu.SemaphoreType.DMA((4,)),
            pltpu.SemaphoreType.DMA((T,)),
        ],
        compiler_params=pltpu.CompilerParams(
            dimension_semantics=("arbitrary",), vmem_limit_bytes=110 * 1024 * 1024),
    )(
        A_x.reshape(G, T, SEG, DM),
        A_Wq.reshape(64, 16, NH, DH), A_Wk.reshape(64, 16, NH, DH), A_Wv.reshape(64, 16, NH, DH),
        A_Wo.reshape(NH * DH, DM), B_x.reshape(128, 16, 1024), wr_t, wi_t, smat,
        A_mem0.reshape(MEM, DM), wr_t, wi_t, dmat, mask,
    )
    return out.reshape(1, 2048, 2 * DM)
```

```python
import functools

import jax
import jax.numpy as jnp
import numpy as np
from jax import lax
from jax.experimental import pallas as pl
from jax.experimental.pallas import tpu as pltpu

F32 = jnp.float32
BF16 = jnp.bfloat16
U32 = jnp.uint32

G = 8
T = 8
SEG = 32
MEM = 8
DM = 1024
NH = 32
DH = 128
NP = NH // 2
XH = G // 2 * SEG
MH = G // 2 * MEM
HH = XH + MH
LOG2E = 1.4426950408889634
QSCALE = float(DH ** -0.5 * LOG2E)
MASKED = float(-1e9 * LOG2E)
TOL = 2.0 ** -10
NT = (((1,), (1,)), ((), ()))
KROWS = 528
ROW_OFF = {0: 0, 4: 64, 1: 128, 7: 192, 2: 256, 6: 320, 3: 384, 5: 448}


def _constants():
    beta = np.arange(128)[None, :]
    m = np.arange(64)[:, None]
    d = np.zeros((4, 256, 256))
    for blk, r in enumerate((0, 4)):
        th = 2 * np.pi * (8 * m + r) * beta / 1024
        d[0, 64 * blk:64 * blk + 64, 128 * blk:128 * blk + 128] = np.cos(th)
        d[0, 128 + 64 * blk:192 + 64 * blk, 128 * blk:128 * blk + 128] = -np.sin(th)
    d[0, 128, 0:128] = np.cos(np.pi * np.arange(128))
    for r, sg in ((1, -1.0), (2, -1.0), (3, 1.0)):
        for blk, (res, cj) in enumerate(((r, 1.0), (8 - r, -1.0))):
            th = 2 * np.pi * (8 * m + res) * beta / 1024
            re, im = slice(64 * blk, 64 * blk + 64), slice(128 + 64 * blk, 192 + 64 * blk)
            d[r, re, 0:128] = np.cos(th)
            d[r, im, 0:128] = -np.sin(th)
            d[r, re, 128:256] = sg * cj * np.sin(th)
            d[r, im, 128:256] = sg * cj * np.cos(th)
    d *= 2.0 ** -10
    b = np.arange(128)[:, None]
    kb = np.arange(128)[None, :]
    s = np.zeros((16, 256, 256))
    for a in range(16):
        th = 2 * np.pi * ((kb * (16 * b + a)) % 2048) / 2048
        s[a, :128, :128] = np.cos(th)
        s[a, 128:, :128] = np.sin(th)
        s[a, :128, 128:] = -np.sin(th)
        s[a, 128:, 128:] = np.cos(th)
    mask = np.zeros((2, 128, 128), np.float32)
    for i, ns in enumerate((3, 2)):
        idx = np.arange(128)
        isx = idx < SEG * ns
        pad = idx >= (SEG + MEM) * ns
        seg = np.where(isx, idx // SEG, (idx - SEG * ns) // MEM)
        same = (seg[:, None] == seg[None, :]) & ~pad[None, :]
        future = isx[:, None] & isx[None, :] & (idx[None, :] > idx[:, None])
        mk = np.where(same, np.where(future, MASKED, 0.0), -np.inf)
        mask[i] = np.where(pad[:, None], 0.0, mk)
    return d.astype(BF16), s.astype(BF16), mask


def _lo(w):
    return lax.bitcast_convert_type(w << 16, F32)


def _hi(w):
    return lax.bitcast_convert_type(w & np.uint32(0xFFFF0000), F32)


def _bf16_bits(y):
    return lax.bitcast_convert_type(y.astype(BF16).astype(F32), U32)


def _r4(x, sg):
    (ar, ai), (br, bi), (cr, ci), (dr, di) = x
    s0r, s0i, d0r, d0i = ar + cr, ai + ci, ar - cr, ai - ci
    s1r, s1i, d1r, d1i = br + dr, bi + di, br - dr, bi - di
    p = (d0r - d1i, d0i + d1r)
    q = (d0r + d1i, d0i - d1r)
    y1, y3 = (p, q) if sg > 0 else (q, p)
    return [(s0r + s1r, s0i + s1i), y1, (s0r - s1r, s0i - s1i), y3]


def _tw(z, e, sg):
    r, i = z
    if e == 0:
        return z
    if e == 4:
        return (-i, r) if sg > 0 else (i, -r)
    h = float(np.sqrt(0.5))
    if e == 2:
        return ((r - i) * h, (r + i) * h) if sg > 0 else ((r + i) * h, (i - r) * h)
    if e == 6:
        return ((r + i) * -h, (r - i) * h) if sg > 0 else ((i - r) * h, (r + i) * -h)
    c = float(np.cos(2 * np.pi * e / 16))
    s = float(sg * np.sin(2 * np.pi * e / 16))
    return (r * c - i * s, r * s + i * c)


def _fft16(x, sg):
    t = [_r4([x[4 * a1 + a0] for a1 in range(4)], sg) for a0 in range(4)]
    out = [None] * 16
    for k0 in range(4):
        u = _r4([_tw(t[a0][k0], a0 * k0, sg) for a0 in range(4)], sg)
        for k1 in range(4):
            out[k0 + 4 * k1] = u[k1]
    return out


def _lhs7(a11, a12, a21, a22):
    return [v.astype(BF16) for v in
            (a21 + a22, a11, a22, a11 + a12, a11 + a22, a21 - a11, a12 - a22)]


def _rhs7(b11, b12, b21, b22):
    return [v.astype(BF16) for v in
            (b11, b12 - b22, b21 - b11, b22, b11 + b22, b11 + b12, b21 + b22)]


def _out4(m):
    return m[4] + m[2] - m[3] + m[6], m[1] + m[3], m[0] + m[2], m[4] - m[0] + m[1] + m[5]


def _kernel(ax_hbm, wq_hbm, wk_hbm, wv_hbm, wo_hbm, bx_hbm, wr_hbm, wi_hbm, s_hbm,
            mem0_ref, wrn_ref, win_ref, d_ref, mask_ref,
            out_hbm,
            ax, wqkv, wo, xw, wr, wi, sm, yb, vb, kret, vret, hs, qt, kt, vt, ob,
            mstart, mend, ostage, sem_b, sem_w, sem_m, sem_o):
    def cp_bx(c):
        return pltpu.make_async_copy(bx_hbm.bitcast(U32).at[:, :, c, :], xw.at[c], sem_b.at[0, c])

    def cp_s(c):
        sl = pl.ds(2 * c, 2)
        return pltpu.make_async_copy(s_hbm.at[sl], sm.at[sl], sem_b.at[1, c])

    def cp_by(c):
        return pltpu.make_async_copy(
            xw.at[c], out_hbm.bitcast(U32).at[:, :, c, pl.ds(DM, DM)], sem_b.at[2, c])

    def cp_w(j, p):
        src = (wq_hbm, wk_hbm, wv_hbm)[j]
        return pltpu.make_async_copy(src.bitcast(U32).at[:, :, p, :],
                                     wqkv.at[p, :, pl.ds(0, 256), pl.ds(DH * j, DH)],
                                     sem_w.at[j, p])

    def cp_wo(e):
        return pltpu.make_async_copy(wo_hbm.at[:, e], wo.at[:, :, pl.ds(DM * e, DM)],
                                     sem_m.at[2 + e])

    def cp_ax(t):
        return pltpu.make_async_copy(ax_hbm.at[:, t], ax.at[t], sem_o.at[1, t])

    def cp_ao(t):
        return pltpu.make_async_copy(
            ostage.at[t], out_hbm.at[:, pl.ds(2 * t, 2), :, pl.ds(0, DM)], sem_o.at[0, t])

    def cp_f(j, k):
        src, dst = ((wr_hbm, wr), (wi_hbm, wi))[j]
        return pltpu.make_async_copy(
            src.at[pl.ds(0, 512), pl.ds(pl.multiple_of(128 * k, 128), 128)].bitcast(U32),
            dst.at[k], sem_m.at[j])

    for c in range(2):
        cp_bx(c).start()
        cp_s(c).start()

    rt = float(np.sqrt(0.5))
    row8 = lax.broadcasted_iota(jnp.int32, (8, 128), 0)

    def b_forward(c, carry):
        @pl.when(c < 6)
        def _():
            cp_bx(c + 2).start()
            cp_s(c + 2).start()

        for j in range(2):
            cp_f(j, 2 * c).start()
            cp_f(j, 2 * c + 1).start()

        @pl.when(c == 7)
        def _():
            cp_ax(T - 1).start()
            cp_ax(T - 2).start()
            cp_wo(0).start()
            cp_wo(1).start()

        cp_bx(c).wait()
        cp_s(c).wait()
        w = xw[c].reshape(128, DM)
        for half, xf in enumerate((_lo(w), _hi(w))):
            x = [xf[:, 128 * al:128 * (al + 1)] for al in range(8)]
            s = [x[i] + x[i + 4] for i in range(4)]
            d = [x[i] - x[i + 4] for i in range(4)]
            e, o = s[0] + s[2], s[1] + s[3]
            p, q = (d[1] - d[3]) * rt, (d[1] + d[3]) * rt
            u = [(e + o, e - o), (d[0] + p, d[2] + q), (s[0] - s[2], s[1] - s[3]),
                 (d[0] - p, d[2] - q)]
            tt = [lax.dot_general(d_ref[k], jnp.concatenate(u[k], axis=1).astype(BF16), NT,
                                  preferred_element_type=F32) for k in range(4)]
            dc, ny = tt[0][0:8], tt[0][128:136]
            re = [jnp.where(row8 == 0, dc * 0.5, dc), tt[0][8:128]]
            im = [jnp.where(row8 == 0, 0.0, ny), tt[0][136:256]]
            for k in range(1, 4):
                re.append(tt[k][0:128])
                im.append(tt[k][128:256])
            re += [jnp.where(row8 == 0, ny * 0.5, 0.0), jnp.zeros((8, 128), F32)]
            im.append(jnp.zeros((16, 128), F32))
            lhs = jnp.concatenate([jnp.concatenate(re, axis=0), jnp.concatenate(im, axis=0)],
                                  axis=1).astype(BF16)
            a = 2 * c + half
            yb[a] = jnp.dot(lhs, sm[a], preferred_element_type=F32)
        return carry

    lax.fori_loop(0, 8, b_forward, 0)
    pltpu.make_async_copy(wr, wr, sem_m.at[0]).wait()
    pltpu.make_async_copy(wi, wi, sem_m.at[1]).wait()

    def filt(row, wre, wim):
        y = [(yb[a, pl.ds(row, 8), 0:128], yb[a, pl.ds(row, 8), 128:256]) for a in range(16)]
        z = _fft16(y, -1)
        z = [(z[k][0] * wre(k) - z[k][1] * wim(k), z[k][0] * wim(k) + z[k][1] * wre(k))
             for k in range(16)]
        return _fft16(z, 1)

    def b_filter(i, carry):
        mg, j = i // 4, i % 4
        cp_w(1, i).start()
        cp_w(2, i).start()
        for half, un in enumerate((_lo, _hi)):
            off = [ROW_OFF[2 * jj + half] for jj in range(4)]
            base = jnp.where(j < 2, jnp.where(j == 0, off[0], off[1]),
                             jnp.where(j == 2, off[2], off[3])) + 16 * mg
            base = pl.multiple_of(base, 16)
            res = []
            for r8 in range(2):
                sl = pl.ds(64 * mg + 32 * r8 + j, 8, stride=4)
                res.append(filt(pl.multiple_of(base + 8 * r8, 8),
                                lambda k: un(wr[k, sl, :]),
                                lambda k: un(wi[k, sl, :])))
            for a in range(16):
                for ri in range(2):
                    vb[a, pl.ds(base, 16), 128 * ri:128 * (ri + 1)] = jnp.concatenate(
                        [res[0][a][ri], res[1][a][ri]], axis=0).astype(BF16)
        return carry

    lax.fori_loop(0, 16, b_filter, 0)
    res = filt(512, lambda k: wrn_ref[0:1, 128 * k:128 * (k + 1)].astype(F32),
               lambda k: win_ref[0:1, 128 * k:128 * (k + 1)].astype(F32))
    for a in range(16):
        for ri in range(2):
            vb[a, 512:KROWS, 128 * ri:128 * (ri + 1)] = jnp.concatenate(
                [res[a][ri], jnp.zeros((8, 128), F32)], axis=0).astype(BF16)
        vb[a, KROWS:640, :] = jnp.zeros((640 - KROWS, 256), BF16)

    lane0 = lax.broadcasted_iota(jnp.int32, (128, 128), 1) == 0

    def b_inverse(c, carry):
        cp_w(0, 2 * c).start()
        cp_w(0, 2 * c + 1).start()
        lhs = [[] for _ in range(4)]
        for half in range(2):
            a = 2 * c + half
            z = lax.dot_general(sm[a], vb[a, 0:512, :], NT, preferred_element_type=F32)
            ny = lax.dot_general(sm[a, 0:128, :], vb[a, 512:640, :], NT,
                                 preferred_element_type=F32)
            for k in range(4):
                zr, zi = z[0:128, 128 * k:128 * (k + 1)], z[128:256, 128 * k:128 * (k + 1)]
                if k == 0:
                    zi = jnp.where(lane0, ny, zi)
                lhs[k].append(jnp.concatenate([zr, zi], axis=1).astype(BF16))
        g = [jnp.dot(jnp.concatenate(lhs[k], axis=0), d_ref[k], preferred_element_type=F32)
             for k in range(4)]
        (g0, g4), (g1r, g1i), (g2r, g2i), (g3r, g3i) = [(v[:, :128], v[:, 128:]) for v in g]
        e, o = g0 + g4, g0 - g4
        s = [e + g2r, o + g2i, e - g2r, o - g2i]
        p, q = (g1r - g3r) * rt, (g1i - g3i) * rt
        d = [g1r + g3r, q + p, g1i + g3i, q - p]
        y = [s[i] + d[i] for i in range(4)] + [s[i] - d[i] for i in range(4)]
        for al in range(8):
            bits = _bf16_bits(y[al])
            xw[c, :, :, 128 * al:128 * (al + 1)] = (
                (bits[0:128] >> 16) | bits[128:256]).reshape(8, 16, 128)
        return carry

    lax.fori_loop(0, 8, b_inverse, 0)

    def prep_w(p, j):
        cols = slice(DH * j, DH * (j + 1))
        for i in range(4):
            w1, w2 = wqkv[p, i, 0:128, cols], wqkv[p, i, 128:256, cols]
            for n, v in enumerate(_rhs7(_lo(w1), _hi(w1), _lo(w2), _hi(w2))):
                wqkv[p, i, 64 * n:64 * (n + 1), cols] = pltpu.bitcast(v, U32)

    def prep_wo(p):
        for r in range(0, DH, 32):
            w = wo[p, r:r + 32, 0:2 * DM].astype(F32)
            for i in range(4):
                b = [w[:, DM * e + 256 * i + 128 * k:DM * e + 256 * i + 128 * (k + 1)]
                     for e in range(2) for k in range(2)]
                for n, v in enumerate(_rhs7(*b)):
                    c0 = ((i // 2) * 7 + n) * 256 + (i % 2) * 128
                    wo[p, r:r + 32, c0:c0 + 128] = v

    def halves(v):
        n = v.shape[1] // 256
        return [jnp.concatenate([v[:, 256 * i + 128 * k:256 * i + 128 * (k + 1)]
                                 for i in range(n)], axis=1) for k in range(2)]

    def load_x(t):
        for g in range(G // 2):
            top, bot = ax[t, g].astype(F32), ax[t, g + G // 2].astype(F32)
            for n, v in enumerate(_lhs7(*halves(top), *halves(bot))):
                hs[n, SEG * g:SEG * (g + 1), :] = v

    def set_mem(m):
        for n, v in enumerate(_lhs7(*halves(m[0:MH]), *halves(m[MH:2 * MH]))):
            hs[n, XH:HH, :] = v

    def project(p, r0, r1, lo, hi):
        m = []
        for n in range(7):
            w = pltpu.bitcast(wqkv[p, :, 64 * n:64 * (n + 1), DH * lo:DH * hi], BF16)
            m.append(jnp.dot(hs[n, r0:r1, :], w.reshape(DM // 2, DH * (hi - lo)),
                             preferred_element_type=F32))
        c11, c12, c21, c22 = _out4(m)
        return (c11, c21), (c12, c22)

    def put_o(p, r0, o):
        for n, v in enumerate(_lhs7(o[0][0], o[1][0], o[0][1], o[1][1])):
            ob[n, p, r0:HH, :] = v

    def out_proj(c, r0):
        m = []
        for n in range(7):
            o = jnp.concatenate([ob[n, p, r0:HH, :] for p in range(NP)], axis=1)
            w = wo[:, :, pl.ds(pl.multiple_of((c * 7 + n) * 256, 256), 256)]
            m.append(jnp.dot(o, w.reshape(NP * DH, 256), preferred_element_type=F32))
        return _out4(m)

    def weave(a, b):
        return jnp.concatenate([a[:, 0:128], b[:, 0:128], a[:, 128:256], b[:, 128:256]], axis=1)

    def out_mem(c, r0, keep):
        c11, c12, c21, c22 = out_proj(c, r0)
        x0 = XH - r0
        if keep:
            cols = pl.ds(pl.multiple_of(512 * c, 512), 512)
            mend[0:MH, cols] = weave(c11[x0:], c12[x0:])
            mend[MH:2 * MH, cols] = weave(c21[x0:], c22[x0:])
        else:
            for n, v in enumerate(_lhs7(c11[x0:], c12[x0:], c21[x0:], c22[x0:])):
                hs[n, XH:HH, pl.ds(pl.multiple_of(256 * c, 256), 256)] = v
        return weave(c11[:x0], c12[:x0]), weave(c21[:x0], c22[:x0])

    cp_ax(T - 1).wait()
    load_x(T - 1)
    cp_wo(0).wait()
    cp_wo(1).wait()
    for j in (1, 2):
        cp_w(j, 0).wait()
        prep_w(0, j)

    def kv_last(p, nxt):
        if nxt:
            cp_w(1, p + 1).wait()
            cp_w(2, p + 1).wait()
        r = project(p, 0, XH, 1, 3)
        for e in range(2):
            v = jnp.concatenate(r[e], axis=0).astype(BF16)
            kret[p, e] = v[:, 0:DH]
            vret[p, e] = v[:, DH:2 * DH]
        prep_wo(p)
        if nxt:
            prep_w(p + 1, 1)
            prep_w(p + 1, 2)

    lax.fori_loop(0, NP - 1, lambda p, c: (kv_last(p, True), c)[1], 0)
    kv_last(NP - 1, False)
    for t in range(T - 2):
        cp_ax(t).start()
    for c in range(8):
        cp_by(c).start()

    cp_ax(T - 2).wait()
    xbar = jnp.sum(ax[T - 2].astype(F32), axis=1, keepdims=True) * (1.0 / (SEG + MEM))
    set_mem(jnp.broadcast_to(xbar, (G, MEM, DM)).reshape(G * MEM, DM))

    def guess(p, carry):
        put_o(p, XH, project(p, XH, HH, 2, 3))
        return carry

    lax.fori_loop(0, NP, guess, 0, unroll=2)
    lax.fori_loop(0, 2, lambda c, carry: (out_mem(c, XH, False), carry)[1], 0)

    TILES = ((0, 1, 2), (3, 4, 5), (6, 7))
    nx = [SEG * len(tl) for tl in TILES]
    nm = (32, 32, 16)

    def tile(v, g, with_x):
        m0 = XH if with_x else 0
        parts = [v[ch // 4][SEG * (ch % 4):SEG * (ch % 4 + 1)] for ch in TILES[g]] if with_x else []
        parts += [v[ch // 4][m0 + MEM * (ch % 4):m0 + MEM * (ch % 4 + 1)] for ch in TILES[g]]
        if len(TILES[g]) == 3:
            parts.append(jnp.zeros((MEM, DH), F32))
        return jnp.concatenate(parts, axis=0).astype(BF16)

    def step(mode, t):
        q_x, kv_x = mode != "pred", mode == "mid"
        q0, kv0 = (0 if q_x else XH), (0 if kv_x else XH)

        def put(ref, e, v, with_x):
            for g in range(3):
                ref[e, g, (0 if with_x else nx[g]):nx[g] + nm[g], :] = tile(v, g, with_x)

        def proj_qk(p):
            if q_x == kv_x:
                r = project(p, q0, HH, 0, 2)
                q = [[v[:, 0:DH] for v in r[e]] for e in range(2)]
                k = [[v[:, DH:2 * DH] for v in r[e]] for e in range(2)]
            else:
                q, k = project(p, q0, HH, 0, 1), project(p, kv0, HH, 1, 2)
            for e in range(2):
                put(qt, e, [v * QSCALE for v in q[e]], q_x)
                put(kt, e, k[e], kv_x)

        def proj_v(p):
            v = project(p, kv0, HH, 2, 3)
            for e in range(2):
                put(vt, e, v[e], kv_x)

        def get(ref, ret, p, e, g):
            if kv_x:
                return ref[e, g]
            return jnp.concatenate([ret[p, e, 96 * g:96 * g + nx[g], :], ref[e, g, nx[g]:128, :]],
                                   axis=0)

        def scores(p, e):
            out = []
            for g in range(3):
                r0 = 0 if q_x else nx[g]
                s = lax.dot_general(qt[e, g, r0:nx[g] + nm[g], :], get(kt, kret, p, e, g), NT,
                                    preferred_element_type=F32)
                fill = mask_ref[g // 2, r0:nx[g] + nm[g], :]
                s = jnp.where(fill == 0.0, s, fill)
                pr = jnp.exp2(s - jnp.max(s, axis=1, keepdims=True))
                out.append((pr.astype(BF16), jnp.sum(pr, axis=1, keepdims=True)))
            return out

        def values(p, e, sc):
            xs, ms = [], []
            for g in range(3):
                pr, den = sc[g]
                o = jnp.dot(pr, get(vt, vret, p, e, g), preferred_element_type=F32) / den
                m0 = nx[g] if q_x else 0
                for i in range(len(TILES[g])):
                    if q_x:
                        xs.append(o[SEG * i:SEG * (i + 1)])
                    ms.append(o[m0 + MEM * i:m0 + MEM * (i + 1)])
            return [jnp.concatenate(xs[4 * k:4 * k + 4] + ms[4 * k:4 * k + 4], axis=0)
                    for k in range(2)]

        def pair(p, nxt):
            if nxt and mode == "pred":
                cp_w(0, p + 1).wait()
                prep_w(p + 1, 0)
            sc = [scores(p, e) for e in range(2)]
            if nxt:
                proj_qk(p + 1)
            put_o(p, q0, [values(p, e, sc[e]) for e in range(2)])
            if nxt:
                proj_v(p + 1)

        if mode == "pred":
            cp_w(0, 0).wait()
            prep_w(0, 0)
        proj_qk(0)
        proj_v(0)
        lax.fori_loop(0, NP - 1, lambda p, c: (pair(p, True), c)[1], 0)
        pair(NP - 1, False)

        def out_loop(c, carry):
            top, bot = out_mem(c, q0, mode != "mid")
            if q_x:
                cols = pl.ds(pl.multiple_of(512 * c, 512), 512)
                ostage[t, 0:G // 2, :, :, cols] = top.astype(BF16).reshape(G // 2, 2, 16, 512)
                ostage[t, G // 2:G, :, :, cols] = bot.astype(BF16).reshape(G // 2, 2, 16, 512)
            return carry

        lax.fori_loop(0, 2, out_loop, 0)

    kt[:, 2, 80:128, :] = jnp.zeros((2, 48, DH), BF16)
    vt[:, 2, 80:128, :] = jnp.zeros((2, 48, DH), BF16)

    step("pred", 0)
    for t in range(T - 2):
        cp_ax(t).wait()

    def one_pass(carry):
        it, _ = carry
        start = mend[0:(G - 1) * MEM, :]
        mstart[...] = start
        set_mem(jnp.concatenate([mem0_ref[...].astype(F32), start], axis=0))

        def mid(t, c):
            load_x(t)
            step("mid", t)
            cp_ao(t).start()
            return c

        lax.fori_loop(0, T - 1, mid, 0)
        load_x(T - 1)
        step("last", T - 1)
        cp_ao(T - 1).start()
        real = mend[0:(G - 1) * MEM, :]
        lim = jnp.max(jnp.abs(real), axis=1, keepdims=True) * TOL
        good = jnp.abs(real - mstart[...]) <= lim
        bad = jnp.max(jnp.where(good, 0.0, 1.0))
        for t in range(T):
            cp_ao(t).wait()
        return it + 1, bad

    lax.while_loop(lambda c: jnp.logical_and(c[0] < G, c[1] > 0.0), one_pass,
                   (jnp.int32(0), jnp.float32(1.0)))
    for c in range(8):
        cp_by(c).wait()


@functools.partial(jax.jit, static_argnames=("A_seg_len",))
def pallas_concat_heads__memory_aug_recurrent_mem_tr__spectral_gfnet__prompt_kernel(
    A_x, A_mem0, A_Wq, A_Wk, A_Wv, A_Wo, A_seg_len, B_x, B_w_r, B_w_i,
):
    assert A_seg_len == SEG and A_x.shape == (1, G * T * SEG, DM) and A_Wq.shape == (DM, NH, DH)
    assert A_mem0.shape == (1, MEM, DM) and B_x.shape == (1, 2048, 1024)
    dmat, smat, mask = _constants()
    wr_t, wi_t = B_w_r.T, B_w_i.T
    hbm = pl.BlockSpec(memory_space=pl.ANY)
    nyq = pl.BlockSpec((16, 2048), lambda i: (32, 0))

    def full(shape):
        return pl.BlockSpec(shape, lambda i: (0,) * len(shape))

    out = pl.pallas_call(
        _kernel,
        grid=(1,),
        in_specs=[hbm] * 9 + [full((MEM, DM)), nyq, nyq, full(dmat.shape), full(mask.shape)],
        out_specs=hbm,
        out_shape=jax.ShapeDtypeStruct((G, 16, 16, 2 * DM), BF16),
        scratch_shapes=[
            pltpu.VMEM((T, G, SEG, DM), BF16),
            pltpu.VMEM((NP, 4, 7 * 64, 3 * DH), U32),
            pltpu.VMEM((NP, DH, 7 * 512), BF16),
            pltpu.VMEM((8, 8, 16, 1024), U32),
            pltpu.VMEM((16, 256, 128), U32),
            pltpu.VMEM((16, 256, 128), U32),
            pltpu.VMEM((16, 256, 256), BF16),
            pltpu.VMEM((16, KROWS, 256), F32),
            pltpu.VMEM((16, 640, 256), BF16),
            pltpu.VMEM((NP, 2, G * SEG, DH), BF16),
            pltpu.VMEM((NP, 2, G * SEG, DH), BF16),
            pltpu.VMEM((7, HH, DM // 2), BF16),
            pltpu.VMEM((2, 3, 128, DH), BF16),
            pltpu.VMEM((2, 3, 128, DH), BF16),
            pltpu.VMEM((2, 3, 128, DH), BF16),
            pltpu.VMEM((7, NP, HH, DH), BF16),
            pltpu.VMEM(((G - 1) * MEM, DM), F32),
            pltpu.VMEM((G * MEM, DM), F32),
            pltpu.VMEM((T, G, 2, 16, DM), BF16),
            pltpu.SemaphoreType.DMA((3, 8)),
            pltpu.SemaphoreType.DMA((3, NP)),
            pltpu.SemaphoreType.DMA((4,)),
            pltpu.SemaphoreType.DMA((2, T)),
        ],
        compiler_params=pltpu.CompilerParams(
            dimension_semantics=("arbitrary",), vmem_limit_bytes=120 * 1024 * 1024),
    )(
        A_x.reshape(G, T, SEG, DM),
        A_Wq.reshape(4, 256, NH, DH), A_Wk.reshape(4, 256, NH, DH), A_Wv.reshape(4, 256, NH, DH),
        A_Wo.reshape(NP, 2, DH, DM), B_x.reshape(8, 16, 16, 1024), wr_t, wi_t, smat,
        A_mem0.reshape(MEM, DM), wr_t, wi_t, dmat, mask,
    )
    return out.reshape(1, 2048, 2 * DM)
```

```python
import functools

import jax
import jax.numpy as jnp
import numpy as np
from jax import lax
from jax.experimental import pallas as pl
from jax.experimental.pallas import tpu as pltpu

F32 = jnp.float32
BF16 = jnp.bfloat16
U32 = jnp.uint32

G = 8
T = 8
SEG = 32
MEM = 8
DM = 1024
NH = 32
DH = 128
NP = NH // 2
XH = G // 2 * SEG
MH = G // 2 * MEM
HH = XH + MH
LOG2E = 1.4426950408889634
QSCALE = float(DH ** -0.5 * LOG2E)
MASKED = float(-1e9 * LOG2E)
TOL = 2.0 ** -9
NT = (((1,), (1,)), ((), ()))
KROWS = 528
ROW_OFF = {0: 0, 4: 64, 1: 128, 7: 192, 2: 256, 6: 320, 3: 384, 5: 448}


def _constants():
    beta = np.arange(128)[None, :]
    m = np.arange(64)[:, None]
    d = np.zeros((4, 256, 256))
    for blk, r in enumerate((0, 4)):
        th = 2 * np.pi * (8 * m + r) * beta / 1024
        d[0, 64 * blk:64 * blk + 64, 128 * blk:128 * blk + 128] = np.cos(th)
        d[0, 128 + 64 * blk:192 + 64 * blk, 128 * blk:128 * blk + 128] = -np.sin(th)
    d[0, 128, 0:128] = np.cos(np.pi * np.arange(128))
    for r, sg in ((1, -1.0), (2, -1.0), (3, 1.0)):
        for blk, (res, cj) in enumerate(((r, 1.0), (8 - r, -1.0))):
            th = 2 * np.pi * (8 * m + res) * beta / 1024
            re, im = slice(64 * blk, 64 * blk + 64), slice(128 + 64 * blk, 192 + 64 * blk)
            d[r, re, 0:128] = np.cos(th)
            d[r, im, 0:128] = -np.sin(th)
            d[r, re, 128:256] = sg * cj * np.sin(th)
            d[r, im, 128:256] = sg * cj * np.cos(th)
    d *= 2.0 ** -10
    b = np.arange(128)[:, None]
    kb = np.arange(128)[None, :]
    s = np.zeros((16, 256, 256))
    for a in range(16):
        th = 2 * np.pi * ((kb * (16 * b + a)) % 2048) / 2048
        s[a, :128, :128] = np.cos(th)
        s[a, 128:, :128] = np.sin(th)
        s[a, :128, 128:] = -np.sin(th)
        s[a, 128:, 128:] = np.cos(th)
    mask = np.zeros((2, 128, 128), np.float32)
    for i, ns in enumerate((3, 2)):
        idx = np.arange(128)
        isx = idx < SEG * ns
        pad = idx >= (SEG + MEM) * ns
        seg = np.where(isx, idx // SEG, (idx - SEG * ns) // MEM)
        same = (seg[:, None] == seg[None, :]) & ~pad[None, :]
        future = isx[:, None] & isx[None, :] & (idx[None, :] > idx[:, None])
        mk = np.where(same, np.where(future, MASKED, 0.0), -np.inf)
        mask[i] = np.where(pad[:, None], 0.0, mk)
    return d.astype(BF16), s.astype(BF16), mask


def _lo(w):
    return lax.bitcast_convert_type(w << 16, F32)


def _hi(w):
    return lax.bitcast_convert_type(w & np.uint32(0xFFFF0000), F32)


def _bf16_bits(y):
    return lax.bitcast_convert_type(y.astype(BF16).astype(F32), U32)


def _r4(x, sg):
    (ar, ai), (br, bi), (cr, ci), (dr, di) = x
    s0r, s0i, d0r, d0i = ar + cr, ai + ci, ar - cr, ai - ci
    s1r, s1i, d1r, d1i = br + dr, bi + di, br - dr, bi - di
    p = (d0r - d1i, d0i + d1r)
    q = (d0r + d1i, d0i - d1r)
    y1, y3 = (p, q) if sg > 0 else (q, p)
    return [(s0r + s1r, s0i + s1i), y1, (s0r - s1r, s0i - s1i), y3]


def _tw(z, e, sg):
    r, i = z
    if e == 0:
        return z
    if e == 4:
        return (-i, r) if sg > 0 else (i, -r)
    h = float(np.sqrt(0.5))
    if e == 2:
        return ((r - i) * h, (r + i) * h) if sg > 0 else ((r + i) * h, (i - r) * h)
    if e == 6:
        return ((r + i) * -h, (r - i) * h) if sg > 0 else ((i - r) * h, (r + i) * -h)
    c = float(np.cos(2 * np.pi * e / 16))
    s = float(sg * np.sin(2 * np.pi * e / 16))
    return (r * c - i * s, r * s + i * c)


def _fft16(x, sg):
    t = [_r4([x[4 * a1 + a0] for a1 in range(4)], sg) for a0 in range(4)]
    out = [None] * 16
    for k0 in range(4):
        u = _r4([_tw(t[a0][k0], a0 * k0, sg) for a0 in range(4)], sg)
        for k1 in range(4):
            out[k0 + 4 * k1] = u[k1]
    return out


def _lhs7(a11, a12, a21, a22):
    return [v.astype(BF16) for v in
            (a21 + a22, a11, a22, a11 + a12, a11 + a22, a21 - a11, a12 - a22)]


def _rhs7(b11, b12, b21, b22):
    return [v.astype(BF16) for v in
            (b11, b12 - b22, b21 - b11, b22, b11 + b22, b11 + b12, b21 + b22)]


def _out4(m):
    return m[4] + m[2] - m[3] + m[6], m[1] + m[3], m[0] + m[2], m[4] - m[0] + m[1] + m[5]


def _kernel(ax_hbm, wq_hbm, wk_hbm, wv_hbm, wo_hbm, bx_hbm, wr_hbm, wi_hbm, s_hbm,
            mem0_ref, wrn_ref, win_ref, d_ref, mask_ref,
            out_hbm,
            ax, weven, wodd, wo, xw, wr, wi, sm, yb, vb, kret, vret, hs, qt, kt, vt, ob,
            mstart, mend, ostage, sem_b, sem_w, sem_m, sem_o):
    def cp_bx(c):
        return pltpu.make_async_copy(bx_hbm.bitcast(U32).at[:, :, c, :], xw.at[c], sem_b.at[0, c])

    def cp_s(c):
        sl = pl.ds(2 * c, 2)
        return pltpu.make_async_copy(s_hbm.at[sl], sm.at[sl], sem_b.at[1, c])

    def cp_by(c):
        return pltpu.make_async_copy(
            xw.at[c], out_hbm.bitcast(U32).at[:, :, c, pl.ds(DM, DM)], sem_b.at[2, c])

    def cp_w(j, i, par):
        src = (wq_hbm, wk_hbm, wv_hbm)[j]
        return pltpu.make_async_copy(
            src.bitcast(U32).at[:, :, 2 * i + par, :],
            (weven, wodd)[par].at[i, :, pl.ds(0, 256), pl.ds(DH * j, DH)], sem_w.at[j, par, i])

    def cp_wo(e):
        return pltpu.make_async_copy(wo_hbm.at[:, e], wo.at[:, :, pl.ds(DM * e, DM)],
                                     sem_m.at[2 + e])

    def cp_ax(t):
        return pltpu.make_async_copy(ax_hbm.at[:, t], ax.at[t], sem_o.at[1, t])

    def cp_ao(t):
        return pltpu.make_async_copy(
            ostage.at[t], out_hbm.at[:, pl.ds(2 * t, 2), :, pl.ds(0, DM)], sem_o.at[0, t])

    def cp_f(j, k):
        src, dst = ((wr_hbm, wr), (wi_hbm, wi))[j]
        return pltpu.make_async_copy(
            src.at[pl.ds(0, 512), pl.ds(pl.multiple_of(128 * k, 128), 128)].bitcast(U32),
            dst.at[k], sem_m.at[j])

    for c in range(2):
        cp_bx(c).start()
        cp_s(c).start()

    rt = float(np.sqrt(0.5))
    row8 = lax.broadcasted_iota(jnp.int32, (8, 128), 0)

    def b_forward(c, carry):
        @pl.when(c < 6)
        def _():
            cp_bx(c + 2).start()
            cp_s(c + 2).start()

        for j in range(2):
            cp_f(j, 2 * c).start()
            cp_f(j, 2 * c + 1).start()

        @pl.when(c == 7)
        def _():
            cp_ax(T - 1).start()
            cp_ax(T - 2).start()

        cp_bx(c).wait()
        cp_s(c).wait()
        w = xw[c].reshape(128, DM)
        for half, xf in enumerate((_lo(w), _hi(w))):
            x = [xf[:, 128 * al:128 * (al + 1)] for al in range(8)]
            s = [x[i] + x[i + 4] for i in range(4)]
            d = [x[i] - x[i + 4] for i in range(4)]
            e, o = s[0] + s[2], s[1] + s[3]
            p, q = (d[1] - d[3]) * rt, (d[1] + d[3]) * rt
            u = [(e + o, e - o), (d[0] + p, d[2] + q), (s[0] - s[2], s[1] - s[3]),
                 (d[0] - p, d[2] - q)]
            tt = [lax.dot_general(d_ref[k], jnp.concatenate(u[k], axis=1).astype(BF16), NT,
                                  preferred_element_type=F32) for k in range(4)]
            dc, ny = tt[0][0:8], tt[0][128:136]
            re = [jnp.where(row8 == 0, dc * 0.5, dc), tt[0][8:128]]
            im = [jnp.where(row8 == 0, 0.0, ny), tt[0][136:256]]
            for k in range(1, 4):
                re.append(tt[k][0:128])
                im.append(tt[k][128:256])
            re += [jnp.where(row8 == 0, ny * 0.5, 0.0), jnp.zeros((8, 128), F32)]
            im.append(jnp.zeros((16, 128), F32))
            lhs = jnp.concatenate([jnp.concatenate(re, axis=0), jnp.concatenate(im, axis=0)],
                                  axis=1).astype(BF16)
            a = 2 * c + half
            yb[a] = jnp.dot(lhs, sm[a], preferred_element_type=F32)
        return carry

    lax.fori_loop(0, 8, b_forward, 0)
    pltpu.make_async_copy(wr, wr, sem_m.at[0]).wait()
    pltpu.make_async_copy(wi, wi, sem_m.at[1]).wait()

    def filt(row, wre, wim):
        y = [(yb[a, pl.ds(row, 8), 0:128], yb[a, pl.ds(row, 8), 128:256]) for a in range(16)]
        z = _fft16(y, -1)
        z = [(z[k][0] * wre(k) - z[k][1] * wim(k), z[k][0] * wim(k) + z[k][1] * wre(k))
             for k in range(16)]
        return _fft16(z, 1)

    def b_filter(i, carry):
        mg, j = i // 4, i % 4

        @pl.when(i < NP // 2)
        def _():
            for par in range(2):
                cp_w(1, i, par).start()
                cp_w(2, i, par).start()

        for half, un in enumerate((_lo, _hi)):
            off = [ROW_OFF[2 * jj + half] for jj in range(4)]
            base = jnp.where(j < 2, jnp.where(j == 0, off[0], off[1]),
                             jnp.where(j == 2, off[2], off[3])) + 16 * mg
            base = pl.multiple_of(base, 16)
            res = []
            for r8 in range(2):
                sl = pl.ds(64 * mg + 32 * r8 + j, 8, stride=4)
                res.append(filt(pl.multiple_of(base + 8 * r8, 8),
                                lambda k: un(wr[k, sl, :]),
                                lambda k: un(wi[k, sl, :])))
            for a in range(16):
                for ri in range(2):
                    vb[a, pl.ds(base, 16), 128 * ri:128 * (ri + 1)] = jnp.concatenate(
                        [res[0][a][ri], res[1][a][ri]], axis=0).astype(BF16)
        return carry

    lax.fori_loop(0, 16, b_filter, 0)
    res = filt(512, lambda k: wrn_ref[0:1, 128 * k:128 * (k + 1)].astype(F32),
               lambda k: win_ref[0:1, 128 * k:128 * (k + 1)].astype(F32))
    for a in range(16):
        for ri in range(2):
            vb[a, 512:KROWS, 128 * ri:128 * (ri + 1)] = jnp.concatenate(
                [res[a][ri], jnp.zeros((8, 128), F32)], axis=0).astype(BF16)
        vb[a, KROWS:640, :] = jnp.zeros((640 - KROWS, 256), BF16)

    lane0 = lax.broadcasted_iota(jnp.int32, (128, 128), 1) == 0

    def b_inverse(c, carry):
        lhs = [[] for _ in range(4)]
        for half in range(2):
            a = 2 * c + half
            z = lax.dot_general(sm[a], vb[a, 0:512, :], NT, preferred_element_type=F32)
            ny = lax.dot_general(sm[a, 0:128, :], vb[a, 512:640, :], NT,
                                 preferred_element_type=F32)
            for k in range(4):
                zr, zi = z[0:128, 128 * k:128 * (k + 1)], z[128:256, 128 * k:128 * (k + 1)]
                if k == 0:
                    zi = jnp.where(lane0, ny, zi)
                lhs[k].append(jnp.concatenate([zr, zi], axis=1).astype(BF16))
        g = [jnp.dot(jnp.concatenate(lhs[k], axis=0), d_ref[k], preferred_element_type=F32)
             for k in range(4)]
        (g0, g4), (g1r, g1i), (g2r, g2i), (g3r, g3i) = [(v[:, :128], v[:, 128:]) for v in g]
        e, o = g0 + g4, g0 - g4
        s = [e + g2r, o + g2i, e - g2r, o - g2i]
        p, q = (g1r - g3r) * rt, (g1i - g3i) * rt
        d = [g1r + g3r, q + p, g1i + g3i, q - p]
        y = [s[i] + d[i] for i in range(4)] + [s[i] - d[i] for i in range(4)]
        for al in range(8):
            bits = _bf16_bits(y[al])
            xw[c, :, :, 128 * al:128 * (al + 1)] = (
                (bits[0:128] >> 16) | bits[128:256]).reshape(8, 16, 128)
        return carry

    lax.fori_loop(0, 8, b_inverse, 0)

    def prep_w(j, p, par):
        wqkv = (weven, wodd)[par]
        cols = slice(DH * j, DH * (j + 1))
        cp_w(j, p, par).wait()
        for i in range(4):
            w1, w2 = wqkv[p, i, 0:128, cols], wqkv[p, i, 128:256, cols]
            for r in range(0, 128, 32):
                a, b = w1[r:r + 32], w2[r:r + 32]
                for n, v in enumerate(_rhs7(_lo(a), _hi(a), _lo(b), _hi(b))):
                    wqkv[p, i, 64 * n + r // 2:64 * n + r // 2 + 16, cols] = pltpu.bitcast(v, U32)

    def prep_wo(p):
        for r in range(0, DH, 32):
            w = wo[p, r:r + 32, 0:2 * DM].astype(F32)
            for i in range(4):
                b = [w[:, DM * e + 256 * i + 128 * k:DM * e + 256 * i + 128 * (k + 1)]
                     for e in range(2) for k in range(2)]
                for n, v in enumerate(_rhs7(*b)):
                    c0 = ((i // 2) * 7 + n) * 256 + (i % 2) * 128
                    wo[p, r:r + 32, c0:c0 + 128] = v

    def halves(v):
        n = v.shape[1] // 256
        return [jnp.concatenate([v[:, 256 * i + 128 * k:256 * i + 128 * (k + 1)]
                                 for i in range(n)], axis=1) for k in range(2)]

    def load_x(t):
        for g in range(G // 2):
            top, bot = ax[t, g].astype(F32), ax[t, g + G // 2].astype(F32)
            for n, v in enumerate(_lhs7(*halves(top), *halves(bot))):
                hs[n, SEG * g:SEG * (g + 1), :] = v

    def set_mem(m):
        for n, v in enumerate(_lhs7(*halves(m[0:MH]), *halves(m[MH:2 * MH]))):
            hs[n, XH:HH, :] = v

    def project(p, par, r0, r1, lo, hi):
        wqkv = (weven, wodd)[par]
        m = []
        for n in range(7):
            w = pltpu.bitcast(wqkv[p, :, 64 * n:64 * (n + 1), DH * lo:DH * hi], BF16)
            m.append(jnp.dot(hs[n, r0:r1, :], w.reshape(DM // 2, DH * (hi - lo)),
                             preferred_element_type=F32))
        c11, c12, c21, c22 = _out4(m)
        return (c11, c21), (c12, c22)

    def put_o(p, r0, o):
        for n, v in enumerate(_lhs7(o[0][0], o[1][0], o[0][1], o[1][1])):
            ob[n, p, r0:HH, :] = v

    def out_proj(c, r0):
        m = []
        for n in range(7):
            o = jnp.concatenate([ob[n, p, r0:HH, :] for p in range(NP)], axis=1)
            w = wo[:, :, pl.ds(pl.multiple_of((c * 7 + n) * 256, 256), 256)]
            m.append(jnp.dot(o, w.reshape(NP * DH, 256), preferred_element_type=F32))
        return _out4(m)

    def weave(a, b):
        return jnp.concatenate([a[:, 0:128], b[:, 0:128], a[:, 128:256], b[:, 128:256]], axis=1)

    def out_mem(c, r0, keep, feed):
        c11, c12, c21, c22 = out_proj(c, r0)
        x0 = XH - r0
        if keep:
            cols = pl.ds(pl.multiple_of(512 * c, 512), 512)
            mend[0:MH, cols] = weave(c11[x0:], c12[x0:])
            mend[MH:2 * MH, cols] = weave(c21[x0:], c22[x0:])
        if feed:
            for n, v in enumerate(_lhs7(c11[x0:], c12[x0:], c21[x0:], c22[x0:])):
                hs[n, XH:HH, pl.ds(pl.multiple_of(256 * c, 256), 256)] = v
        return weave(c11[:x0], c12[:x0]), weave(c21[:x0], c22[:x0])

    cp_ax(T - 1).wait()
    load_x(T - 1)
    prep_w(1, 0, 0)
    prep_w(2, 0, 0)

    def kv_last(i, par, nxt):
        r = project(i, par, 0, XH, 1, 3)
        for e in range(2):
            v = jnp.concatenate(r[e], axis=0).astype(BF16)
            kret[2 * i + par, e] = v[:, 0:DH]
            vret[2 * i + par, e] = v[:, DH:2 * DH]
        if nxt:
            prep_w(1, i + par, 1 - par)
            prep_w(2, i + par, 1 - par)

    def kv_loop(i, carry):
        @pl.when(i == 0)
        def _():
            cp_wo(0).start()
            cp_wo(1).start()

        cp_w(0, i, 0).start()
        cp_w(0, i, 1).start()
        kv_last(i, 0, True)
        kv_last(i, 1, True)
        return carry

    lax.fori_loop(0, NP // 2 - 1, kv_loop, 0)
    cp_w(0, NP // 2 - 1, 0).start()
    cp_w(0, NP // 2 - 1, 1).start()
    kv_last(NP // 2 - 1, 0, True)
    kv_last(NP // 2 - 1, 1, False)
    for t in range(T - 2):
        cp_ax(t).start()
    for c in range(8):
        cp_by(c).start()

    cp_ax(T - 2).wait()
    xbar = jnp.sum(ax[T - 2].astype(F32), axis=1, keepdims=True) * (1.0 / (SEG + MEM))
    set_mem(jnp.broadcast_to(xbar, (G, MEM, DM)).reshape(G * MEM, DM))
    cp_wo(0).wait()
    cp_wo(1).wait()

    def guess(i, carry):
        for par in range(2):
            put_o(2 * i + par, XH, project(i, par, XH, HH, 2, 3))
            prep_wo(2 * i + par)
        return carry

    lax.fori_loop(0, NP // 2, guess, 0)
    lax.fori_loop(0, 2, lambda c, carry: (out_mem(c, XH, False, True), carry)[1], 0)

    TILES = ((0, 1, 2), (3, 4, 5), (6, 7))
    nx = [SEG * len(tl) for tl in TILES]
    nm = (32, 32, 16)

    def tile(v, g, with_x):
        m0 = XH if with_x else 0
        parts = [v[ch // 4][SEG * (ch % 4):SEG * (ch % 4 + 1)] for ch in TILES[g]] if with_x else []
        parts += [v[ch // 4][m0 + MEM * (ch % 4):m0 + MEM * (ch % 4 + 1)] for ch in TILES[g]]
        if len(TILES[g]) == 3:
            parts.append(jnp.zeros((MEM, DH), F32))
        return jnp.concatenate(parts, axis=0).astype(BF16)

    def step(mode):
        q_x, kv_x = mode != "pred", mode == "mid"
        q0, kv0 = (0 if q_x else XH), (0 if kv_x else XH)

        def put(ref, e, v, with_x):
            for g in range(3):
                ref[e, g, (0 if with_x else nx[g]):nx[g] + nm[g], :] = tile(v, g, with_x)

        def proj_qk(i, par):
            if q_x == kv_x:
                r = project(i, par, q0, HH, 0, 2)
                q = [[v[:, 0:DH] for v in r[e]] for e in range(2)]
                k = [[v[:, DH:2 * DH] for v in r[e]] for e in range(2)]
            else:
                q, k = project(i, par, q0, HH, 0, 1), project(i, par, kv0, HH, 1, 2)
            for e in range(2):
                put(qt, e, [v * QSCALE for v in q[e]], q_x)
                put(kt, e, k[e], kv_x)

        def proj_v(i, par):
            v = project(i, par, kv0, HH, 2, 3)
            for e in range(2):
                put(vt, e, v[e], kv_x)

        def get(ref, ret, p, e, g):
            if kv_x:
                return ref[e, g]
            return jnp.concatenate([ret[p, e, 96 * g:96 * g + nx[g], :], ref[e, g, nx[g]:128, :]],
                                   axis=0)

        def scores(p, e):
            out = []
            for g in range(3):
                r0 = 0 if q_x else nx[g]
                s = lax.dot_general(qt[e, g, r0:nx[g] + nm[g], :], get(kt, kret, p, e, g), NT,
                                    preferred_element_type=F32)
                fill = mask_ref[g // 2, r0:nx[g] + nm[g], :]
                s = jnp.where(fill == 0.0, s, fill)
                pr = jnp.exp2(s - jnp.max(s, axis=1, keepdims=True))
                out.append((pr.astype(BF16), jnp.sum(pr, axis=1, keepdims=True)))
            return out

        def values(p, e, sc):
            xs, ms = [], []
            for g in range(3):
                pr, den = sc[g]
                o = jnp.dot(pr, get(vt, vret, p, e, g), preferred_element_type=F32) / den
                m0 = nx[g] if q_x else 0
                for i in range(len(TILES[g])):
                    if q_x:
                        xs.append(o[SEG * i:SEG * (i + 1)])
                    ms.append(o[m0 + MEM * i:m0 + MEM * (i + 1)])
            return [jnp.concatenate(xs[4 * k:4 * k + 4] + ms[4 * k:4 * k + 4], axis=0)
                    for k in range(2)]

        def pair(i, par, nxt):
            p = 2 * i + par
            sc = [scores(p, e) for e in range(2)]
            if nxt:
                proj_qk(i + par, 1 - par)
            put_o(p, q0, [values(p, e, sc[e]) for e in range(2)])
            if nxt:
                proj_v(i + par, 1 - par)

        return proj_qk, proj_v, pair

    kt[:, 2, 80:128, :] = jnp.zeros((2, 48, DH), BF16)
    vt[:, 2, 80:128, :] = jnp.zeros((2, 48, DH), BF16)

    proj_qk, proj_v, pair = step("pred")
    prep_w(0, 0, 0)
    proj_qk(0, 0)
    proj_v(0, 0)
    prep_w(0, 0, 1)

    def pred_loop(i, carry):
        pair(i, 0, True)
        prep_w(0, i + 1, 0)
        pair(i, 1, True)
        prep_w(0, i + 1, 1)
        return carry

    lax.fori_loop(0, NP // 2 - 1, pred_loop, 0)
    pair(NP // 2 - 1, 0, True)
    pair(NP // 2 - 1, 1, False)
    lax.fori_loop(0, 2, lambda c, carry: (out_mem(c, XH, True, False), carry)[1], 0)
    for t in range(T - 2):
        cp_ax(t).wait()

    proj_qk, proj_v, pair = step("mid")
    pair_last = step("last")[2]

    def pairs(fn):
        def pair_loop(i, carry):
            fn(i, 1, True)
            fn(i + 1, 0, True)
            return carry

        lax.fori_loop(0, NP // 2 - 1, pair_loop, 0)

    def segment(t, carry):
        load_x(t)
        proj_qk(0, 0)
        proj_v(0, 0)
        pair(0, 0, True)

        @pl.when(t < T - 1)
        def _():
            pairs(pair)

        @pl.when(t == T - 1)
        def _():
            pairs(pair_last)
            for e in range(2):
                for g in range(3):
                    kt[e, g, 0:nx[g], :] = kret[NP - 1, e, 96 * g:96 * g + nx[g], :]
                    vt[e, g, 0:nx[g], :] = vret[NP - 1, e, 96 * g:96 * g + nx[g], :]

        pair(NP // 2 - 1, 1, False)
        for c in range(2):
            top, bot = out_mem(c, 0, True, True)
            cols = slice(512 * c, 512 * (c + 1))
            ostage[t, 0:G // 2, :, :, cols] = top.astype(BF16).reshape(G // 2, 2, 16, 512)
            ostage[t, G // 2:G, :, :, cols] = bot.astype(BF16).reshape(G // 2, 2, 16, 512)
        cp_ao(t).start()
        return carry

    def one_pass(carry):
        it, _ = carry
        start = mend[0:(G - 1) * MEM, :]
        mstart[...] = start
        set_mem(jnp.concatenate([mem0_ref[...].astype(F32), start], axis=0))
        lax.fori_loop(0, T, segment, 0)
        real = mend[0:(G - 1) * MEM, :]
        lim = jnp.max(jnp.abs(real), axis=1, keepdims=True) * TOL
        good = jnp.abs(real - mstart[...]) <= lim
        bad = jnp.max(jnp.where(good, 0.0, 1.0))
        for t in range(T):
            cp_ao(t).wait()
        return it + 1, bad

    lax.while_loop(lambda c: jnp.logical_and(c[0] < G, c[1] > 0.0), one_pass,
                   (jnp.int32(0), jnp.float32(1.0)))
    for c in range(8):
        cp_by(c).wait()


@functools.partial(jax.jit, static_argnames=("A_seg_len",))
def pallas_concat_heads__memory_aug_recurrent_mem_tr__spectral_gfnet__prompt_kernel(
    A_x, A_mem0, A_Wq, A_Wk, A_Wv, A_Wo, A_seg_len, B_x, B_w_r, B_w_i,
):
    assert A_seg_len == SEG and A_x.shape == (1, G * T * SEG, DM) and A_Wq.shape == (DM, NH, DH)
    assert A_mem0.shape == (1, MEM, DM) and B_x.shape == (1, 2048, 1024)
    dmat, smat, mask = _constants()
    wr_t, wi_t = B_w_r.T, B_w_i.T
    hbm = pl.BlockSpec(memory_space=pl.ANY)
    nyq = pl.BlockSpec((16, 2048), lambda i: (32, 0))

    def full(shape):
        return pl.BlockSpec(shape, lambda i: (0,) * len(shape))

    out = pl.pallas_call(
        _kernel,
        grid=(1,),
        in_specs=[hbm] * 9 + [full((MEM, DM)), nyq, nyq, full(dmat.shape), full(mask.shape)],
        out_specs=hbm,
        out_shape=jax.ShapeDtypeStruct((G, 16, 16, 2 * DM), BF16),
        scratch_shapes=[
            pltpu.VMEM((T, G, SEG, DM), BF16),
            pltpu.VMEM((NP // 2, 4, 7 * 64, 3 * DH), U32),
            pltpu.VMEM((NP // 2, 4, 7 * 64, 3 * DH), U32),
            pltpu.VMEM((NP, DH, 7 * 512), BF16),
            pltpu.VMEM((8, 8, 16, 1024), U32),
            pltpu.VMEM((16, 256, 128), U32),
            pltpu.VMEM((16, 256, 128), U32),
            pltpu.VMEM((16, 256, 256), BF16),
            pltpu.VMEM((16, KROWS, 256), F32),
            pltpu.VMEM((16, 640, 256), BF16),
            pltpu.VMEM((NP, 2, G * SEG, DH), BF16),
            pltpu.VMEM((NP, 2, G * SEG, DH), BF16),
            pltpu.VMEM((7, HH, DM // 2), BF16),
            pltpu.VMEM((2, 3, 128, DH), BF16),
            pltpu.VMEM((2, 3, 128, DH), BF16),
            pltpu.VMEM((2, 3, 128, DH), BF16),
            pltpu.VMEM((7, NP, HH, DH), BF16),
            pltpu.VMEM(((G - 1) * MEM, DM), F32),
            pltpu.VMEM((G * MEM, DM), F32),
            pltpu.VMEM((T, G, 2, 16, DM), BF16),
            pltpu.SemaphoreType.DMA((3, 8)),
            pltpu.SemaphoreType.DMA((3, 2, NP // 2)),
            pltpu.SemaphoreType.DMA((4,)),
            pltpu.SemaphoreType.DMA((2, T)),
        ],
        compiler_params=pltpu.CompilerParams(
            dimension_semantics=("arbitrary",), vmem_limit_bytes=120 * 1024 * 1024),
    )(
        A_x.reshape(G, T, SEG, DM),
        A_Wq.reshape(4, 256, NH, DH), A_Wk.reshape(4, 256, NH, DH), A_Wv.reshape(4, 256, NH, DH),
        A_Wo.reshape(NP, 2, DH, DM), B_x.reshape(8, 16, 16, 1024), wr_t, wi_t, smat,
        A_mem0.reshape(MEM, DM), wr_t, wi_t, dmat, mask,
    )
    return out.reshape(1, 2048, 2 * DM)
```

```python
import functools

import jax
import jax.numpy as jnp
import numpy as np
from jax import lax
from jax.experimental import pallas as pl
from jax.experimental.pallas import tpu as pltpu

F32 = jnp.float32
BF16 = jnp.bfloat16
U32 = jnp.uint32

G = 8
T = 8
SEG = 32
MEM = 8
DM = 1024
NH = 32
DH = 128
NP = NH // 2
XH = G // 2 * SEG
MH = G // 2 * MEM
HH = XH + MH
LOG2E = 1.4426950408889634
QSCALE = float(DH ** -0.5 * LOG2E)
MASKED = float(-1e9 * LOG2E)
TOL = 2.0 ** -9
NT = (((1,), (1,)), ((), ()))
KROWS = 528
ROW_OFF = {0: 0, 4: 64, 1: 128, 7: 192, 2: 256, 6: 320, 3: 384, 5: 448}


def _constants():
    beta = np.arange(128)[None, :]
    m = np.arange(64)[:, None]
    d = np.zeros((4, 256, 256))
    for blk, r in enumerate((0, 4)):
        th = 2 * np.pi * (8 * m + r) * beta / 1024
        d[0, 64 * blk:64 * blk + 64, 128 * blk:128 * blk + 128] = np.cos(th)
        d[0, 128 + 64 * blk:192 + 64 * blk, 128 * blk:128 * blk + 128] = -np.sin(th)
    d[0, 128, 0:128] = np.cos(np.pi * np.arange(128))
    for r, sg in ((1, -1.0), (2, -1.0), (3, 1.0)):
        for blk, (res, cj) in enumerate(((r, 1.0), (8 - r, -1.0))):
            th = 2 * np.pi * (8 * m + res) * beta / 1024
            re, im = slice(64 * blk, 64 * blk + 64), slice(128 + 64 * blk, 192 + 64 * blk)
            d[r, re, 0:128] = np.cos(th)
            d[r, im, 0:128] = -np.sin(th)
            d[r, re, 128:256] = sg * cj * np.sin(th)
            d[r, im, 128:256] = sg * cj * np.cos(th)
    d *= 2.0 ** -10
    b = np.arange(128)[:, None]
    kb = np.arange(128)[None, :]
    s = np.zeros((16, 256, 256))
    for a in range(16):
        th = 2 * np.pi * ((kb * (16 * b + a)) % 2048) / 2048
        s[a, :128, :128] = np.cos(th)
        s[a, 128:, :128] = np.sin(th)
        s[a, :128, 128:] = -np.sin(th)
        s[a, 128:, 128:] = np.cos(th)
    mask = np.zeros((2, 128, 128), np.float32)
    for i, ns in enumerate((3, 2)):
        idx = np.arange(128)
        isx = idx < SEG * ns
        pad = idx >= (SEG + MEM) * ns
        seg = np.where(isx, idx // SEG, (idx - SEG * ns) // MEM)
        same = (seg[:, None] == seg[None, :]) & ~pad[None, :]
        future = isx[:, None] & isx[None, :] & (idx[None, :] > idx[:, None])
        mk = np.where(same, np.where(future, MASKED, 0.0), -np.inf)
        mask[i] = np.where(pad[:, None], 0.0, mk)
    return d.astype(BF16), s.astype(BF16), mask


def _lo(w):
    return lax.bitcast_convert_type(w << 16, F32)


def _hi(w):
    return lax.bitcast_convert_type(w & np.uint32(0xFFFF0000), F32)


def _bf16_bits(y):
    return lax.bitcast_convert_type(y.astype(BF16).astype(F32), U32)


def _r4(x, sg):
    (ar, ai), (br, bi), (cr, ci), (dr, di) = x
    s0r, s0i, d0r, d0i = ar + cr, ai + ci, ar - cr, ai - ci
    s1r, s1i, d1r, d1i = br + dr, bi + di, br - dr, bi - di
    p = (d0r - d1i, d0i + d1r)
    q = (d0r + d1i, d0i - d1r)
    y1, y3 = (p, q) if sg > 0 else (q, p)
    return [(s0r + s1r, s0i + s1i), y1, (s0r - s1r, s0i - s1i), y3]


def _tw(z, e, sg):
    r, i = z
    if e == 0:
        return z
    if e == 4:
        return (-i, r) if sg > 0 else (i, -r)
    h = float(np.sqrt(0.5))
    if e == 2:
        return ((r - i) * h, (r + i) * h) if sg > 0 else ((r + i) * h, (i - r) * h)
    if e == 6:
        return ((r + i) * -h, (r - i) * h) if sg > 0 else ((i - r) * h, (r + i) * -h)
    c = float(np.cos(2 * np.pi * e / 16))
    s = float(sg * np.sin(2 * np.pi * e / 16))
    return (r * c - i * s, r * s + i * c)


def _fft16(x, sg):
    t = [_r4([x[4 * a1 + a0] for a1 in range(4)], sg) for a0 in range(4)]
    out = [None] * 16
    for k0 in range(4):
        u = _r4([_tw(t[a0][k0], a0 * k0, sg) for a0 in range(4)], sg)
        for k1 in range(4):
            out[k0 + 4 * k1] = u[k1]
    return out


def _lhs7(a11, a12, a21, a22):
    return [v.astype(BF16) for v in
            (a21 + a22, a11, a22, a11 + a12, a11 + a22, a21 - a11, a12 - a22)]


def _rhs7(b11, b12, b21, b22):
    return [v.astype(BF16) for v in
            (b11, b12 - b22, b21 - b11, b22, b11 + b22, b11 + b12, b21 + b22)]


def _out4(m):
    return m[4] + m[2] - m[3] + m[6], m[1] + m[3], m[0] + m[2], m[4] - m[0] + m[1] + m[5]


def _kernel(ax_hbm, wq_hbm, wk_hbm, wv_hbm, wo_hbm, bx_hbm, wr_hbm, wi_hbm, s_hbm,
            mem0_ref, wrn_ref, win_ref, d_ref, mask_ref,
            out_hbm,
            ax, wq, wk, wv, wo, xw, wr, wi, sm, yb, vb, kret, vret, hs, qt, kt, vt, ob,
            mstart, mend, ostage, sem_b, sem_w, sem_m, sem_o):
    wqkv = (wq, wk, wv)

    def cp_bx(c):
        return pltpu.make_async_copy(bx_hbm.bitcast(U32).at[:, :, c, :], xw.at[c], sem_b.at[0, c])

    def cp_s(c):
        sl = pl.ds(2 * c, 2)
        return pltpu.make_async_copy(s_hbm.at[sl], sm.at[sl], sem_b.at[1, c])

    def cp_by(c):
        return pltpu.make_async_copy(
            xw.at[c], out_hbm.bitcast(U32).at[:, :, c, pl.ds(DM, DM)], sem_b.at[2, c])

    def cp_w(j, p):
        src = (wq_hbm, wk_hbm, wv_hbm)[j]
        return pltpu.make_async_copy(src.bitcast(U32).at[:, :, p, :],
                                     wqkv[j].at[p, :, pl.ds(0, 256), :], sem_w.at[j, p])

    def cp_wo(n):
        c, e = divmod(n, 2)
        return pltpu.make_async_copy(wo_hbm.at[:, e, :, pl.ds(512 * c, 512)],
                                     wo.at[:, :, pl.ds(1792 * c + 512 * e, 512)], sem_m.at[2 + n])

    def cp_ax(t):
        return pltpu.make_async_copy(ax_hbm.at[:, t], ax.at[t], sem_o.at[1, t])

    def cp_ao(t):
        return pltpu.make_async_copy(
            ostage.at[t], out_hbm.at[:, pl.ds(2 * t, 2), :, pl.ds(0, DM)], sem_o.at[0, t])

    def cp_f(j, k):
        src, dst = ((wr_hbm, wr), (wi_hbm, wi))[j]
        return pltpu.make_async_copy(
            src.at[pl.ds(0, 512), pl.ds(pl.multiple_of(128 * k, 128), 128)].bitcast(U32),
            dst.at[k], sem_m.at[j])

    for c in range(2):
        cp_bx(c).start()
        cp_s(c).start()

    rt = float(np.sqrt(0.5))
    row8 = lax.broadcasted_iota(jnp.int32, (8, 128), 0)

    def b_forward(c, carry):
        @pl.when(c < 6)
        def _():
            cp_bx(c + 2).start()
            cp_s(c + 2).start()

        for j in range(2):
            cp_f(j, 2 * c).start()
            cp_f(j, 2 * c + 1).start()

        @pl.when(c == 7)
        def _():
            cp_ax(T - 1).start()
            cp_ax(T - 2).start()

        cp_bx(c).wait()
        cp_s(c).wait()
        w = xw[c].reshape(128, DM)
        for half, xf in enumerate((_lo(w), _hi(w))):
            x = [xf[:, 128 * al:128 * (al + 1)] for al in range(8)]
            s = [x[i] + x[i + 4] for i in range(4)]
            d = [x[i] - x[i + 4] for i in range(4)]
            e, o = s[0] + s[2], s[1] + s[3]
            p, q = (d[1] - d[3]) * rt, (d[1] + d[3]) * rt
            u = [(e + o, e - o), (d[0] + p, d[2] + q), (s[0] - s[2], s[1] - s[3]),
                 (d[0] - p, d[2] - q)]
            tt = [lax.dot_general(d_ref[k], jnp.concatenate(u[k], axis=1).astype(BF16), NT,
                                  preferred_element_type=F32) for k in range(4)]
            dc, ny = tt[0][0:8], tt[0][128:136]
            re = [jnp.where(row8 == 0, dc * 0.5, dc), tt[0][8:128]]
            im = [jnp.where(row8 == 0, 0.0, ny), tt[0][136:256]]
            for k in range(1, 4):
                re.append(tt[k][0:128])
                im.append(tt[k][128:256])
            re += [jnp.where(row8 == 0, ny * 0.5, 0.0), jnp.zeros((8, 128), F32)]
            im.append(jnp.zeros((16, 128), F32))
            lhs = jnp.concatenate([jnp.concatenate(re, axis=0), jnp.concatenate(im, axis=0)],
                                  axis=1).astype(BF16)
            a = 2 * c + half
            yb[a] = jnp.dot(lhs, sm[a], preferred_element_type=F32)
        return carry

    lax.fori_loop(0, 8, b_forward, 0)
    pltpu.make_async_copy(wr, wr, sem_m.at[0]).wait()
    pltpu.make_async_copy(wi, wi, sem_m.at[1]).wait()

    def filt(row, wre, wim):
        y = [(yb[a, pl.ds(row, 8), 0:128], yb[a, pl.ds(row, 8), 128:256]) for a in range(16)]
        z = _fft16(y, -1)
        z = [(z[k][0] * wre(k) - z[k][1] * wim(k), z[k][0] * wim(k) + z[k][1] * wre(k))
             for k in range(16)]
        return _fft16(z, 1)

    def b_filter(i, carry):
        mg, j = i // 4, i % 4
        cp_w(1, i).start()
        cp_w(2, i).start()
        for half, un in enumerate((_lo, _hi)):
            off = [ROW_OFF[2 * jj + half] for jj in range(4)]
            base = jnp.where(j < 2, jnp.where(j == 0, off[0], off[1]),
                             jnp.where(j == 2, off[2], off[3])) + 16 * mg
            base = pl.multiple_of(base, 16)
            res = []
            for r8 in range(2):
                sl = pl.ds(64 * mg + 32 * r8 + j, 8, stride=4)
                res.append(filt(pl.multiple_of(base + 8 * r8, 8),
                                lambda k: un(wr[k, sl, :]),
                                lambda k: un(wi[k, sl, :])))
            for a in range(16):
                for ri in range(2):
                    vb[a, pl.ds(base, 16), 128 * ri:128 * (ri + 1)] = jnp.concatenate(
                        [res[0][a][ri], res[1][a][ri]], axis=0).astype(BF16)
        return carry

    lax.fori_loop(0, 16, b_filter, 0)
    res = filt(512, lambda k: wrn_ref[0:1, 128 * k:128 * (k + 1)].astype(F32),
               lambda k: win_ref[0:1, 128 * k:128 * (k + 1)].astype(F32))
    for a in range(16):
        for ri in range(2):
            vb[a, 512:KROWS, 128 * ri:128 * (ri + 1)] = jnp.concatenate(
                [res[a][ri], jnp.zeros((8, 128), F32)], axis=0).astype(BF16)
        vb[a, KROWS:640, :] = jnp.zeros((640 - KROWS, 256), BF16)

    lane0 = lax.broadcasted_iota(jnp.int32, (128, 128), 1) == 0

    def b_inverse(c, carry):
        @pl.when(c == 0)
        def _():
            for n in range(4):
                cp_wo(n).start()

        lhs = [[] for _ in range(4)]
        for half in range(2):
            a = 2 * c + half
            z = lax.dot_general(sm[a], vb[a, 0:512, :], NT, preferred_element_type=F32)
            ny = lax.dot_general(sm[a, 0:128, :], vb[a, 512:640, :], NT,
                                 preferred_element_type=F32)
            for k in range(4):
                zr, zi = z[0:128, 128 * k:128 * (k + 1)], z[128:256, 128 * k:128 * (k + 1)]
                if k == 0:
                    zi = jnp.where(lane0, ny, zi)
                lhs[k].append(jnp.concatenate([zr, zi], axis=1).astype(BF16))
        g = [jnp.dot(jnp.concatenate(lhs[k], axis=0), d_ref[k], preferred_element_type=F32)
             for k in range(4)]
        (g0, g4), (g1r, g1i), (g2r, g2i), (g3r, g3i) = [(v[:, :128], v[:, 128:]) for v in g]
        e, o = g0 + g4, g0 - g4
        s = [e + g2r, o + g2i, e - g2r, o - g2i]
        p, q = (g1r - g3r) * rt, (g1i - g3i) * rt
        d = [g1r + g3r, q + p, g1i + g3i, q - p]
        y = [s[i] + d[i] for i in range(4)] + [s[i] - d[i] for i in range(4)]
        for al in range(8):
            bits = _bf16_bits(y[al])
            xw[c, :, :, 128 * al:128 * (al + 1)] = (
                (bits[0:128] >> 16) | bits[128:256]).reshape(8, 16, 128)
        return carry

    lax.fori_loop(0, 8, b_inverse, 0)

    def halves(v):
        n = v.shape[1] // 256
        return [jnp.concatenate([v[:, 256 * i + 128 * k:256 * i + 128 * (k + 1)]
                                 for i in range(n)], axis=1) for k in range(2)]

    def load_x(t):
        for g in range(G // 2):
            top, bot = ax[t, g].astype(F32), ax[t, g + G // 2].astype(F32)
            for n, v in enumerate(_lhs7(*halves(top), *halves(bot))):
                hs[n, SEG * g:SEG * (g + 1), :] = v

    def set_mem(m):
        for n, v in enumerate(_lhs7(*halves(m[0:MH]), *halves(m[MH:2 * MH]))):
            hs[n, XH:HH, :] = v

    def project(p, r0, r1, lo, hi, first=False):
        if first:
            m = [0.0] * 7
            for i in range(4):
                w = []
                for j in range(lo, hi):
                    w1, w2 = wqkv[j][p, i, 0:128, :], wqkv[j][p, i, 128:256, :]
                    w.append(_rhs7(_lo(w1), _hi(w1), _lo(w2), _hi(w2)))
                    for n in range(7):
                        wqkv[j][p, i, 64 * n:64 * (n + 1), :] = pltpu.bitcast(w[-1][n], U32)
                for n in range(7):
                    r = jnp.dot(hs[n, r0:r1, 128 * i:128 * (i + 1)],
                                jnp.concatenate([v[n] for v in w], axis=1),
                                preferred_element_type=F32)
                    m[n] = r if i == 0 else m[n] + r
        else:
            m = []
            for n in range(7):
                w = [pltpu.bitcast(wqkv[j][p, :, 64 * n:64 * (n + 1), :], BF16)
                     .reshape(DM // 2, DH) for j in range(lo, hi)]
                m.append(jnp.dot(hs[n, r0:r1, :], jnp.concatenate(w, axis=1),
                                 preferred_element_type=F32))
        c11, c12, c21, c22 = _out4(m)
        return (c11, c21), (c12, c22)

    def put_o(p, r0, o):
        for n, v in enumerate(_lhs7(o[0][0], o[1][0], o[0][1], o[1][1])):
            ob[n, p, r0:HH, :] = v

    def out_proj(c, r0, first):
        def cols(n, size=256):
            return pl.ds(pl.multiple_of((c * 7 + n) * 256, 256), size)

        if first:
            def one_pair(p, m):
                w = wo[p, :, cols(0, 1024)].astype(F32)
                b = [jnp.concatenate([w[:, 512 * e + 256 * i + 128 * k:][:, :128]
                                      for i in range(2)], axis=1)
                     for e in range(2) for k in range(2)]
                out = []
                for n, v in enumerate(_rhs7(*b)):
                    wo[p, :, cols(n)] = v
                    out.append(m[n] + jnp.dot(ob[n, p, r0:HH, :], v, preferred_element_type=F32))
                return out

            m = lax.fori_loop(0, NP, one_pair, [jnp.zeros((HH - r0, 256), F32)] * 7, unroll=2)
        else:
            m = []
            for n in range(7):
                o = jnp.concatenate([ob[n, p, r0:HH, :] for p in range(NP)], axis=1)
                m.append(jnp.dot(o, wo[:, :, cols(n)].reshape(NP * DH, 256),
                                 preferred_element_type=F32))
        return _out4(m)

    def weave(a, b):
        return jnp.concatenate([a[:, 0:128], b[:, 0:128], a[:, 128:256], b[:, 128:256]], axis=1)

    def out_mem(c, r0, keep, feed, first=False):
        c11, c12, c21, c22 = out_proj(c, r0, first)
        x0 = XH - r0
        if keep:
            cols = pl.ds(pl.multiple_of(512 * c, 512), 512)
            mend[0:MH, cols] = weave(c11[x0:], c12[x0:])
            mend[MH:2 * MH, cols] = weave(c21[x0:], c22[x0:])
        if feed:
            for n, v in enumerate(_lhs7(c11[x0:], c12[x0:], c21[x0:], c22[x0:])):
                hs[n, XH:HH, pl.ds(pl.multiple_of(256 * c, 256), 256)] = v
        return weave(c11[:x0], c12[:x0]), weave(c21[:x0], c22[:x0])

    cp_ax(T - 1).wait()
    load_x(T - 1)

    def kv_loop(p, carry):
        cp_w(0, p).start()
        cp_w(1, p).wait()
        cp_w(2, p).wait()
        r = project(p, 0, XH, 1, 3, first=True)
        for e in range(2):
            v = jnp.concatenate(r[e], axis=0).astype(BF16)
            kret[p, e] = v[:, 0:DH]
            vret[p, e] = v[:, DH:2 * DH]
        return carry

    lax.fori_loop(0, NP, kv_loop, 0)

    cp_ax(T - 2).wait()
    xbar = jnp.sum(ax[T - 2].astype(F32), axis=1, keepdims=True) * (1.0 / (SEG + MEM))
    set_mem(jnp.broadcast_to(xbar, (G, MEM, DM)).reshape(G * MEM, DM))

    def guess(p, carry):
        put_o(p, XH, project(p, XH, HH, 2, 3))
        return carry

    lax.fori_loop(0, NP, guess, 0, unroll=2)
    for n in range(4):
        cp_wo(n).wait()
    lax.fori_loop(0, 2, lambda c, carry: (out_mem(c, XH, False, True, True), carry)[1], 0)

    TILES = ((0, 1, 2), (3, 4, 5), (6, 7))
    nx = [SEG * len(tl) for tl in TILES]
    nm = (32, 32, 16)

    def tile(v, g, with_x):
        m0 = XH if with_x else 0
        parts = [v[ch // 4][SEG * (ch % 4):SEG * (ch % 4 + 1)] for ch in TILES[g]] if with_x else []
        parts += [v[ch // 4][m0 + MEM * (ch % 4):m0 + MEM * (ch % 4 + 1)] for ch in TILES[g]]
        if len(TILES[g]) == 3:
            parts.append(jnp.zeros((MEM, DH), F32))
        return jnp.concatenate(parts, axis=0).astype(BF16)

    def step(mode):
        q_x, kv_x = mode != "pred", mode == "mid"
        q0, kv0 = (0 if q_x else XH), (0 if kv_x else XH)

        def put(ref, e, v, with_x):
            for g in range(3):
                ref[e, g, (0 if with_x else nx[g]):nx[g] + nm[g], :] = tile(v, g, with_x)

        def proj_qk(p):
            if mode == "mid":
                r = project(p, q0, HH, 0, 2)
                q = [[v[:, 0:DH] for v in r[e]] for e in range(2)]
                k = [[v[:, DH:2 * DH] for v in r[e]] for e in range(2)]
            else:
                q = project(p, q0, HH, 0, 1, first=mode == "pred")
                k = project(p, kv0, HH, 1, 2)
            for e in range(2):
                put(qt, e, [v * QSCALE for v in q[e]], q_x)
                put(kt, e, k[e], kv_x)

        def proj_v(p):
            v = project(p, kv0, HH, 2, 3)
            for e in range(2):
                put(vt, e, v[e], kv_x)

        def get(ref, ret, p, e, g):
            if kv_x:
                return ref[e, g]
            return jnp.concatenate([ret[p, e, 96 * g:96 * g + nx[g], :], ref[e, g, nx[g]:128, :]],
                                   axis=0)

        def scores(p, e):
            out = []
            for g in range(3):
                r0 = 0 if q_x else nx[g]
                s = lax.dot_general(qt[e, g, r0:nx[g] + nm[g], :], get(kt, kret, p, e, g), NT,
                                    preferred_element_type=F32)
                fill = mask_ref[g // 2, r0:nx[g] + nm[g], :]
                s = jnp.where(fill == 0.0, s, fill)
                pr = jnp.exp2(s - jnp.max(s, axis=1, keepdims=True))
                out.append((pr.astype(BF16), jnp.sum(pr, axis=1, keepdims=True)))
            return out

        def values(p, e, sc):
            xs, ms = [], []
            for g in range(3):
                pr, den = sc[g]
                o = jnp.dot(pr, get(vt, vret, p, e, g), preferred_element_type=F32) / den
                m0 = nx[g] if q_x else 0
                for i in range(len(TILES[g])):
                    if q_x:
                        xs.append(o[SEG * i:SEG * (i + 1)])
                    ms.append(o[m0 + MEM * i:m0 + MEM * (i + 1)])
            return [jnp.concatenate(xs[4 * k:4 * k + 4] + ms[4 * k:4 * k + 4], axis=0)
                    for k in range(2)]

        def pair(p, nxt=True):
            sc = [scores(p, e) for e in range(2)]
            if nxt:
                proj_qk(p + 1)
            put_o(p, q0, [values(p, e, sc[e]) for e in range(2)])
            if nxt:
                proj_v(p + 1)

        return proj_qk, proj_v, pair

    kt[:, 2, 80:128, :] = jnp.zeros((2, 48, DH), BF16)
    vt[:, 2, 80:128, :] = jnp.zeros((2, 48, DH), BF16)

    proj_qk, proj_v, pair = step("pred")
    cp_w(0, 0).wait()
    proj_qk(0)
    proj_v(0)

    def pred_loop(p, carry):
        cp_w(0, p + 1).wait()
        pair(p)
        return carry

    for t in range(T - 2):
        cp_ax(t).start()
    lax.fori_loop(0, NP - 1, pred_loop, 0)
    pair(NP - 1, False)
    lax.fori_loop(0, 2, lambda c, carry: (out_mem(c, XH, True, False), carry)[1], 0)
    for t in range(T - 2):
        cp_ax(t).wait()
    for c in range(8):
        cp_by(c).start()

    proj_qk, proj_v, pair = step("mid")
    pair_last = step("last")[2]

    def pairs(fn):
        def pair_loop(i, carry):
            fn(2 * i + 1)
            fn(2 * i + 2)
            return carry

        lax.fori_loop(0, NP // 2 - 1, pair_loop, 0)

    def segment(t, carry):
        load_x(t)
        proj_qk(0)
        proj_v(0)
        pair(0)

        @pl.when(t < T - 1)
        def _():
            pairs(pair)

        @pl.when(t == T - 1)
        def _():
            pairs(pair_last)
            for e in range(2):
                for g in range(3):
                    kt[e, g, 0:nx[g], :] = kret[NP - 1, e, 96 * g:96 * g + nx[g], :]
                    vt[e, g, 0:nx[g], :] = vret[NP - 1, e, 96 * g:96 * g + nx[g], :]

        pair(NP - 1, False)
        for c in range(2):
            top, bot = out_mem(c, 0, True, True)
            cols = slice(512 * c, 512 * (c + 1))
            ostage[t, 0:G // 2, :, :, cols] = top.astype(BF16).reshape(G // 2, 2, 16, 512)
            ostage[t, G // 2:G, :, :, cols] = bot.astype(BF16).reshape(G // 2, 2, 16, 512)
        cp_ao(t).start()
        return carry

    def one_pass(carry):
        it, _ = carry
        start = mend[0:(G - 1) * MEM, :]
        mstart[...] = start
        set_mem(jnp.concatenate([mem0_ref[...].astype(F32), start], axis=0))
        lax.fori_loop(0, T, segment, 0)
        real = mend[0:(G - 1) * MEM, :]
        lim = jnp.max(jnp.abs(real), axis=1, keepdims=True) * TOL
        good = jnp.abs(real - mstart[...]) <= lim
        bad = jnp.max(jnp.where(good, 0.0, 1.0))
        for t in range(T):
            cp_ao(t).wait()
        return it + 1, bad

    lax.while_loop(lambda c: jnp.logical_and(c[0] < G, c[1] > 0.0), one_pass,
                   (jnp.int32(0), jnp.float32(1.0)))
    for c in range(8):
        cp_by(c).wait()


@functools.partial(jax.jit, static_argnames=("A_seg_len",))
def pallas_concat_heads__memory_aug_recurrent_mem_tr__spectral_gfnet__prompt_kernel(
    A_x, A_mem0, A_Wq, A_Wk, A_Wv, A_Wo, A_seg_len, B_x, B_w_r, B_w_i,
):
    assert A_seg_len == SEG and A_x.shape == (1, G * T * SEG, DM) and A_Wq.shape == (DM, NH, DH)
    assert A_mem0.shape == (1, MEM, DM) and B_x.shape == (1, 2048, 1024)
    dmat, smat, mask = _constants()
    wr_t, wi_t = B_w_r.T, B_w_i.T
    hbm = pl.BlockSpec(memory_space=pl.ANY)
    nyq = pl.BlockSpec((16, 2048), lambda i: (32, 0))

    def full(shape):
        return pl.BlockSpec(shape, lambda i: (0,) * len(shape))

    out = pl.pallas_call(
        _kernel,
        grid=(1,),
        in_specs=[hbm] * 9 + [full((MEM, DM)), nyq, nyq, full(dmat.shape), full(mask.shape)],
        out_specs=hbm,
        out_shape=jax.ShapeDtypeStruct((G, 16, 16, 2 * DM), BF16),
        scratch_shapes=[
            pltpu.VMEM((T, G, SEG, DM), BF16),
            *[pltpu.VMEM((NP, 4, 7 * 64, DH), U32)] * 3,
            pltpu.VMEM((NP, DH, 7 * 512), BF16),
            pltpu.VMEM((8, 8, 16, 1024), U32),
            pltpu.VMEM((16, 256, 128), U32),
            pltpu.VMEM((16, 256, 128), U32),
            pltpu.VMEM((16, 256, 256), BF16),
            pltpu.VMEM((16, KROWS, 256), F32),
            pltpu.VMEM((16, 640, 256), BF16),
            pltpu.VMEM((NP, 2, G * SEG, DH), BF16),
            pltpu.VMEM((NP, 2, G * SEG, DH), BF16),
            pltpu.VMEM((7, HH, DM // 2), BF16),
            pltpu.VMEM((2, 3, 128, DH), BF16),
            pltpu.VMEM((2, 3, 128, DH), BF16),
            pltpu.VMEM((2, 3, 128, DH), BF16),
            pltpu.VMEM((7, NP, HH, DH), BF16),
            pltpu.VMEM(((G - 1) * MEM, DM), F32),
            pltpu.VMEM((G * MEM, DM), F32),
            pltpu.VMEM((T, G, 2, 16, DM), BF16),
            pltpu.SemaphoreType.DMA((3, 8)),
            pltpu.SemaphoreType.DMA((3, NP)),
            pltpu.SemaphoreType.DMA((6,)),
            pltpu.SemaphoreType.DMA((2, T)),
        ],
        compiler_params=pltpu.CompilerParams(
            dimension_semantics=("arbitrary",), vmem_limit_bytes=120 * 1024 * 1024),
    )(
        A_x.reshape(G, T, SEG, DM),
        A_Wq.reshape(4, 256, NH, DH), A_Wk.reshape(4, 256, NH, DH), A_Wv.reshape(4, 256, NH, DH),
        A_Wo.reshape(NP, 2, DH, DM), B_x.reshape(8, 16, 16, 1024), wr_t, wi_t, smat,
        A_mem0.reshape(MEM, DM), wr_t, wi_t, dmat, mask,
    )
    return out.reshape(1, 2048, 2 * DM)
```

```python
import functools

import jax
import jax.numpy as jnp
import numpy as np
from jax import lax
from jax.experimental import pallas as pl
from jax.experimental.pallas import tpu as pltpu

F32 = jnp.float32
BF16 = jnp.bfloat16
U32 = jnp.uint32

G = 8
T = 8
SEG = 32
MEM = 8
DM = 1024
NH = 32
DH = 128
NP = NH // 2
XH = G // 2 * SEG
MH = G // 2 * MEM
HH = XH + MH
LOG2E = 1.4426950408889634
QSCALE = float(DH ** -0.5 * LOG2E)
MASKED = float(-1e9 * LOG2E)
TOL = 2.0 ** -9
NT = (((1,), (1,)), ((), ()))
KROWS = 528
ROW_OFF = {0: 0, 4: 64, 1: 128, 7: 192, 2: 256, 6: 320, 3: 384, 5: 448}


def _constants():
    beta = np.arange(128)[None, :]
    m = np.arange(64)[:, None]
    d = np.zeros((4, 256, 256))
    for blk, r in enumerate((0, 4)):
        th = 2 * np.pi * (8 * m + r) * beta / 1024
        d[0, 64 * blk:64 * blk + 64, 128 * blk:128 * blk + 128] = np.cos(th)
        d[0, 128 + 64 * blk:192 + 64 * blk, 128 * blk:128 * blk + 128] = -np.sin(th)
    d[0, 128, 0:128] = np.cos(np.pi * np.arange(128))
    for r, sg in ((1, -1.0), (2, -1.0), (3, 1.0)):
        for blk, (res, cj) in enumerate(((r, 1.0), (8 - r, -1.0))):
            th = 2 * np.pi * (8 * m + res) * beta / 1024
            re, im = slice(64 * blk, 64 * blk + 64), slice(128 + 64 * blk, 192 + 64 * blk)
            d[r, re, 0:128] = np.cos(th)
            d[r, im, 0:128] = -np.sin(th)
            d[r, re, 128:256] = sg * cj * np.sin(th)
            d[r, im, 128:256] = sg * cj * np.cos(th)
    d *= 2.0 ** -10
    b = np.arange(128)[:, None]
    kb = np.arange(128)[None, :]
    s = np.zeros((16, 256, 256))
    for a in range(16):
        th = 2 * np.pi * ((kb * (16 * b + a)) % 2048) / 2048
        s[a, :128, :128] = np.cos(th)
        s[a, 128:, :128] = np.sin(th)
        s[a, :128, 128:] = -np.sin(th)
        s[a, 128:, 128:] = np.cos(th)
    mask = np.zeros((2, 128, 128), np.float32)
    for i, ns in enumerate((3, 2)):
        idx = np.arange(128)
        isx = idx < SEG * ns
        pad = idx >= (SEG + MEM) * ns
        seg = np.where(isx, idx // SEG, (idx - SEG * ns) // MEM)
        same = (seg[:, None] == seg[None, :]) & ~pad[None, :]
        future = isx[:, None] & isx[None, :] & (idx[None, :] > idx[:, None])
        mk = np.where(same, np.where(future, MASKED, 0.0), -np.inf)
        mask[i] = np.where(pad[:, None], 0.0, mk)
    return d.astype(BF16), s.astype(BF16), mask


def _lo(w):
    return lax.bitcast_convert_type(w << 16, F32)


def _hi(w):
    return lax.bitcast_convert_type(w & np.uint32(0xFFFF0000), F32)


def _bf16_bits(y):
    return lax.bitcast_convert_type(y.astype(BF16).astype(F32), U32)


def _r4(x, sg):
    (ar, ai), (br, bi), (cr, ci), (dr, di) = x
    s0r, s0i, d0r, d0i = ar + cr, ai + ci, ar - cr, ai - ci
    s1r, s1i, d1r, d1i = br + dr, bi + di, br - dr, bi - di
    p = (d0r - d1i, d0i + d1r)
    q = (d0r + d1i, d0i - d1r)
    y1, y3 = (p, q) if sg > 0 else (q, p)
    return [(s0r + s1r, s0i + s1i), y1, (s0r - s1r, s0i - s1i), y3]


def _tw(z, e, sg):
    r, i = z
    if e == 0:
        return z
    if e == 4:
        return (-i, r) if sg > 0 else (i, -r)
    h = float(np.sqrt(0.5))
    if e == 2:
        return ((r - i) * h, (r + i) * h) if sg > 0 else ((r + i) * h, (i - r) * h)
    if e == 6:
        return ((r + i) * -h, (r - i) * h) if sg > 0 else ((i - r) * h, (r + i) * -h)
    c = float(np.cos(2 * np.pi * e / 16))
    s = float(sg * np.sin(2 * np.pi * e / 16))
    return (r * c - i * s, r * s + i * c)


def _fft16(x, sg):
    t = [_r4([x[4 * a1 + a0] for a1 in range(4)], sg) for a0 in range(4)]
    out = [None] * 16
    for k0 in range(4):
        u = _r4([_tw(t[a0][k0], a0 * k0, sg) for a0 in range(4)], sg)
        for k1 in range(4):
            out[k0 + 4 * k1] = u[k1]
    return out


def _lhs7(a11, a12, a21, a22):
    return [a21 + a22, a11, a22, a11 + a12, a11 + a22, a21 - a11, a12 - a22]


def _rhs7(b11, b12, b21, b22):
    return [b11, b12 - b22, b21 - b11, b22, b11 + b22, b11 + b12, b21 + b22]


def _words(even, odd):
    return pltpu.pack_elementwise([even, odd], packed_dtype=BF16)


def _out4(m):
    return m[4] + m[2] - m[3] + m[6], m[1] + m[3], m[0] + m[2], m[4] - m[0] + m[1] + m[5]


def _kernel(ax_hbm, wq_hbm, wk_hbm, wv_hbm, wo_hbm, bx_hbm, wr_hbm, wi_hbm, s_hbm,
            mem0_ref, wrn_ref, win_ref, d_ref, mask_ref,
            out_hbm,
            ax, wq, wk, wv, wo, xw, wr, wi, sm, yb, vb, kret, vret, hs, qt, kt, vt, ob,
            mstart, mend, ostage, sem_b, sem_w, sem_m, sem_o):
    wqkv = (wq, wk, wv)

    def cp_bx(c):
        return pltpu.make_async_copy(bx_hbm.bitcast(U32).at[:, :, c, :], xw.at[c], sem_b.at[0, c])

    def cp_s(c):
        sl = pl.ds(2 * c, 2)
        return pltpu.make_async_copy(s_hbm.at[sl], sm.at[sl], sem_b.at[1, c])

    def cp_by(c):
        return pltpu.make_async_copy(
            xw.at[c], out_hbm.bitcast(U32).at[:, :, c, pl.ds(DM, DM)], sem_b.at[2, c])

    def cp_w(j, p):
        src = (wq_hbm, wk_hbm, wv_hbm)[j]
        return pltpu.make_async_copy(src.bitcast(U32).at[:, :, p, :],
                                     wqkv[j].at[p, :, pl.ds(0, 256), :], sem_w.at[j, p])

    def cp_wo(n):
        c, e = divmod(n, 2)
        return pltpu.make_async_copy(wo_hbm.bitcast(U32).at[:, e, :, pl.ds(512 * c, 512)],
                                     wo.at[:, :, pl.ds(1792 * c + 512 * e, 512)], sem_m.at[2 + n])

    def cp_ax(t):
        return pltpu.make_async_copy(ax_hbm.bitcast(U32).at[:, t], ax.at[t], sem_o.at[1, t])

    def cp_ao(t):
        return pltpu.make_async_copy(
            ostage.at[t], out_hbm.at[:, pl.ds(2 * t, 2), :, pl.ds(0, DM)], sem_o.at[0, t])

    def cp_f(j, k):
        src, dst = ((wr_hbm, wr), (wi_hbm, wi))[j]
        return pltpu.make_async_copy(
            src.at[pl.ds(0, 512), pl.ds(pl.multiple_of(128 * k, 128), 128)].bitcast(U32),
            dst.at[k], sem_m.at[j])

    for c in range(2):
        cp_bx(c).start()
        cp_s(c).start()

    rt = float(np.sqrt(0.5))
    row8 = lax.broadcasted_iota(jnp.int32, (8, 128), 0)

    def b_forward(c, carry):
        @pl.when(c < 6)
        def _():
            cp_bx(c + 2).start()
            cp_s(c + 2).start()

        for j in range(2):
            cp_f(j, 2 * c).start()
            cp_f(j, 2 * c + 1).start()

        @pl.when(c == 7)
        def _():
            cp_ax(T - 1).start()
            cp_ax(T - 2).start()

        cp_bx(c).wait()
        cp_s(c).wait()
        w = xw[c].reshape(128, DM)
        for half, xf in enumerate((_lo(w), _hi(w))):
            x = [xf[:, 128 * al:128 * (al + 1)] for al in range(8)]
            s = [x[i] + x[i + 4] for i in range(4)]
            d = [x[i] - x[i + 4] for i in range(4)]
            e, o = s[0] + s[2], s[1] + s[3]
            p, q = (d[1] - d[3]) * rt, (d[1] + d[3]) * rt
            u = [(e + o, e - o), (d[0] + p, d[2] + q), (s[0] - s[2], s[1] - s[3]),
                 (d[0] - p, d[2] - q)]
            tt = [lax.dot_general(d_ref[k], jnp.concatenate(u[k], axis=1).astype(BF16), NT,
                                  preferred_element_type=F32) for k in range(4)]
            dc, ny = tt[0][0:8], tt[0][128:136]
            re = [jnp.where(row8 == 0, dc * 0.5, dc), tt[0][8:128]]
            im = [jnp.where(row8 == 0, 0.0, ny), tt[0][136:256]]
            for k in range(1, 4):
                re.append(tt[k][0:128])
                im.append(tt[k][128:256])
            re += [jnp.where(row8 == 0, ny * 0.5, 0.0), jnp.zeros((8, 128), F32)]
            im.append(jnp.zeros((16, 128), F32))
            lhs = jnp.concatenate([jnp.concatenate(re, axis=0), jnp.concatenate(im, axis=0)],
                                  axis=1).astype(BF16)
            a = 2 * c + half
            yb[a] = jnp.dot(lhs, sm[a], preferred_element_type=F32)
        return carry

    lax.fori_loop(0, 8, b_forward, 0)
    pltpu.make_async_copy(wr, wr, sem_m.at[0]).wait()
    pltpu.make_async_copy(wi, wi, sem_m.at[1]).wait()

    def filt(row, wre, wim):
        y = [(yb[a, pl.ds(row, 8), 0:128], yb[a, pl.ds(row, 8), 128:256]) for a in range(16)]
        z = _fft16(y, -1)
        z = [(z[k][0] * wre(k) - z[k][1] * wim(k), z[k][0] * wim(k) + z[k][1] * wre(k))
             for k in range(16)]
        return _fft16(z, 1)

    def b_filter(i, carry):
        mg, j = i // 4, i % 4
        cp_w(1, i).start()
        cp_w(2, i).start()
        for half, un in enumerate((_lo, _hi)):
            off = [ROW_OFF[2 * jj + half] for jj in range(4)]
            base = jnp.where(j < 2, jnp.where(j == 0, off[0], off[1]),
                             jnp.where(j == 2, off[2], off[3])) + 16 * mg
            base = pl.multiple_of(base, 16)
            res = []
            for r8 in range(2):
                sl = pl.ds(64 * mg + 32 * r8 + j, 8, stride=4)
                res.append(filt(pl.multiple_of(base + 8 * r8, 8),
                                lambda k: un(wr[k, sl, :]),
                                lambda k: un(wi[k, sl, :])))
            for a in range(16):
                for ri in range(2):
                    vb[a, pl.ds(base, 16), 128 * ri:128 * (ri + 1)] = jnp.concatenate(
                        [res[0][a][ri], res[1][a][ri]], axis=0).astype(BF16)
        return carry

    lax.fori_loop(0, 16, b_filter, 0)
    res = filt(512, lambda k: wrn_ref[0:1, 128 * k:128 * (k + 1)].astype(F32),
               lambda k: win_ref[0:1, 128 * k:128 * (k + 1)].astype(F32))
    for a in range(16):
        for ri in range(2):
            vb[a, 512:KROWS, 128 * ri:128 * (ri + 1)] = jnp.concatenate(
                [res[a][ri], jnp.zeros((8, 128), F32)], axis=0).astype(BF16)
        vb[a, KROWS:640, :] = jnp.zeros((640 - KROWS, 256), BF16)

    lane0 = lax.broadcasted_iota(jnp.int32, (128, 128), 1) == 0

    def b_inverse(c, carry):
        @pl.when(c == 0)
        def _():
            for n in range(4):
                cp_wo(n).start()

        lhs = [[] for _ in range(4)]
        for half in range(2):
            a = 2 * c + half
            z = lax.dot_general(sm[a], vb[a, 0:512, :], NT, preferred_element_type=F32)
            ny = lax.dot_general(sm[a, 0:128, :], vb[a, 512:640, :], NT,
                                 preferred_element_type=F32)
            for k in range(4):
                zr, zi = z[0:128, 128 * k:128 * (k + 1)], z[128:256, 128 * k:128 * (k + 1)]
                if k == 0:
                    zi = jnp.where(lane0, ny, zi)
                lhs[k].append(jnp.concatenate([zr, zi], axis=1).astype(BF16))
        g = [jnp.dot(jnp.concatenate(lhs[k], axis=0), d_ref[k], preferred_element_type=F32)
             for k in range(4)]
        (g0, g4), (g1r, g1i), (g2r, g2i), (g3r, g3i) = [(v[:, :128], v[:, 128:]) for v in g]
        e, o = g0 + g4, g0 - g4
        s = [e + g2r, o + g2i, e - g2r, o - g2i]
        p, q = (g1r - g3r) * rt, (g1i - g3i) * rt
        d = [g1r + g3r, q + p, g1i + g3i, q - p]
        y = [s[i] + d[i] for i in range(4)] + [s[i] - d[i] for i in range(4)]
        for al in range(8):
            bits = _bf16_bits(y[al])
            xw[c, :, :, 128 * al:128 * (al + 1)] = (
                (bits[0:128] >> 16) | bits[128:256]).reshape(8, 16, 128)
        return carry

    lax.fori_loop(0, 8, b_inverse, 0)

    def halves(v):
        n = v.shape[1] // 256
        return [jnp.concatenate([v[:, 256 * i + 128 * k:256 * i + 128 * (k + 1)]
                                 for i in range(n)], axis=1) for k in range(2)]

    def load_x(t):
        for g in range(G // 2):
            top, bot = ax[t, g], ax[t, g + G // 2]
            ev, od = [_lhs7(*halves(un(top)), *halves(un(bot))) for un in (_lo, _hi)]
            for n in range(7):
                hs[n, SEG // 2 * g:SEG // 2 * (g + 1), :] = _words(ev[n], od[n])

    def set_mem(m):
        for n, v in enumerate(_lhs7(*halves(m[0:MH]), *halves(m[MH:2 * MH]))):
            hs[n, XH // 2:HH // 2, :] = pltpu.bitcast(v.astype(BF16), U32)

    def project(p, r0, r1, lo, hi, first=False):
        if first:
            m = [0.0] * 7
            for i in range(4):
                w = []
                for j in range(lo, hi):
                    raw = [[wqkv[j][p, i, pl.ds(128 * k + d, 64, stride=2), :] for k in range(2)]
                           for d in range(2)]
                    ev, od = [_rhs7(_lo(w1), _hi(w1), _lo(w2), _hi(w2)) for w1, w2 in raw]
                    w.append([_words(ev[n], od[n]) for n in range(7)])
                    for n in range(7):
                        wqkv[j][p, i, 64 * n:64 * (n + 1), :] = w[-1][n]
                for n in range(7):
                    r = jnp.dot(
                        pltpu.bitcast(hs[n, r0 // 2:r1 // 2, 128 * i:128 * (i + 1)], BF16),
                        pltpu.bitcast(jnp.concatenate([v[n] for v in w], axis=1), BF16),
                        preferred_element_type=F32)
                    m[n] = r if i == 0 else m[n] + r
        else:
            m = []
            for n in range(7):
                w = [pltpu.bitcast(wqkv[j][p, :, 64 * n:64 * (n + 1), :], BF16)
                     .reshape(DM // 2, DH) for j in range(lo, hi)]
                m.append(jnp.dot(pltpu.bitcast(hs[n, r0 // 2:r1 // 2, :], BF16),
                                 jnp.concatenate(w, axis=1), preferred_element_type=F32))
        c11, c12, c21, c22 = _out4(m)
        return (c11, c21), (c12, c22)

    def put_o(p, r0, o):
        for n, v in enumerate(_lhs7(o[0][0], o[1][0], o[0][1], o[1][1])):
            ob[n, p, r0:HH, :] = v.astype(BF16)

    def out_proj(c, r0, first):
        def cols(n, size=256):
            return pl.ds(pl.multiple_of((c * 7 + n) * 256, 256), size)

        if first:
            def one_pair(p, m):
                for r in range(0, DH // 2, 16):
                    w = wo[p, r:r + 16, cols(0, 1024)]
                    b = halves(w[:, 0:512]) + halves(w[:, 512:1024])
                    ev, od = [_rhs7(*[un(v) for v in b]) for un in (_lo, _hi)]
                    for n in range(7):
                        wo[p, r:r + 16, cols(n)] = _words(ev[n], od[n])
                return [m[n] + jnp.dot(ob[n, p, r0:HH, :], pltpu.bitcast(wo[p, :, cols(n)], BF16),
                                       preferred_element_type=F32) for n in range(7)]

            m = lax.fori_loop(0, NP, one_pair, [jnp.zeros((HH - r0, 256), F32)] * 7, unroll=2)
        else:
            m = []
            for n in range(7):
                o = jnp.concatenate([ob[n, p, r0:HH, :] for p in range(NP)], axis=1)
                w = pltpu.bitcast(wo[:, :, cols(n)], BF16).reshape(NP * DH, 256)
                m.append(jnp.dot(o, w, preferred_element_type=F32))
        return _out4(m)

    def weave(a, b):
        return jnp.concatenate([a[:, 0:128], b[:, 0:128], a[:, 128:256], b[:, 128:256]], axis=1)

    def out_mem(c, r0, keep, feed, first=False):
        c11, c12, c21, c22 = out_proj(c, r0, first)
        x0 = XH - r0
        if keep:
            cols = pl.ds(pl.multiple_of(512 * c, 512), 512)
            mend[0:MH, cols] = weave(c11[x0:], c12[x0:])
            mend[MH:2 * MH, cols] = weave(c21[x0:], c22[x0:])
        if feed:
            for n, v in enumerate(_lhs7(c11[x0:], c12[x0:], c21[x0:], c22[x0:])):
                hs[n, XH // 2:HH // 2, pl.ds(pl.multiple_of(256 * c, 256), 256)] = (
                    pltpu.bitcast(v.astype(BF16), U32))
        return weave(c11[:x0], c12[:x0]), weave(c21[:x0], c22[:x0])

    cp_ax(T - 1).wait()
    load_x(T - 1)

    def kv_loop(p, carry):
        cp_w(0, p).start()
        cp_w(1, p).wait()
        cp_w(2, p).wait()
        r = project(p, 0, XH, 1, 3, first=True)
        for e in range(2):
            v = jnp.concatenate(r[e], axis=0).astype(BF16)
            kret[p, e] = v[:, 0:DH]
            vret[p, e] = v[:, DH:2 * DH]
        return carry

    lax.fori_loop(0, NP, kv_loop, 0)

    cp_ax(T - 2).wait()
    xbar = jnp.sum(_lo(ax[T - 2]) + _hi(ax[T - 2]), axis=1, keepdims=True) * (1.0 / (SEG + MEM))
    set_mem(jnp.broadcast_to(xbar, (G, MEM, DM)).reshape(G * MEM, DM))

    def guess(p, carry):
        put_o(p, XH, project(p, XH, HH, 2, 3))
        return carry

    lax.fori_loop(0, NP, guess, 0, unroll=2)
    for n in range(4):
        cp_wo(n).wait()
    lax.fori_loop(0, 2, lambda c, carry: (out_mem(c, XH, False, True, True), carry)[1], 0)

    TILES = ((0, 1, 2), (3, 4, 5), (6, 7))
    nx = [SEG * len(tl) for tl in TILES]
    nm = (32, 32, 16)

    def tile(v, g, with_x):
        m0 = XH if with_x else 0
        parts = [v[ch // 4][SEG * (ch % 4):SEG * (ch % 4 + 1)] for ch in TILES[g]] if with_x else []
        parts += [v[ch // 4][m0 + MEM * (ch % 4):m0 + MEM * (ch % 4 + 1)] for ch in TILES[g]]
        if len(TILES[g]) == 3:
            parts.append(jnp.zeros((MEM, DH), F32))
        return jnp.concatenate(parts, axis=0).astype(BF16)

    def step(mode):
        q_x, kv_x = mode != "pred", mode == "mid"
        q0, kv0 = (0 if q_x else XH), (0 if kv_x else XH)

        def put(ref, e, v, with_x):
            for g in range(3):
                ref[e, g, (0 if with_x else nx[g]):nx[g] + nm[g], :] = tile(v, g, with_x)

        def proj_qk(p):
            if mode == "mid":
                r = project(p, q0, HH, 0, 2)
                q = [[v[:, 0:DH] for v in r[e]] for e in range(2)]
                k = [[v[:, DH:2 * DH] for v in r[e]] for e in range(2)]
            else:
                q = project(p, q0, HH, 0, 1, first=mode == "pred")
                k = project(p, kv0, HH, 1, 2)
            for e in range(2):
                put(qt, e, [v * QSCALE for v in q[e]], q_x)
                put(kt, e, k[e], kv_x)

        def proj_v(p):
            v = project(p, kv0, HH, 2, 3)
            for e in range(2):
                put(vt, e, v[e], kv_x)

        def get(ref, ret, p, e, g):
            if kv_x:
                return ref[e, g]
            return jnp.concatenate([ret[p, e, 96 * g:96 * g + nx[g], :], ref[e, g, nx[g]:128, :]],
                                   axis=0)

        def scores(p, e):
            out = []
            for g in range(3):
                r0 = 0 if q_x else nx[g]
                s = lax.dot_general(qt[e, g, r0:nx[g] + nm[g], :], get(kt, kret, p, e, g), NT,
                                    preferred_element_type=F32)
                fill = mask_ref[g // 2, r0:nx[g] + nm[g], :]
                s = jnp.where(fill == 0.0, s, fill)
                pr = jnp.exp2(s - jnp.max(s, axis=1, keepdims=True))
                out.append((pr.astype(BF16), jnp.sum(pr, axis=1, keepdims=True)))
            return out

        def values(p, e, sc):
            xs, ms = [], []
            for g in range(3):
                pr, den = sc[g]
                inv = pl.reciprocal(den, approx=True)
                inv = inv * (2.0 - den * inv)
                o = jnp.dot(pr, get(vt, vret, p, e, g), preferred_element_type=F32) * inv
                m0 = nx[g] if q_x else 0
                for i in range(len(TILES[g])):
                    if q_x:
                        xs.append(o[SEG * i:SEG * (i + 1)])
                    ms.append(o[m0 + MEM * i:m0 + MEM * (i + 1)])
            return [jnp.concatenate(xs[4 * k:4 * k + 4] + ms[4 * k:4 * k + 4], axis=0)
                    for k in range(2)]

        def pair(p, nxt=True):
            sc = [scores(p, e) for e in range(2)]
            if nxt:
                proj_qk(p + 1)
            put_o(p, q0, [values(p, e, sc[e]) for e in range(2)])
            if nxt:
                proj_v(p + 1)

        return proj_qk, proj_v, pair

    kt[:, 2, 80:128, :] = jnp.zeros((2, 48, DH), BF16)
    vt[:, 2, 80:128, :] = jnp.zeros((2, 48, DH), BF16)

    proj_qk, proj_v, pair = step("pred")
    cp_w(0, 0).wait()
    proj_qk(0)
    proj_v(0)

    def pred_loop(p, carry):
        cp_w(0, p + 1).wait()
        pair(p)
        return carry

    for t in range(T - 2):
        cp_ax(t).start()
    lax.fori_loop(0, NP - 1, pred_loop, 0)
    pair(NP - 1, False)
    lax.fori_loop(0, 2, lambda c, carry: (out_mem(c, XH, True, False), carry)[1], 0)
    for t in range(T - 2):
        cp_ax(t).wait()
    for c in range(8):
        cp_by(c).start()

    proj_qk, proj_v, pair = step("mid")
    pair_last = step("last")[2]

    def pairs(fn):
        def pair_loop(i, carry):
            fn(2 * i + 1)
            fn(2 * i + 2)
            return carry

        lax.fori_loop(0, NP // 2 - 1, pair_loop, 0)

    def segment(t, carry):
        load_x(t)
        proj_qk(0)
        proj_v(0)
        pair(0)

        @pl.when(t < T - 1)
        def _():
            pairs(pair)

        @pl.when(t == T - 1)
        def _():
            pairs(pair_last)
            for e in range(2):
                for g in range(3):
                    kt[e, g, 0:nx[g], :] = kret[NP - 1, e, 96 * g:96 * g + nx[g], :]
                    vt[e, g, 0:nx[g], :] = vret[NP - 1, e, 96 * g:96 * g + nx[g], :]

        pair(NP - 1, False)
        for c in range(2):
            top, bot = out_mem(c, 0, True, True)
            cols = slice(512 * c, 512 * (c + 1))
            ostage[t, 0:G // 2, :, :, cols] = top.astype(BF16).reshape(G // 2, 2, 16, 512)
            ostage[t, G // 2:G, :, :, cols] = bot.astype(BF16).reshape(G // 2, 2, 16, 512)
        cp_ao(t).start()
        return carry

    def one_pass(carry):
        it, _ = carry
        start = mend[0:(G - 1) * MEM, :]
        mstart[...] = start
        set_mem(jnp.concatenate([mem0_ref[...].astype(F32), start], axis=0))
        lax.fori_loop(0, T, segment, 0)
        real = mend[0:(G - 1) * MEM, :]
        lim = jnp.max(jnp.abs(real), axis=1, keepdims=True) * TOL
        good = jnp.abs(real - mstart[...]) <= lim
        bad = jnp.max(jnp.where(good, 0.0, 1.0))
        for t in range(T):
            cp_ao(t).wait()
        return it + 1, bad

    lax.while_loop(lambda c: jnp.logical_and(c[0] < G, c[1] > 0.0), one_pass,
                   (jnp.int32(0), jnp.float32(1.0)))
    for c in range(8):
        cp_by(c).wait()


@functools.partial(jax.jit, static_argnames=("A_seg_len",))
def pallas_concat_heads__memory_aug_recurrent_mem_tr__spectral_gfnet__prompt_kernel(
    A_x, A_mem0, A_Wq, A_Wk, A_Wv, A_Wo, A_seg_len, B_x, B_w_r, B_w_i,
):
    assert A_seg_len == SEG and A_x.shape == (1, G * T * SEG, DM) and A_Wq.shape == (DM, NH, DH)
    assert A_mem0.shape == (1, MEM, DM) and B_x.shape == (1, 2048, 1024)
    dmat, smat, mask = _constants()
    wr_t, wi_t = B_w_r.T, B_w_i.T
    hbm = pl.BlockSpec(memory_space=pl.ANY)
    nyq = pl.BlockSpec((16, 2048), lambda i: (32, 0))

    def full(shape):
        return pl.BlockSpec(shape, lambda i: (0,) * len(shape))

    out = pl.pallas_call(
        _kernel,
        grid=(1,),
        in_specs=[hbm] * 9 + [full((MEM, DM)), nyq, nyq, full(dmat.shape), full(mask.shape)],
        out_specs=hbm,
        out_shape=jax.ShapeDtypeStruct((G, 16, 16, 2 * DM), BF16),
        scratch_shapes=[
            pltpu.VMEM((T, G, SEG // 2, DM), U32),
            *[pltpu.VMEM((NP, 4, 7 * 64, DH), U32)] * 3,
            pltpu.VMEM((NP, DH // 2, 7 * 512), U32),
            pltpu.VMEM((8, 8, 16, 1024), U32),
            pltpu.VMEM((16, 256, 128), U32),
            pltpu.VMEM((16, 256, 128), U32),
            pltpu.VMEM((16, 256, 256), BF16),
            pltpu.VMEM((16, KROWS, 256), F32),
            pltpu.VMEM((16, 640, 256), BF16),
            pltpu.VMEM((NP, 2, G * SEG, DH), BF16),
            pltpu.VMEM((NP, 2, G * SEG, DH), BF16),
            pltpu.VMEM((7, HH // 2, DM // 2), U32),
            pltpu.VMEM((2, 3, 128, DH), BF16),
            pltpu.VMEM((2, 3, 128, DH), BF16),
            pltpu.VMEM((2, 3, 128, DH), BF16),
            pltpu.VMEM((7, NP, HH, DH), BF16),
            pltpu.VMEM(((G - 1) * MEM, DM), F32),
            pltpu.VMEM((G * MEM, DM), F32),
            pltpu.VMEM((T, G, 2, 16, DM), BF16),
            pltpu.SemaphoreType.DMA((3, 8)),
            pltpu.SemaphoreType.DMA((3, NP)),
            pltpu.SemaphoreType.DMA((6,)),
            pltpu.SemaphoreType.DMA((2, T)),
        ],
        compiler_params=pltpu.CompilerParams(
            dimension_semantics=("arbitrary",), vmem_limit_bytes=120 * 1024 * 1024),
    )(
        A_x.reshape(G, T, SEG, DM),
        A_Wq.reshape(4, 256, NH, DH), A_Wk.reshape(4, 256, NH, DH), A_Wv.reshape(4, 256, NH, DH),
        A_Wo.reshape(NP, 2, DH, DM), B_x.reshape(8, 16, 16, 1024), wr_t, wi_t, smat,
        A_mem0.reshape(MEM, DM), wr_t, wi_t, dmat, mask,
    )
    return out.reshape(1, 2048, 2 * DM)
```

```python
import functools

import jax
import jax.numpy as jnp
import numpy as np
from jax import lax
from jax.experimental import pallas as pl
from jax.experimental.pallas import tpu as pltpu

F32 = jnp.float32
BF16 = jnp.bfloat16
U32 = jnp.uint32

G = 8
T = 8
SEG = 32
MEM = 8
DM = 1024
NH = 32
DH = 128
KS = (-4.0 / 3, -1.0 / 3, 1.0 / 3, 4.0 / 3)
NB = len(KS)
PAIRS = [(i, j) for i in range(NB) for j in range(i + 1, NB)]
NL = 2 * NB + 3 * len(PAIRS)
NX = NB + len(PAIRS)
NG = NH // NB
NI = DM // 128 // NB
XH = G // 2 * SEG
MH = G // 2 * MEM
HH = XH + MH
LOG2E = 1.4426950408889634
QSCALE = float(DH ** -0.5 * LOG2E)
MASKED = float(-1e9 * LOG2E)
TOL = 2.0 ** -9
NT = (((1,), (1,)), ((), ()))
KROWS = 528
ROW_OFF = {0: 0, 4: 64, 1: 128, 7: 192, 2: 256, 6: 320, 3: 384, 5: 448}


def _constants():
    beta = np.arange(128)[None, :]
    m = np.arange(64)[:, None]
    d = np.zeros((4, 256, 256))
    for blk, r in enumerate((0, 4)):
        th = 2 * np.pi * (8 * m + r) * beta / 1024
        d[0, 64 * blk:64 * blk + 64, 128 * blk:128 * blk + 128] = np.cos(th)
        d[0, 128 + 64 * blk:192 + 64 * blk, 128 * blk:128 * blk + 128] = -np.sin(th)
    d[0, 128, 0:128] = np.cos(np.pi * np.arange(128))
    for r, sg in ((1, -1.0), (2, -1.0), (3, 1.0)):
        for blk, (res, cj) in enumerate(((r, 1.0), (8 - r, -1.0))):
            th = 2 * np.pi * (8 * m + res) * beta / 1024
            re, im = slice(64 * blk, 64 * blk + 64), slice(128 + 64 * blk, 192 + 64 * blk)
            d[r, re, 0:128] = np.cos(th)
            d[r, im, 0:128] = -np.sin(th)
            d[r, re, 128:256] = sg * cj * np.sin(th)
            d[r, im, 128:256] = sg * cj * np.cos(th)
    d *= 2.0 ** -10
    b = np.arange(128)[:, None]
    kb = np.arange(128)[None, :]
    s = np.zeros((16, 256, 256))
    for a in range(16):
        th = 2 * np.pi * ((kb * (16 * b + a)) % 2048) / 2048
        s[a, :128, :128] = np.cos(th)
        s[a, 128:, :128] = np.sin(th)
        s[a, :128, 128:] = -np.sin(th)
        s[a, 128:, 128:] = np.cos(th)
    mask = np.zeros((2, 128, 128), np.float32)
    for i, ns in enumerate((3, 2)):
        idx = np.arange(128)
        isx = idx < SEG * ns
        pad = idx >= (SEG + MEM) * ns
        seg = np.where(isx, idx // SEG, (idx - SEG * ns) // MEM)
        same = (seg[:, None] == seg[None, :]) & ~pad[None, :]
        future = isx[:, None] & isx[None, :] & (idx[None, :] > idx[:, None])
        mk = np.where(same, np.where(future, MASKED, 0.0), -np.inf)
        mask[i] = np.where(pad[:, None], 0.0, mk)
    return d.astype(BF16), s.astype(BF16), mask


def _lo(w):
    return lax.bitcast_convert_type(w << 16, F32)


def _hi(w):
    return lax.bitcast_convert_type(w & np.uint32(0xFFFF0000), F32)


def _bf16_bits(y):
    return lax.bitcast_convert_type(y.astype(BF16).astype(F32), U32)


def _r4(x, sg):
    (ar, ai), (br, bi), (cr, ci), (dr, di) = x
    s0r, s0i, d0r, d0i = ar + cr, ai + ci, ar - cr, ai - ci
    s1r, s1i, d1r, d1i = br + dr, bi + di, br - dr, bi - di
    p = (d0r - d1i, d0i + d1r)
    q = (d0r + d1i, d0i - d1r)
    y1, y3 = (p, q) if sg > 0 else (q, p)
    return [(s0r + s1r, s0i + s1i), y1, (s0r - s1r, s0i - s1i), y3]


def _tw(z, e, sg):
    r, i = z
    if e == 0:
        return z
    if e == 4:
        return (-i, r) if sg > 0 else (i, -r)
    h = float(np.sqrt(0.5))
    if e == 2:
        return ((r - i) * h, (r + i) * h) if sg > 0 else ((r + i) * h, (i - r) * h)
    if e == 6:
        return ((r + i) * -h, (r - i) * h) if sg > 0 else ((i - r) * h, (r + i) * -h)
    c = float(np.cos(2 * np.pi * e / 16))
    s = float(sg * np.sin(2 * np.pi * e / 16))
    return (r * c - i * s, r * s + i * c)


def _fft16(x, sg):
    t = [_r4([x[4 * a1 + a0] for a1 in range(4)], sg) for a0 in range(4)]
    out = [None] * 16
    for k0 in range(4):
        u = _r4([_tw(t[a0][k0], a0 * k0, sg) for a0 in range(4)], sg)
        for k1 in range(4):
            out[k0 + 4 * k1] = u[k1]
    return out


def _words(even, odd):
    return pltpu.pack_elementwise([even, odd], packed_dtype=BF16)


def _left(x, y):
    z = [x[i] + KS[i] * y[i] for i in range(NB)]
    out = z + list(y)
    for i, j in PAIRS:
        sx, sy = x[i] + x[j], y[i] + y[j]
        out += [z[i] + z[j], sx + KS[j] * sy, sx + KS[i] * sy]
    return out


def _right(b):
    rows = [functools.reduce(lambda u, v: u + v, b[i]) for i in range(NB)]
    extra = [functools.reduce(lambda u, v: u - v, [b[j][i] for j in range(NB) if j != i], b[i][i])
             for i in range(NB)]
    extra += [(b[i][j] + b[j][i]) * (1.0 / (KS[j] - KS[i])) for i, j in PAIRS]
    return rows, extra


def _combine(mm):
    s = [mm(i, i) for i in range(NB)]
    r = [mm(NB + i, (i, i)) for i in range(NB)]
    for n, (i, j) in enumerate(PAIRS):
        p1 = mm(2 * NB + 3 * n, NB + n)
        p2 = mm(2 * NB + 3 * n + 1, (i, j))
        p3 = mm(2 * NB + 3 * n + 2, (j, i))
        d = 1.0 / (KS[j] - KS[i])
        e = (p2 + p3 if d == 1.0 else (p2 + p3) * d) - p1
        r[j], r[i], s[j], s[i] = r[j] + e, r[i] - e, s[j] + p2, s[i] + p3
    return [s[i] - KS[i] * r[i] for i in range(NB)], r


def _kernel(ax_hbm, wq_hbm, wk_hbm, wv_hbm, wo_hbm, bx_hbm, wr_hbm, wi_hbm, s_hbm,
            mem0_ref, wrn_ref, win_ref, d_ref, mask_ref,
            out_hbm,
            ax, wq, wk, wv, wqx, wkx, wvx, wo, wox, xw, wr, wi, sm, yb, vb, kret, vret, hs,
            qt, kt, vt, ob, mstart, mend, ostage, sem_b, sem_w, sem_m, sem_o):
    wblk, wext = (wq, wk, wv), (wqx, wkx, wvx)

    def cp_bx(c):
        return pltpu.make_async_copy(bx_hbm.bitcast(U32).at[:, :, c, :], xw.at[c], sem_b.at[0, c])

    def cp_s(c):
        sl = pl.ds(2 * c, 2)
        return pltpu.make_async_copy(s_hbm.at[sl], sm.at[sl], sem_b.at[1, c])

    def cp_by(c):
        return pltpu.make_async_copy(
            xw.at[c], out_hbm.bitcast(U32).at[:, :, c, pl.ds(DM, DM)], sem_b.at[2, c])

    def cp_w(j, g, a):
        src = (wq_hbm, wk_hbm, wv_hbm)[j].bitcast(U32).at[:, :, :, NB // 2 * g + a, :]
        return pltpu.make_async_copy(src, wblk[j].at[g, :, :, pl.ds(128 * a, 128), :],
                                     sem_w.at[j, a, g])

    def cp_wo(g):
        return pltpu.make_async_copy(wo_hbm.bitcast(U32).at[g], wo.at[g], sem_w.at[3, 0, g])

    def cp_ax(t):
        return pltpu.make_async_copy(ax_hbm.bitcast(U32).at[:, t], ax.at[t], sem_o.at[1, t])

    def cp_ao(t):
        return pltpu.make_async_copy(
            ostage.at[t], out_hbm.at[:, pl.ds(2 * t, 2), :, pl.ds(0, DM)], sem_o.at[0, t])

    def cp_f(j, k):
        src, dst = ((wr_hbm, wr), (wi_hbm, wi))[j]
        return pltpu.make_async_copy(
            src.at[pl.ds(0, 512), pl.ds(pl.multiple_of(128 * k, 128), 128)].bitcast(U32),
            dst.at[k], sem_m.at[j])

    for c in range(2):
        cp_bx(c).start()
        cp_s(c).start()

    rt = float(np.sqrt(0.5))
    row8 = lax.broadcasted_iota(jnp.int32, (8, 128), 0)

    def b_forward(c, carry):
        @pl.when(c < 6)
        def _():
            cp_bx(c + 2).start()
            cp_s(c + 2).start()

        for j in range(2):
            cp_f(j, 2 * c).start()
            cp_f(j, 2 * c + 1).start()

        @pl.when(c == 7)
        def _():
            cp_ax(T - 1).start()
            cp_ax(T - 2).start()

        cp_bx(c).wait()
        cp_s(c).wait()
        w = xw[c].reshape(128, DM)
        for half, xf in enumerate((_lo(w), _hi(w))):
            x = [xf[:, 128 * al:128 * (al + 1)] for al in range(8)]
            s = [x[i] + x[i + 4] for i in range(4)]
            d = [x[i] - x[i + 4] for i in range(4)]
            e, o = s[0] + s[2], s[1] + s[3]
            p, q = (d[1] - d[3]) * rt, (d[1] + d[3]) * rt
            u = [(e + o, e - o), (d[0] + p, d[2] + q), (s[0] - s[2], s[1] - s[3]),
                 (d[0] - p, d[2] - q)]
            tt = [lax.dot_general(d_ref[k], jnp.concatenate(u[k], axis=1).astype(BF16), NT,
                                  preferred_element_type=F32) for k in range(4)]
            dc, ny = tt[0][0:8], tt[0][128:136]
            re = [jnp.where(row8 == 0, dc * 0.5, dc), tt[0][8:128]]
            im = [jnp.where(row8 == 0, 0.0, ny), tt[0][136:256]]
            for k in range(1, 4):
                re.append(tt[k][0:128])
                im.append(tt[k][128:256])
            re += [jnp.where(row8 == 0, ny * 0.5, 0.0), jnp.zeros((8, 128), F32)]
            im.append(jnp.zeros((16, 128), F32))
            lhs = jnp.concatenate([jnp.concatenate(re, axis=0), jnp.concatenate(im, axis=0)],
                                  axis=1).astype(BF16)
            a = 2 * c + half
            yb[a] = jnp.dot(lhs, sm[a], preferred_element_type=F32)
        return carry

    lax.fori_loop(0, 8, b_forward, 0)
    pltpu.make_async_copy(wr, wr, sem_m.at[0]).wait()
    pltpu.make_async_copy(wi, wi, sem_m.at[1]).wait()

    def filt(row, wre, wim):
        y = [(yb[a, pl.ds(row, 8), 0:128], yb[a, pl.ds(row, 8), 128:256]) for a in range(16)]
        z = _fft16(y, -1)
        z = [(z[k][0] * wre(k) - z[k][1] * wim(k), z[k][0] * wim(k) + z[k][1] * wre(k))
             for k in range(16)]
        return _fft16(z, 1)

    def b_filter(i, carry):
        mg, j = i // 4, i % 4

        @pl.when(i < NG)
        def _():
            cp_wo(i).start()

        for half, un in enumerate((_lo, _hi)):
            off = [ROW_OFF[2 * jj + half] for jj in range(4)]
            base = jnp.where(j < 2, jnp.where(j == 0, off[0], off[1]),
                             jnp.where(j == 2, off[2], off[3])) + 16 * mg
            base = pl.multiple_of(base, 16)
            res = []
            for r8 in range(2):
                sl = pl.ds(64 * mg + 32 * r8 + j, 8, stride=4)
                res.append(filt(pl.multiple_of(base + 8 * r8, 8),
                                lambda k: un(wr[k, sl, :]),
                                lambda k: un(wi[k, sl, :])))
            for a in range(16):
                for ri in range(2):
                    vb[a, pl.ds(base, 16), 128 * ri:128 * (ri + 1)] = jnp.concatenate(
                        [res[0][a][ri], res[1][a][ri]], axis=0).astype(BF16)
        return carry

    lax.fori_loop(0, 16, b_filter, 0)
    res = filt(512, lambda k: wrn_ref[0:1, 128 * k:128 * (k + 1)].astype(F32),
               lambda k: win_ref[0:1, 128 * k:128 * (k + 1)].astype(F32))
    for a in range(16):
        for ri in range(2):
            vb[a, 512:KROWS, 128 * ri:128 * (ri + 1)] = jnp.concatenate(
                [res[a][ri], jnp.zeros((8, 128), F32)], axis=0).astype(BF16)
        vb[a, KROWS:640, :] = jnp.zeros((640 - KROWS, 256), BF16)

    lane0 = lax.broadcasted_iota(jnp.int32, (128, 128), 1) == 0

    def prep_wo(g):
        for c in range(NI):
            for r in range(0, 64, 8):
                w = [[wo[g, i, r:r + 8, 128 * (NB * c + j):128 * (NB * c + j + 1)]
                      for j in range(NB)] for i in range(NB)]
                ev, od = [_right([[un(v) for v in row] for row in w]) for un in (_lo, _hi)]
                for i in range(NB):
                    wo[g, i, r:r + 8, 128 * (NB * c + i):128 * (NB * c + i + 1)] = _words(
                        ev[0][i], od[0][i])
                for n in range(NX):
                    wox[g, 64 * n + r:64 * n + r + 8, 128 * c:128 * (c + 1)] = _words(
                        ev[1][n], od[1][n])

    def b_inverse(c, carry):
        for g in range(NG // 8):
            for a in range(NB // 2):
                cp_w(1, NG // 8 * c + g, a).start()
                cp_w(2, NG // 8 * c + g, a).start()
        for g in range(NG // 8):
            cp_wo(NG // 8 * c + g).wait()
        for g in range(NG // 8):
            prep_wo(NG // 8 * c + g)
        lhs = [[] for _ in range(4)]
        for half in range(2):
            a = 2 * c + half
            z = lax.dot_general(sm[a], vb[a, 0:512, :], NT, preferred_element_type=F32)
            ny = lax.dot_general(sm[a, 0:128, :], vb[a, 512:640, :], NT,
                                 preferred_element_type=F32)
            for k in range(4):
                zr, zi = z[0:128, 128 * k:128 * (k + 1)], z[128:256, 128 * k:128 * (k + 1)]
                if k == 0:
                    zi = jnp.where(lane0, ny, zi)
                lhs[k].append(jnp.concatenate([zr, zi], axis=1).astype(BF16))
        g = [jnp.dot(jnp.concatenate(lhs[k], axis=0), d_ref[k], preferred_element_type=F32)
             for k in range(4)]
        (g0, g4), (g1r, g1i), (g2r, g2i), (g3r, g3i) = [(v[:, :128], v[:, 128:]) for v in g]
        e, o = g0 + g4, g0 - g4
        s = [e + g2r, o + g2i, e - g2r, o - g2i]
        p, q = (g1r - g3r) * rt, (g1i - g3i) * rt
        d = [g1r + g3r, q + p, g1i + g3i, q - p]
        y = [s[i] + d[i] for i in range(4)] + [s[i] - d[i] for i in range(4)]
        for al in range(8):
            bits = _bf16_bits(y[al])
            xw[c, :, :, 128 * al:128 * (al + 1)] = (
                (bits[0:128] >> 16) | bits[128:256]).reshape(8, 16, 128)
        return carry

    lax.fori_loop(0, 8, b_inverse, 0)

    def blocks(v):
        n = v.shape[1] // (128 * NB)
        return [jnp.concatenate([v[:, 128 * (NB * c + i):128 * (NB * c + i + 1)]
                                 for c in range(n)], axis=1) for i in range(NB)]

    def load_x(t):
        for g in range(G // 2):
            top, bot = ax[t, g], ax[t, g + G // 2]
            ev, od = [_left(blocks(un(top)), blocks(un(bot))) for un in (_lo, _hi)]
            for n in range(NL):
                hs[n, SEG // 2 * g:SEG // 2 * (g + 1), :] = _words(ev[n], od[n])

    def set_mem(m):
        for n, v in enumerate(_left(blocks(m[0:MH]), blocks(m[MH:2 * MH]))):
            hs[n, XH // 2:HH // 2, :] = pltpu.bitcast(v.astype(BF16), U32)

    def prep_w(j, g):
        for a in range(NB // 2):
            cp_w(j, g, a).wait()
        ref = wblk[j]

        def raw(c, i, r, n):
            w = [[ref[g, c, i, pl.ds(128 * a + 2 * r + d, n, stride=2), :]
                  for a in range(NB // 2)] for d in range(2)]
            return [[un(v) for v in w[d] for un in (_lo, _hi)] for d in range(2)]

        for c in range(NI):
            for r in range(0, 64, 8):
                b = [raw(c, i, r, 8) for i in range(NB)]
                ev, od = [_right([b[i][d] for i in range(NB)])[1] for d in range(2)]
                for n in range(NX):
                    wext[j][g, c, 64 * n + r:64 * n + r + 8, :] = _words(ev[n], od[n])
        for c in range(NI):
            for i in range(NB):
                ev, od = raw(c, i, 0, 64)
                for v in (ev, od):
                    v[i] = functools.reduce(lambda p, q: p + q, v)
                for e in range(NB):
                    ref[g, c, i, 64 * e:64 * (e + 1), :] = _words(ev[e], od[e])

    def right(blk, ext, b):
        w = ext(64 * b) if isinstance(b, int) else blk(*b)
        w = pltpu.bitcast(w, BF16)
        return w.reshape(w.shape[0] * 128, 128)

    def project(g, r0, r1, lo, hi):
        def mm(a, b):
            w = [right(lambda i, e: wblk[j][g, :, i, 64 * e:64 * (e + 1), :],
                       lambda o: wext[j][g, :, o:o + 64, :], b) for j in range(lo, hi)]
            return jnp.dot(pltpu.bitcast(hs[a, r0 // 2:r1 // 2, :], BF16),
                           jnp.concatenate(w, axis=1), preferred_element_type=F32)

        return _combine(mm)

    def put_o(g, r0, o):
        for n, v in enumerate(_left([h[0] for h in o], [h[1] for h in o])):
            ob[n, g, r0:HH, :] = v.astype(BF16)

    def out_mem(c, r0, keep, feed):
        def lanes(k, n=1):
            return pl.ds(pl.multiple_of(128 * k, 128), 128 * n)

        def mm(a, b):
            o = jnp.concatenate([ob[a, g, r0:HH, :] for g in range(NG)], axis=1)
            w = right(lambda i, e: wo[:, i, :, lanes(NB * c + e)],
                      lambda o: wox[:, o:o + 64, lanes(c)], b)
            return jnp.dot(o, w, preferred_element_type=F32)

        top, bot = _combine(mm)
        x0 = XH - r0
        if keep:
            mend[0:MH, lanes(NB * c, NB)] = jnp.concatenate([v[x0:] for v in top], axis=1)
            mend[MH:2 * MH, lanes(NB * c, NB)] = jnp.concatenate([v[x0:] for v in bot], axis=1)
        if feed:
            for n, v in enumerate(_left([v[x0:] for v in top], [v[x0:] for v in bot])):
                hs[n, XH // 2:HH // 2, lanes(c)] = pltpu.bitcast(v.astype(BF16), U32)
        return [[v[:x0] for v in half] for half in (top, bot)]

    cp_ax(T - 1).wait()
    load_x(T - 1)

    def kv_loop(g, carry):
        for a in range(NB // 2):
            cp_w(0, g, a).start()
        prep_w(1, g)
        prep_w(2, g)
        top, bot = project(g, 0, XH, 1, 3)
        for e in range(NB):
            v = jnp.concatenate([top[e], bot[e]], axis=0).astype(BF16)
            kret[NB * g + e] = v[:, 0:DH]
            vret[NB * g + e] = v[:, DH:2 * DH]
        return carry

    lax.fori_loop(0, NG, kv_loop, 0)

    cp_ax(T - 2).wait()
    xbar = jnp.sum(_lo(ax[T - 2]) + _hi(ax[T - 2]), axis=1, keepdims=True) * (1.0 / (SEG + MEM))
    set_mem(jnp.broadcast_to(xbar, (G, MEM, DM)).reshape(G * MEM, DM))

    def guess(g, carry):
        put_o(g, XH, list(zip(*project(g, XH, HH, 2, 3))))
        return carry

    lax.fori_loop(0, NG, guess, 0)
    lax.fori_loop(0, NI, lambda c, carry: (out_mem(c, XH, False, True), carry)[1], 0)

    TILES = ((0, 1, 2), (3, 4, 5), (6, 7))
    nx = [SEG * len(tl) for tl in TILES]
    nm = (32, 32, 16)

    def tile(v, g, with_x):
        m0 = XH if with_x else 0
        parts = [v[ch // 4][SEG * (ch % 4):SEG * (ch % 4 + 1)] for ch in TILES[g]] if with_x else []
        parts += [v[ch // 4][m0 + MEM * (ch % 4):m0 + MEM * (ch % 4 + 1)] for ch in TILES[g]]
        if len(TILES[g]) == 3:
            parts.append(jnp.zeros((MEM, DH), F32))
        return jnp.concatenate(parts, axis=0).astype(BF16)

    def step(mode):
        q_x, kv_x = mode != "pred", mode == "mid"
        q0, kv0 = (0 if q_x else XH), (0 if kv_x else XH)

        def put(ref, e, v, with_x):
            for g in range(3):
                ref[e, g, (0 if with_x else nx[g]):nx[g] + nm[g], :] = tile(v, g, with_x)

        def proj_qk(hg):
            if q_x == kv_x:
                r = project(hg, q0, HH, 0, 2)
                q = [[v[:, 0:DH] for v in half] for half in r]
                k = [[v[:, DH:2 * DH] for v in half] for half in r]
            else:
                q, k = project(hg, q0, HH, 0, 1), project(hg, kv0, HH, 1, 2)
            for e in range(NB):
                put(qt, e, [half[e] * QSCALE for half in q], q_x)
                put(kt, e, [half[e] for half in k], kv_x)

        def proj_v(hg):
            v = project(hg, kv0, HH, 2, 3)
            for e in range(NB):
                put(vt, e, [half[e] for half in v], kv_x)

        def get(ref, ret, hg, e, g):
            if kv_x:
                return ref[e, g]
            return jnp.concatenate(
                [ret[NB * hg + e, 96 * g:96 * g + nx[g], :], ref[e, g, nx[g]:128, :]], axis=0)

        def scores(hg, e):
            out = []
            for g in range(3):
                r0 = 0 if q_x else nx[g]
                s = lax.dot_general(qt[e, g, r0:nx[g] + nm[g], :], get(kt, kret, hg, e, g), NT,
                                    preferred_element_type=F32)
                fill = mask_ref[g // 2, r0:nx[g] + nm[g], :]
                s = jnp.where(fill == 0.0, s, fill)
                pr = jnp.exp2(s - jnp.max(s, axis=1, keepdims=True))
                out.append((pr.astype(BF16), jnp.sum(pr, axis=1, keepdims=True)))
            return out

        def values(hg, e, sc):
            xs, ms = [], []
            for g in range(3):
                pr, den = sc[g]
                inv = pl.reciprocal(den, approx=True)
                inv = inv * (2.0 - den * inv)
                o = jnp.dot(pr, get(vt, vret, hg, e, g), preferred_element_type=F32) * inv
                m0 = nx[g] if q_x else 0
                for i in range(len(TILES[g])):
                    if q_x:
                        xs.append(o[SEG * i:SEG * (i + 1)])
                    ms.append(o[m0 + MEM * i:m0 + MEM * (i + 1)])
            return [jnp.concatenate(xs[4 * k:4 * k + 4] + ms[4 * k:4 * k + 4], axis=0)
                    for k in range(2)]

        def group(hg, nxt=True):
            sc = [scores(hg, e) for e in range(NB)]
            if nxt:
                proj_qk(hg + 1)
            put_o(hg, q0, [values(hg, e, sc[e]) for e in range(NB)])
            if nxt:
                proj_v(hg + 1)

        return proj_qk, proj_v, group

    kt[:, 2, 80:128, :] = jnp.zeros((NB, 48, DH), BF16)
    vt[:, 2, 80:128, :] = jnp.zeros((NB, 48, DH), BF16)

    proj_qk, proj_v, group = step("pred")
    for t in range(T - 2):
        cp_ax(t).start()
    prep_w(0, 0)
    proj_qk(0)
    proj_v(0)

    def pred_loop(hg, carry):
        prep_w(0, hg + 1)
        group(hg)
        return carry

    lax.fori_loop(0, NG - 1, pred_loop, 0)
    group(NG - 1, False)
    lax.fori_loop(0, NI, lambda c, carry: (out_mem(c, XH, True, False), carry)[1], 0)
    for t in range(T - 2):
        cp_ax(t).wait()
    for c in range(8):
        cp_by(c).start()
    load_x(0)

    proj_qk, proj_v, group = step("mid")
    group_last = step("last")[2]

    def segment(t, carry):
        proj_qk(0)
        proj_v(0)

        @pl.when(t < T - 1)
        def _():
            lax.fori_loop(0, NG - 1, lambda hg, c: (group(hg), c)[1], 0)

        @pl.when(t == T - 1)
        def _():
            lax.fori_loop(0, NG - 1, lambda hg, c: (group_last(hg), c)[1], 0)
            for e in range(NB):
                for g in range(3):
                    kt[e, g, 0:nx[g], :] = kret[NH - NB + e, 96 * g:96 * g + nx[g], :]
                    vt[e, g, 0:nx[g], :] = vret[NH - NB + e, 96 * g:96 * g + nx[g], :]

        load_x((t + 1) % T)
        group(NG - 1, False)
        for c in range(NI):
            for k, half in enumerate(out_mem(c, 0, True, True)):
                for e, v in enumerate(half):
                    ostage[t, 4 * k:4 * k + 4, :, :, 128 * (NB * c + e):128 * (NB * c + e + 1)] = (
                        v.astype(BF16).reshape(G // 2, 2, 16, 128))
        cp_ao(t).start()
        return carry

    def one_pass(carry):
        it, _ = carry
        start = mend[0:(G - 1) * MEM, :]
        mstart[...] = start
        set_mem(jnp.concatenate([mem0_ref[...].astype(F32), start], axis=0))
        lax.fori_loop(0, T, segment, 0)
        real = mend[0:(G - 1) * MEM, :]
        lim = jnp.max(jnp.abs(real), axis=1, keepdims=True) * TOL
        good = jnp.abs(real - mstart[...]) <= lim
        bad = jnp.max(jnp.where(good, 0.0, 1.0))
        for t in range(T):
            cp_ao(t).wait()
        return it + 1, bad

    lax.while_loop(lambda c: jnp.logical_and(c[0] < G, c[1] > 0.0), one_pass,
                   (jnp.int32(0), jnp.float32(1.0)))
    for c in range(8):
        cp_by(c).wait()


@functools.partial(jax.jit, static_argnames=("A_seg_len",))
def pallas_concat_heads__memory_aug_recurrent_mem_tr__spectral_gfnet__prompt_kernel(
    A_x, A_mem0, A_Wq, A_Wk, A_Wv, A_Wo, A_seg_len, B_x, B_w_r, B_w_i,
):
    assert A_seg_len == SEG and A_x.shape == (1, G * T * SEG, DM) and A_Wq.shape == (DM, NH, DH)
    assert A_mem0.shape == (1, MEM, DM) and B_x.shape == (1, 2048, 1024)
    dmat, smat, mask = _constants()
    wr_t, wi_t = B_w_r.T, B_w_i.T
    hbm = pl.BlockSpec(memory_space=pl.ANY)
    nyq = pl.BlockSpec((16, 2048), lambda i: (32, 0))

    def full(shape):
        return pl.BlockSpec(shape, lambda i: (0,) * len(shape))

    out = pl.pallas_call(
        _kernel,
        grid=(1,),
        in_specs=[hbm] * 9 + [full((MEM, DM)), nyq, nyq, full(dmat.shape), full(mask.shape)],
        out_specs=hbm,
        out_shape=jax.ShapeDtypeStruct((G, 16, 16, 2 * DM), BF16),
        scratch_shapes=[
            pltpu.VMEM((T, G, SEG // 2, DM), U32),
            *[pltpu.VMEM((NG, NI, NB, NB * 64, DH), U32)] * 3,
            *[pltpu.VMEM((NG, NI, NX * 64, DH), U32)] * 3,
            pltpu.VMEM((NG, NB, 64, DM), U32),
            pltpu.VMEM((NG, NX * 64, NI * 128), U32),
            pltpu.VMEM((8, 8, 16, 1024), U32),
            pltpu.VMEM((16, 256, 128), U32),
            pltpu.VMEM((16, 256, 128), U32),
            pltpu.VMEM((16, 256, 256), BF16),
            pltpu.VMEM((16, KROWS, 256), F32),
            pltpu.VMEM((16, 640, 256), BF16),
            pltpu.VMEM((NH, G * SEG, DH), BF16),
            pltpu.VMEM((NH, G * SEG, DH), BF16),
            pltpu.VMEM((NL, HH // 2, NI * 128), U32),
            pltpu.VMEM((NB, 3, 128, DH), BF16),
            pltpu.VMEM((NB, 3, 128, DH), BF16),
            pltpu.VMEM((NB, 3, 128, DH), BF16),
            pltpu.VMEM((NL, NG, HH, DH), BF16),
            pltpu.VMEM(((G - 1) * MEM, DM), F32),
            pltpu.VMEM((G * MEM, DM), F32),
            pltpu.VMEM((T, G, 2, 16, DM), BF16),
            pltpu.SemaphoreType.DMA((3, 8)),
            pltpu.SemaphoreType.DMA((4, NB // 2, NG)),
            pltpu.SemaphoreType.DMA((2,)),
            pltpu.SemaphoreType.DMA((2, T)),
        ],
        compiler_params=pltpu.CompilerParams(
            dimension_semantics=("arbitrary",), vmem_limit_bytes=120 * 1024 * 1024),
    )(
        A_x.reshape(G, T, SEG, DM),
        *[w.reshape(NI, NB, 128, NH, DH) for w in (A_Wq, A_Wk, A_Wv)],
        A_Wo.reshape(NG, NB, DH, DM), B_x.reshape(8, 16, 16, 1024), wr_t, wi_t, smat,
        A_mem0.reshape(MEM, DM), wr_t, wi_t, dmat, mask,
    )
    return out.reshape(1, 2048, 2 * DM)
```

```python
import functools

import jax
import jax.numpy as jnp
import numpy as np
from jax import lax
from jax.experimental import pallas as pl
from jax.experimental.pallas import tpu as pltpu

F32 = jnp.float32
BF16 = jnp.bfloat16
U32 = jnp.uint32

G = 8
T = 8
SEG = 32
MEM = 8
DM = 1024
NH = 32
DH = 128
KS = (-4.0 / 3, -1.0 / 3, 1.0 / 3, 4.0 / 3)
NB = len(KS)
PAIRS = [(i, j) for i in range(NB) for j in range(i + 1, NB)]
NL = 2 * NB + 3 * len(PAIRS)
NX = NB + len(PAIRS)
NG = NH // NB
NI = DM // 128 // NB
XH = G // 2 * SEG
MH = G // 2 * MEM
HH = XH + MH
LOG2E = 1.4426950408889634
QSCALE = float(DH ** -0.5 * LOG2E)
MASKED = float(-1e9 * LOG2E)
TOL = 2.0 ** -9
NT = (((1,), (1,)), ((), ()))
KROWS = 528
ROW_OFF = {0: 0, 4: 64, 1: 128, 7: 192, 2: 256, 6: 320, 3: 384, 5: 448}


def _constants():
    beta = np.arange(128)[None, :]
    m = np.arange(64)[:, None]
    d = np.zeros((4, 256, 256))
    for blk, r in enumerate((0, 4)):
        th = 2 * np.pi * (8 * m + r) * beta / 1024
        d[0, 64 * blk:64 * blk + 64, 128 * blk:128 * blk + 128] = np.cos(th)
        d[0, 128 + 64 * blk:192 + 64 * blk, 128 * blk:128 * blk + 128] = -np.sin(th)
    d[0, 128, 0:128] = np.cos(np.pi * np.arange(128))
    for r, sg in ((1, -1.0), (2, -1.0), (3, 1.0)):
        for blk, (res, cj) in enumerate(((r, 1.0), (8 - r, -1.0))):
            th = 2 * np.pi * (8 * m + res) * beta / 1024
            re, im = slice(64 * blk, 64 * blk + 64), slice(128 + 64 * blk, 192 + 64 * blk)
            d[r, re, 0:128] = np.cos(th)
            d[r, im, 0:128] = -np.sin(th)
            d[r, re, 128:256] = sg * cj * np.sin(th)
            d[r, im, 128:256] = sg * cj * np.cos(th)
    d *= 2.0 ** -10
    b = np.arange(128)[:, None]
    kb = np.arange(128)[None, :]
    s = np.zeros((16, 256, 256))
    for a in range(16):
        th = 2 * np.pi * ((kb * (16 * b + a)) % 2048) / 2048
        s[a, :128, :128] = np.cos(th)
        s[a, 128:, :128] = np.sin(th)
        s[a, :128, 128:] = -np.sin(th)
        s[a, 128:, 128:] = np.cos(th)
    mask = np.zeros((2, 128, 128), np.float32)
    for i, ns in enumerate((3, 2)):
        idx = np.arange(128)
        isx = idx < SEG * ns
        pad = idx >= (SEG + MEM) * ns
        seg = np.where(isx, idx // SEG, (idx - SEG * ns) // MEM)
        same = (seg[:, None] == seg[None, :]) & ~pad[None, :]
        future = isx[:, None] & isx[None, :] & (idx[None, :] > idx[:, None])
        mk = np.where(same, np.where(future, MASKED, 0.0), -np.inf)
        mask[i] = np.where(pad[:, None], 0.0, mk)
    return d.astype(BF16), s.astype(BF16), mask


def _lo(w):
    return lax.bitcast_convert_type(w << 16, F32)


def _hi(w):
    return lax.bitcast_convert_type(w & np.uint32(0xFFFF0000), F32)


def _bf16_bits(y):
    return lax.bitcast_convert_type(y.astype(BF16).astype(F32), U32)


def _r4(x, sg):
    (ar, ai), (br, bi), (cr, ci), (dr, di) = x
    s0r, s0i, d0r, d0i = ar + cr, ai + ci, ar - cr, ai - ci
    s1r, s1i, d1r, d1i = br + dr, bi + di, br - dr, bi - di
    p = (d0r - d1i, d0i + d1r)
    q = (d0r + d1i, d0i - d1r)
    y1, y3 = (p, q) if sg > 0 else (q, p)
    return [(s0r + s1r, s0i + s1i), y1, (s0r - s1r, s0i - s1i), y3]


def _tw(z, e, sg):
    r, i = z
    if e == 0:
        return z
    if e == 4:
        return (-i, r) if sg > 0 else (i, -r)
    h = float(np.sqrt(0.5))
    if e == 2:
        return ((r - i) * h, (r + i) * h) if sg > 0 else ((r + i) * h, (i - r) * h)
    if e == 6:
        return ((r + i) * -h, (r - i) * h) if sg > 0 else ((i - r) * h, (r + i) * -h)
    c = float(np.cos(2 * np.pi * e / 16))
    s = float(sg * np.sin(2 * np.pi * e / 16))
    return (r * c - i * s, r * s + i * c)


def _fft16(x, sg):
    t = [_r4([x[4 * a1 + a0] for a1 in range(4)], sg) for a0 in range(4)]
    out = [None] * 16
    for k0 in range(4):
        u = _r4([_tw(t[a0][k0], a0 * k0, sg) for a0 in range(4)], sg)
        for k1 in range(4):
            out[k0 + 4 * k1] = u[k1]
    return out


def _words(even, odd):
    return pltpu.pack_elementwise([even, odd], packed_dtype=BF16)


def _left(x, y):
    z = [x[i] + KS[i] * y[i] for i in range(NB)]
    out = z + list(y)
    for i, j in PAIRS:
        sx, sy = x[i] + x[j], y[i] + y[j]
        out += [z[i] + z[j], sx + KS[j] * sy, sx + KS[i] * sy]
    return out


def _right(b):
    rows = [functools.reduce(lambda u, v: u + v, b[i]) for i in range(NB)]
    extra = [functools.reduce(lambda u, v: u - v, [b[j][i] for j in range(NB) if j != i], b[i][i])
             for i in range(NB)]
    extra += [(b[i][j] + b[j][i]) * (1.0 / (KS[j] - KS[i])) for i, j in PAIRS]
    return rows, extra


def _combine(mm):
    s = [mm(i, i) for i in range(NB)]
    r = [mm(NB + i, (i, i)) for i in range(NB)]
    for n, (i, j) in enumerate(PAIRS):
        p1 = mm(2 * NB + 3 * n, NB + n)
        p2 = mm(2 * NB + 3 * n + 1, (i, j))
        p3 = mm(2 * NB + 3 * n + 2, (j, i))
        d = 1.0 / (KS[j] - KS[i])
        e = (p2 + p3 if d == 1.0 else (p2 + p3) * d) - p1
        r[j], r[i], s[j], s[i] = r[j] + e, r[i] - e, s[j] + p2, s[i] + p3
    return [s[i] - KS[i] * r[i] for i in range(NB)], r


def _kernel(ax_hbm, wq_hbm, wk_hbm, wv_hbm, wo_hbm, bx_hbm, wr_hbm, wi_hbm, s_hbm,
            mem0_ref, wrn_ref, win_ref, d_ref, mask_ref,
            out_hbm,
            ax, wq, wk, wv, wqx, wkx, wvx, wo, wox, xw, wr, wi, sm, yb, vb, kret, vret, hs,
            qt, kt, vt, ob, mstart, mend, ostage, sem_b, sem_w, sem_m, sem_o):
    wblk, wext = (wq, wk, wv), (wqx, wkx, wvx)

    def cp_bx(c):
        return pltpu.make_async_copy(bx_hbm.bitcast(U32).at[:, :, c, :], xw.at[c], sem_b.at[0, c])

    def cp_s(c):
        sl = pl.ds(2 * c, 2)
        return pltpu.make_async_copy(s_hbm.at[sl], sm.at[sl], sem_b.at[1, c])

    def cp_by(c):
        return pltpu.make_async_copy(
            xw.at[c], out_hbm.bitcast(U32).at[:, :, c, pl.ds(DM, DM)], sem_b.at[2, c])

    def cp_w(j, g, a):
        src = (wq_hbm, wk_hbm, wv_hbm)[j].bitcast(U32).at[:, :, :, NB // 2 * g + a, :]
        return pltpu.make_async_copy(src, wblk[j].at[g, :, :, pl.ds(128 * a, 128), :],
                                     sem_w.at[j, a, g])

    def cp_wo(g):
        return pltpu.make_async_copy(wo_hbm.bitcast(U32).at[g], wo.at[g], sem_w.at[3, 0, g])

    def cp_ax(t):
        return pltpu.make_async_copy(ax_hbm.bitcast(U32).at[:, t], ax.at[t], sem_o.at[1, t])

    def cp_ao(t):
        return pltpu.make_async_copy(
            ostage.at[t], out_hbm.at[:, pl.ds(2 * t, 2), :, pl.ds(0, DM)], sem_o.at[0, t])

    def cp_f(j, k, half):
        src, dst = ((wr_hbm, wr), (wi_hbm, wi))[j]
        return pltpu.make_async_copy(
            src.at[pl.ds(256 * half, 256), pl.ds(pl.multiple_of(128 * k, 128), 128)].bitcast(U32),
            dst.at[k, pl.ds(128 * half, 128)], sem_m.at[half])

    def wait_f(half):
        for dst in (wr, wi):
            part = dst.at[:, pl.ds(128 * half, 128)]
            pltpu.make_async_copy(part, part, sem_m.at[half]).wait()

    for c in range(2):
        cp_bx(c).start()
        cp_s(c).start()

    rt = float(np.sqrt(0.5))
    row8 = lax.broadcasted_iota(jnp.int32, (8, 128), 0)

    def b_forward(c, carry):
        @pl.when(c < 6)
        def _():
            cp_bx(c + 2).start()
            cp_s(c + 2).start()

        for j in range(2):
            cp_f(j, 2 * c, 0).start()
            cp_f(j, 2 * c + 1, 0).start()

        @pl.when(c == 7)
        def _():
            cp_ax(T - 1).start()
            cp_ax(T - 2).start()

        cp_bx(c).wait()
        cp_s(c).wait()
        w = xw[c].reshape(128, DM)
        for half, xf in enumerate((_lo(w), _hi(w))):
            x = [xf[:, 128 * al:128 * (al + 1)] for al in range(8)]
            s = [x[i] + x[i + 4] for i in range(4)]
            d = [x[i] - x[i + 4] for i in range(4)]
            e, o = s[0] + s[2], s[1] + s[3]
            p, q = (d[1] - d[3]) * rt, (d[1] + d[3]) * rt
            u = [(e + o, e - o), (d[0] + p, d[2] + q), (s[0] - s[2], s[1] - s[3]),
                 (d[0] - p, d[2] - q)]
            tt = [lax.dot_general(d_ref[k], jnp.concatenate(u[k], axis=1).astype(BF16), NT,
                                  preferred_element_type=F32) for k in range(4)]
            dc, ny = tt[0][0:8], tt[0][128:136]
            re = [jnp.where(row8 == 0, dc * 0.5, dc), tt[0][8:128]]
            im = [jnp.where(row8 == 0, 0.0, ny), tt[0][136:256]]
            for k in range(1, 4):
                re.append(tt[k][0:128])
                im.append(tt[k][128:256])
            re += [jnp.where(row8 == 0, ny * 0.5, 0.0), jnp.zeros((8, 128), F32)]
            im.append(jnp.zeros((16, 128), F32))
            lhs = jnp.concatenate([jnp.concatenate(re, axis=0), jnp.concatenate(im, axis=0)],
                                  axis=1).astype(BF16)
            a = 2 * c + half
            yb[a] = jnp.dot(lhs, sm[a], preferred_element_type=F32)
        return carry

    lax.fori_loop(0, 8, b_forward, 0)
    for k in range(16):
        cp_f(0, k, 1).start()
        cp_f(1, k, 1).start()
    wait_f(0)

    def filt(row, wre, wim):
        y = [(yb[a, pl.ds(row, 8), 0:128], yb[a, pl.ds(row, 8), 128:256]) for a in range(16)]
        z = _fft16(y, -1)
        z = [(z[k][0] * wre(k) - z[k][1] * wim(k), z[k][0] * wim(k) + z[k][1] * wre(k))
             for k in range(16)]
        return _fft16(z, 1)

    def b_filter(i, carry):
        mg, j = i // 4, i % 4

        @pl.when(i == 8)
        def _():
            wait_f(1)

        @pl.when(i >= 16 - NG)
        def _():
            cp_wo(i - (16 - NG)).start()

        for half, un in enumerate((_lo, _hi)):
            off = [ROW_OFF[2 * jj + half] for jj in range(4)]
            base = jnp.where(j < 2, jnp.where(j == 0, off[0], off[1]),
                             jnp.where(j == 2, off[2], off[3])) + 16 * mg
            base = pl.multiple_of(base, 16)
            res = []
            for r8 in range(2):
                sl = pl.ds(64 * mg + 32 * r8 + j, 8, stride=4)
                res.append(filt(pl.multiple_of(base + 8 * r8, 8),
                                lambda k: un(wr[k, sl, :]),
                                lambda k: un(wi[k, sl, :])))
            for a in range(16):
                for ri in range(2):
                    vb[a, pl.ds(base, 16), 128 * ri:128 * (ri + 1)] = jnp.concatenate(
                        [res[0][a][ri], res[1][a][ri]], axis=0).astype(BF16)
        return carry

    lax.fori_loop(0, 16, b_filter, 0)
    res = filt(512, lambda k: wrn_ref[0:1, 128 * k:128 * (k + 1)].astype(F32),
               lambda k: win_ref[0:1, 128 * k:128 * (k + 1)].astype(F32))
    for a in range(16):
        for ri in range(2):
            vb[a, 512:KROWS, 128 * ri:128 * (ri + 1)] = jnp.concatenate(
                [res[a][ri], jnp.zeros((8, 128), F32)], axis=0).astype(BF16)
        vb[a, KROWS:640, :] = jnp.zeros((640 - KROWS, 256), BF16)

    lane0 = lax.broadcasted_iota(jnp.int32, (128, 128), 1) == 0

    def prep_wo(g):
        for c in range(NI):
            for r in range(0, 64, 8):
                w = [[wo[g, i, r:r + 8, 128 * (NB * c + j):128 * (NB * c + j + 1)]
                      for j in range(NB)] for i in range(NB)]
                ev, od = [_right([[un(v) for v in row] for row in w]) for un in (_lo, _hi)]
                for i in range(NB):
                    wo[g, i, r:r + 8, 128 * (NB * c + i):128 * (NB * c + i + 1)] = _words(
                        ev[0][i], od[0][i])
                for n in range(NX):
                    wox[g, 64 * n + r:64 * n + r + 8, 128 * c:128 * (c + 1)] = _words(
                        ev[1][n], od[1][n])

    def b_inverse(c, carry):
        for g in range(NG // 8):
            for a in range(NB // 2):
                cp_w(1, NG // 8 * c + g, a).start()
                cp_w(2, NG // 8 * c + g, a).start()
        for g in range(NG // 8):
            cp_wo(NG // 8 * c + g).wait()
        for g in range(NG // 8):
            prep_wo(NG // 8 * c + g)
        lhs = [[] for _ in range(4)]
        for half in range(2):
            a = 2 * c + half
            z = lax.dot_general(sm[a], vb[a, 0:512, :], NT, preferred_element_type=F32)
            ny = lax.dot_general(sm[a, 0:128, :], vb[a, 512:640, :], NT,
                                 preferred_element_type=F32)
            for k in range(4):
                zr, zi = z[0:128, 128 * k:128 * (k + 1)], z[128:256, 128 * k:128 * (k + 1)]
                if k == 0:
                    zi = jnp.where(lane0, ny, zi)
                lhs[k].append(jnp.concatenate([zr, zi], axis=1).astype(BF16))
        g = [jnp.dot(jnp.concatenate(lhs[k], axis=0), d_ref[k], preferred_element_type=F32)
             for k in range(4)]
        (g0, g4), (g1r, g1i), (g2r, g2i), (g3r, g3i) = [(v[:, :128], v[:, 128:]) for v in g]
        e, o = g0 + g4, g0 - g4
        s = [e + g2r, o + g2i, e - g2r, o - g2i]
        p, q = (g1r - g3r) * rt, (g1i - g3i) * rt
        d = [g1r + g3r, q + p, g1i + g3i, q - p]
        y = [s[i] + d[i] for i in range(4)] + [s[i] - d[i] for i in range(4)]
        for al in range(8):
            bits = _bf16_bits(y[al])
            xw[c, :, :, 128 * al:128 * (al + 1)] = (
                (bits[0:128] >> 16) | bits[128:256]).reshape(8, 16, 128)
        return carry

    lax.fori_loop(0, 8, b_inverse, 0)

    def blocks(v):
        n = v.shape[1] // (128 * NB)
        return [jnp.concatenate([v[:, 128 * (NB * c + i):128 * (NB * c + i + 1)]
                                 for c in range(n)], axis=1) for i in range(NB)]

    def load_x(t):
        for g in range(G // 2):
            top, bot = ax[t, g], ax[t, g + G // 2]
            ev, od = [_left(blocks(un(top)), blocks(un(bot))) for un in (_lo, _hi)]
            for n in range(NL):
                hs[n, SEG // 2 * g:SEG // 2 * (g + 1), :] = _words(ev[n], od[n])

    def set_mem(m):
        for n, v in enumerate(_left(blocks(m[0:MH]), blocks(m[MH:2 * MH]))):
            hs[n, XH // 2:HH // 2, :] = pltpu.bitcast(v.astype(BF16), U32)

    def wait_w(j, g):
        for a in range(NB // 2):
            cp_w(j, g, a).wait()

    def prep_w(j, g):
        ref = wblk[j]

        def raw(c, i, r, n):
            w = [[ref[g, c, i, pl.ds(128 * a + 2 * r + d, n, stride=2), :]
                  for a in range(NB // 2)] for d in range(2)]
            return [[un(v) for v in w[d] for un in (_lo, _hi)] for d in range(2)]

        for c in range(NI):
            for r in range(0, 64, 8):
                b = [raw(c, i, r, 8) for i in range(NB)]
                ev, od = [_right([b[i][d] for i in range(NB)])[1] for d in range(2)]
                for n in range(NX):
                    wext[j][g, c, 64 * n + r:64 * n + r + 8, :] = _words(ev[n], od[n])
        for c in range(NI):
            for i in range(NB):
                ev, od = raw(c, i, 0, 64)
                for v in (ev, od):
                    v[i] = functools.reduce(lambda p, q: p + q, v)
                for e in range(NB):
                    ref[g, c, i, 64 * e:64 * (e + 1), :] = _words(ev[e], od[e])

    def right(blk, ext, b):
        w = ext(64 * b) if isinstance(b, int) else blk(*b)
        w = pltpu.bitcast(w, BF16)
        return w.reshape(w.shape[0] * 128, 128)

    def project(g, r0, r1, lo, hi):
        def mm(a, b):
            w = [right(lambda i, e: wblk[j][g, :, i, 64 * e:64 * (e + 1), :],
                       lambda o: wext[j][g, :, o:o + 64, :], b) for j in range(lo, hi)]
            return jnp.dot(pltpu.bitcast(hs[a, r0 // 2:r1 // 2, :], BF16),
                           jnp.concatenate(w, axis=1), preferred_element_type=F32)

        return _combine(mm)

    def put_o(g, r0, o):
        for n, v in enumerate(_left([h[0] for h in o], [h[1] for h in o])):
            ob[n, g, r0:HH, :] = v.astype(BF16)

    def lanes(k, n=1):
        return pl.ds(pl.multiple_of(128 * k, 128), 128 * n)

    def out_mm(c, r0, a, b, g0, g1):
        o = jnp.concatenate([ob[a, g, r0:HH, :] for g in range(g0, g1)], axis=1)
        w = right(lambda i, e: wo[g0:g1, i, :, lanes(NB * c + e)],
                  lambda o: wox[g0:g1, o:o + 64, lanes(c)], b)
        return jnp.dot(o, w, preferred_element_type=F32)

    def out_mem(c, r0, keep, feed, early=()):
        def mm(a, b):
            if a in early:
                return early[a] + out_mm(c, r0, a, b, NG - 1, NG)
            return out_mm(c, r0, a, b, 0, NG)

        top, bot = _combine(mm)
        x0 = XH - r0
        if keep:
            mend[0:MH, lanes(NB * c, NB)] = jnp.concatenate([v[x0:] for v in top], axis=1)
            mend[MH:2 * MH, lanes(NB * c, NB)] = jnp.concatenate([v[x0:] for v in bot], axis=1)
        if feed:
            for n, v in enumerate(_left([v[x0:] for v in top], [v[x0:] for v in bot])):
                hs[n, XH // 2:HH // 2, lanes(c)] = pltpu.bitcast(v.astype(BF16), U32)
        return [[v[:x0] for v in half] for half in (top, bot)]

    cp_ax(T - 1).wait()
    load_x(T - 1)

    def kv_loop(g, carry):
        for a in range(NB // 2):
            cp_w(0, g, a).start()
        for j, ret in ((1, kret), (2, vret)):
            wait_w(j, g)
        for j, ret in ((1, kret), (2, vret)):
            prep_w(j, g)
            top, bot = project(g, 0, XH, j, j + 1)
            for e in range(NB):
                ret[NB * g + e] = jnp.concatenate([top[e], bot[e]], axis=0).astype(BF16)
        return carry

    lax.fori_loop(0, NG, kv_loop, 0)

    cp_ax(T - 2).wait()
    xbar = jnp.sum(_lo(ax[T - 2]) + _hi(ax[T - 2]), axis=1, keepdims=True) * (1.0 / (SEG + MEM))
    set_mem(jnp.broadcast_to(xbar, (G, MEM, DM)).reshape(G * MEM, DM))

    def guess(g, carry):
        put_o(g, XH, list(zip(*project(g, XH, HH, 2, 3))))
        return carry

    lax.fori_loop(0, NG, guess, 0)
    lax.fori_loop(0, NI, lambda c, carry: (out_mem(c, XH, False, True), carry)[1], 0)

    TILES = ((0, 1, 2), (3, 4, 5), (6, 7))
    nx = [SEG * len(tl) for tl in TILES]
    nm = (32, 32, 16)

    def tile(v, g, with_x):
        m0 = XH if with_x else 0
        parts = [v[ch // 4][SEG * (ch % 4):SEG * (ch % 4 + 1)] for ch in TILES[g]] if with_x else []
        parts += [v[ch // 4][m0 + MEM * (ch % 4):m0 + MEM * (ch % 4 + 1)] for ch in TILES[g]]
        if len(TILES[g]) == 3:
            parts.append(jnp.zeros((MEM, DH), F32))
        return jnp.concatenate(parts, axis=0).astype(BF16)

    def step(mode):
        q_x, kv_x = mode != "pred", mode == "mid"
        q0, kv0 = (0 if q_x else XH), (0 if kv_x else XH)

        def put(ref, e, v, with_x):
            for g in range(3):
                ref[e, g, (0 if with_x else nx[g]):nx[g] + nm[g], :] = tile(v, g, with_x)

        def proj_q(hg):
            q = project(hg, q0, HH, 0, 1)
            for e in range(NB):
                put(qt, e, [half[e] * QSCALE for half in q], q_x)

        def proj_k(hg):
            k = project(hg, kv0, HH, 1, 2)
            for e in range(NB):
                put(kt, e, [half[e] for half in k], kv_x)

        def proj_v(hg):
            v = project(hg, kv0, HH, 2, 3)
            for e in range(NB):
                put(vt, e, [half[e] for half in v], kv_x)

        def get(ref, ret, hg, e, g):
            if kv_x:
                return ref[e, g]
            return jnp.concatenate(
                [ret[NB * hg + e, 96 * g:96 * g + nx[g], :], ref[e, g, nx[g]:128, :]], axis=0)

        def scores(hg, e):
            out = []
            for g in range(3):
                r0 = 0 if q_x else nx[g]
                s = lax.dot_general(qt[e, g, r0:nx[g] + nm[g], :], get(kt, kret, hg, e, g), NT,
                                    preferred_element_type=F32)
                fill = mask_ref[g // 2, r0:nx[g] + nm[g], :]
                s = jnp.where(fill == 0.0, s, fill)
                pr = jnp.exp2(s - jnp.max(s, axis=1, keepdims=True))
                out.append((pr.astype(BF16), jnp.sum(pr, axis=1, keepdims=True)))
            return out

        def values(hg, e, sc):
            xs, ms = [], []
            for g in range(3):
                pr, den = sc[g]
                inv = pl.reciprocal(den, approx=True)
                inv = inv * (2.0 - den * inv)
                o = jnp.dot(pr, get(vt, vret, hg, e, g), preferred_element_type=F32) * inv
                m0 = nx[g] if q_x else 0
                for i in range(len(TILES[g])):
                    if q_x:
                        xs.append(o[SEG * i:SEG * (i + 1)])
                    ms.append(o[m0 + MEM * i:m0 + MEM * (i + 1)])
            return [jnp.concatenate(xs[4 * k:4 * k + 4] + ms[4 * k:4 * k + 4], axis=0)
                    for k in range(2)]

        def group(hg, fill=None):
            sc = [scores(hg, e) for e in range(NB)]
            if fill is not None:
                fill()
            elif q_x:
                proj_q(hg + 1)
            else:
                proj_k(hg + 1)
            o = [values(hg, e, sc[e]) for e in range(NB)]
            if fill is None and q_x:
                proj_k(hg + 1)
            put_o(hg, q0, o)
            if fill is None:
                proj_v(hg + 1)
                if not q_x:
                    proj_q(hg + 1)

        def first():
            proj_k(0)
            proj_v(0)
            proj_q(0)

        return first, group

    kt[:, 2, 80:128, :] = jnp.zeros((NB, 48, DH), BF16)
    vt[:, 2, 80:128, :] = jnp.zeros((NB, 48, DH), BF16)

    first, group = step("pred")
    for t in range(T - 2):
        cp_ax(t).start()
    wait_w(0, 0)
    prep_w(0, 0)
    first()

    def pred_loop(hg, carry):
        wait_w(0, hg + 1)
        prep_w(0, hg + 1)
        group(hg)
        return carry

    lax.fori_loop(0, NG - 1, pred_loop, 0)
    group(NG - 1, lambda: None)
    lax.fori_loop(0, NI, lambda c, carry: (out_mem(c, XH, True, False), carry)[1], 0)
    for t in range(T - 2):
        cp_ax(t).wait()
    for c in range(8):
        cp_by(c).start()
    load_x(0)

    first, group = step("mid")
    group_last = step("last")[1]

    def segment(t, carry):
        first()

        @pl.when(t < T - 1)
        def _():
            lax.fori_loop(0, NG - 1, lambda hg, c: (group(hg), c)[1], 0)

        @pl.when(t == T - 1)
        def _():
            lax.fori_loop(0, NG - 1, lambda hg, c: (group_last(hg), c)[1], 0)
            for e in range(NB):
                for g in range(3):
                    kt[e, g, 0:nx[g], :] = kret[NH - NB + e, 96 * g:96 * g + nx[g], :]
                    vt[e, g, 0:nx[g], :] = vret[NH - NB + e, 96 * g:96 * g + nx[g], :]

        load_x((t + 1) % T)
        early = {}
        group(NG - 1, lambda: early.update({i: out_mm(0, 0, i, i, 0, NG - 1) for i in range(3)}))
        for c in range(NI):
            for k, half in enumerate(out_mem(c, 0, True, True, early if c == 0 else {})):
                for e, v in enumerate(half):
                    ostage[t, 4 * k:4 * k + 4, :, :, 128 * (NB * c + e):128 * (NB * c + e + 1)] = (
                        v.astype(BF16).reshape(G // 2, 2, 16, 128))
        cp_ao(t).start()
        return carry

    def one_pass(carry):
        it, _ = carry
        start = mend[0:(G - 1) * MEM, :]
        mstart[...] = start
        set_mem(jnp.concatenate([mem0_ref[...].astype(F32), start], axis=0))
        lax.fori_loop(0, T, segment, 0)
        real = mend[0:(G - 1) * MEM, :]
        lim = jnp.max(jnp.abs(real), axis=1, keepdims=True) * TOL
        good = jnp.abs(real - mstart[...]) <= lim
        bad = jnp.max(jnp.where(good, 0.0, 1.0))
        for t in range(T):
            cp_ao(t).wait()
        return it + 1, bad

    lax.while_loop(lambda c: jnp.logical_and(c[0] < G, c[1] > 0.0), one_pass,
                   (jnp.int32(0), jnp.float32(1.0)))
    for c in range(8):
        cp_by(c).wait()


@functools.partial(jax.jit, static_argnames=("A_seg_len",))
def pallas_concat_heads__memory_aug_recurrent_mem_tr__spectral_gfnet__prompt_kernel(
    A_x, A_mem0, A_Wq, A_Wk, A_Wv, A_Wo, A_seg_len, B_x, B_w_r, B_w_i,
):
    assert A_seg_len == SEG and A_x.shape == (1, G * T * SEG, DM) and A_Wq.shape == (DM, NH, DH)
    assert A_mem0.shape == (1, MEM, DM) and B_x.shape == (1, 2048, 1024)
    dmat, smat, mask = _constants()
    wr_t, wi_t = B_w_r.T, B_w_i.T
    hbm = pl.BlockSpec(memory_space=pl.ANY)
    nyq = pl.BlockSpec((16, 2048), lambda i: (32, 0))

    def full(shape):
        return pl.BlockSpec(shape, lambda i: (0,) * len(shape))

    out = pl.pallas_call(
        _kernel,
        grid=(1,),
        in_specs=[hbm] * 9 + [full((MEM, DM)), nyq, nyq, full(dmat.shape), full(mask.shape)],
        out_specs=hbm,
        out_shape=jax.ShapeDtypeStruct((G, 16, 16, 2 * DM), BF16),
        scratch_shapes=[
            pltpu.VMEM((T, G, SEG // 2, DM), U32),
            *[pltpu.VMEM((NG, NI, NB, NB * 64, DH), U32)] * 3,
            *[pltpu.VMEM((NG, NI, NX * 64, DH), U32)] * 3,
            pltpu.VMEM((NG, NB, 64, DM), U32),
            pltpu.VMEM((NG, NX * 64, NI * 128), U32),
            pltpu.VMEM((8, 8, 16, 1024), U32),
            pltpu.VMEM((16, 256, 128), U32),
            pltpu.VMEM((16, 256, 128), U32),
            pltpu.VMEM((16, 256, 256), BF16),
            pltpu.VMEM((16, KROWS, 256), F32),
            pltpu.VMEM((16, 640, 256), BF16),
            pltpu.VMEM((NH, G * SEG, DH), BF16),
            pltpu.VMEM((NH, G * SEG, DH), BF16),
            pltpu.VMEM((NL, HH // 2, NI * 128), U32),
            pltpu.VMEM((NB, 3, 128, DH), BF16),
            pltpu.VMEM((NB, 3, 128, DH), BF16),
            pltpu.VMEM((NB, 3, 128, DH), BF16),
            pltpu.VMEM((NL, NG, HH, DH), BF16),
            pltpu.VMEM(((G - 1) * MEM, DM), F32),
            pltpu.VMEM((G * MEM, DM), F32),
            pltpu.VMEM((T, G, 2, 16, DM), BF16),
            pltpu.SemaphoreType.DMA((3, 8)),
            pltpu.SemaphoreType.DMA((4, NB // 2, NG)),
            pltpu.SemaphoreType.DMA((2,)),
            pltpu.SemaphoreType.DMA((2, T)),
        ],
        compiler_params=pltpu.CompilerParams(
            dimension_semantics=("arbitrary",), vmem_limit_bytes=120 * 1024 * 1024),
    )(
        A_x.reshape(G, T, SEG, DM),
        *[w.reshape(NI, NB, 128, NH, DH) for w in (A_Wq, A_Wk, A_Wv)],
        A_Wo.reshape(NG, NB, DH, DM), B_x.reshape(8, 16, 16, 1024), wr_t, wi_t, smat,
        A_mem0.reshape(MEM, DM), wr_t, wi_t, dmat, mask,
    )
    return out.reshape(1, 2048, 2 * DM)
```

```python
import functools

import jax
import jax.numpy as jnp
import numpy as np
from jax import lax
from jax.experimental import pallas as pl
from jax.experimental.pallas import tpu as pltpu

F32 = jnp.float32
BF16 = jnp.bfloat16
U32 = jnp.uint32

G = 8
T = 8
SEG = 32
MEM = 8
DM = 1024
NH = 32
DH = 128
KS = (-4.0 / 3, -1.0 / 3, 1.0 / 3, 4.0 / 3)
NB = len(KS)
PAIRS = [(i, j) for i in range(NB) for j in range(i + 1, NB)]
NL = 2 * NB + 3 * len(PAIRS)
NX = NB + len(PAIRS)
NG = NH // NB
NI = DM // 128 // NB
XH = G // 2 * SEG
MH = G // 2 * MEM
HH = XH + MH
LOG2E = 1.4426950408889634
QSCALE = float(DH ** -0.5 * LOG2E)
MASKED = float(-1e9 * LOG2E)
TOL = 2.0 ** -9
NT = (((1,), (1,)), ((), ()))
KROWS = 528
ROW_OFF = {0: 0, 4: 64, 1: 128, 7: 192, 2: 256, 6: 320, 3: 384, 5: 448}


def _constants():
    beta = np.arange(128)[None, :]
    m = np.arange(64)[:, None]
    d = np.zeros((4, 256, 256))
    for blk, r in enumerate((0, 4)):
        th = 2 * np.pi * (8 * m + r) * beta / 1024
        d[0, 64 * blk:64 * blk + 64, 128 * blk:128 * blk + 128] = np.cos(th)
        d[0, 128 + 64 * blk:192 + 64 * blk, 128 * blk:128 * blk + 128] = -np.sin(th)
    d[0, 128, 0:128] = np.cos(np.pi * np.arange(128))
    for r, sg in ((1, -1.0), (2, -1.0), (3, 1.0)):
        for blk, (res, cj) in enumerate(((r, 1.0), (8 - r, -1.0))):
            th = 2 * np.pi * (8 * m + res) * beta / 1024
            re, im = slice(64 * blk, 64 * blk + 64), slice(128 + 64 * blk, 192 + 64 * blk)
            d[r, re, 0:128] = np.cos(th)
            d[r, im, 0:128] = -np.sin(th)
            d[r, re, 128:256] = sg * cj * np.sin(th)
            d[r, im, 128:256] = sg * cj * np.cos(th)
    d *= 2.0 ** -10
    b = np.arange(128)[:, None]
    kb = np.arange(128)[None, :]
    s = np.zeros((16, 256, 256))
    for a in range(16):
        th = 2 * np.pi * ((kb * (16 * b + a)) % 2048) / 2048
        s[a, :128, :128] = np.cos(th)
        s[a, 128:, :128] = np.sin(th)
        s[a, :128, 128:] = -np.sin(th)
        s[a, 128:, 128:] = np.cos(th)
    mask = np.zeros((2, 128, 128), np.float32)
    for i, ns in enumerate((3, 2)):
        idx = np.arange(128)
        isx = idx < SEG * ns
        pad = idx >= (SEG + MEM) * ns
        seg = np.where(isx, idx // SEG, (idx - SEG * ns) // MEM)
        same = (seg[:, None] == seg[None, :]) & ~pad[None, :]
        future = isx[:, None] & isx[None, :] & (idx[None, :] > idx[:, None])
        mk = np.where(same, np.where(future, MASKED, 0.0), -np.inf)
        mask[i] = np.where(pad[:, None], 0.0, mk)
    return d.astype(BF16), s.astype(BF16), mask


def _lo(w):
    return lax.bitcast_convert_type(w << 16, F32)


def _hi(w):
    return lax.bitcast_convert_type(w & np.uint32(0xFFFF0000), F32)


def _bf16_bits(y):
    return lax.bitcast_convert_type(y.astype(BF16).astype(F32), U32)


def _r4(x, sg):
    (ar, ai), (br, bi), (cr, ci), (dr, di) = x
    s0r, s0i, d0r, d0i = ar + cr, ai + ci, ar - cr, ai - ci
    s1r, s1i, d1r, d1i = br + dr, bi + di, br - dr, bi - di
    p = (d0r - d1i, d0i + d1r)
    q = (d0r + d1i, d0i - d1r)
    y1, y3 = (p, q) if sg > 0 else (q, p)
    return [(s0r + s1r, s0i + s1i), y1, (s0r - s1r, s0i - s1i), y3]


def _tw(z, e, sg):
    r, i = z
    if e == 0:
        return z
    if e == 4:
        return (-i, r) if sg > 0 else (i, -r)
    h = float(np.sqrt(0.5))
    if e == 2:
        return ((r - i) * h, (r + i) * h) if sg > 0 else ((r + i) * h, (i - r) * h)
    if e == 6:
        return ((r + i) * -h, (r - i) * h) if sg > 0 else ((i - r) * h, (r + i) * -h)
    c = float(np.cos(2 * np.pi * e / 16))
    s = float(sg * np.sin(2 * np.pi * e / 16))
    return (r * c - i * s, r * s + i * c)


def _fft16(x, sg):
    t = [_r4([x[4 * a1 + a0] for a1 in range(4)], sg) for a0 in range(4)]
    out = [None] * 16
    for k0 in range(4):
        u = _r4([_tw(t[a0][k0], a0 * k0, sg) for a0 in range(4)], sg)
        for k1 in range(4):
            out[k0 + 4 * k1] = u[k1]
    return out


def _words(even, odd):
    return pltpu.pack_elementwise([even, odd], packed_dtype=BF16)


def _left(x, y):
    z = [x[i] + KS[i] * y[i] for i in range(NB)]
    out = z + list(y)
    for i, j in PAIRS:
        sx, sy = x[i] + x[j], y[i] + y[j]
        out += [z[i] + z[j], sx + KS[j] * sy, sx + KS[i] * sy]
    return out


def _right(b):
    rows = [functools.reduce(lambda u, v: u + v, b[i]) for i in range(NB)]
    extra = [functools.reduce(lambda u, v: u - v, [b[j][i] for j in range(NB) if j != i], b[i][i])
             for i in range(NB)]
    extra += [(b[i][j] + b[j][i]) * (1.0 / (KS[j] - KS[i])) for i, j in PAIRS]
    return rows, extra


def _combine(mm):
    s = [mm(i, i) for i in range(NB)]
    r = [mm(NB + i, (i, i)) for i in range(NB)]
    for n, (i, j) in enumerate(PAIRS):
        p1 = mm(2 * NB + 3 * n, NB + n)
        p2 = mm(2 * NB + 3 * n + 1, (i, j))
        p3 = mm(2 * NB + 3 * n + 2, (j, i))
        d = 1.0 / (KS[j] - KS[i])
        e = (p2 + p3 if d == 1.0 else (p2 + p3) * d) - p1
        r[j], r[i], s[j], s[i] = r[j] + e, r[i] - e, s[j] + p2, s[i] + p3
    return [s[i] - KS[i] * r[i] for i in range(NB)], r


def _kernel(ax_hbm, wq_hbm, wk_hbm, wv_hbm, wo_hbm, bx_hbm, wr_hbm, wi_hbm, s_hbm,
            mem0_ref, wrn_ref, win_ref, d_ref, mask_ref,
            out_hbm,
            ax, wq, wk, wv, wqx, wkx, wvx, wo, wox, xw, wr, wi, sm, yb, vb, kret, vret, hs,
            qt, kt, vt, ob, of, mstart, mend, ostage, sem_b, sem_w, sem_m, sem_o):
    wblk, wext = (wq, wk, wv), (wqx, wkx, wvx)

    def cp_bx(c):
        return pltpu.make_async_copy(bx_hbm.bitcast(U32).at[:, :, c, :], xw.at[c], sem_b.at[0, c])

    def cp_s(c):
        sl = pl.ds(2 * c, 2)
        return pltpu.make_async_copy(s_hbm.at[sl], sm.at[sl], sem_b.at[1, c])

    def cp_by(c):
        return pltpu.make_async_copy(
            xw.at[c], out_hbm.bitcast(U32).at[:, :, c, pl.ds(DM, DM)], sem_b.at[2, c])

    def cp_w(j, g, a):
        src = (wq_hbm, wk_hbm, wv_hbm)[j].bitcast(U32).at[:, :, :, NB // 2 * g + a, :]
        return pltpu.make_async_copy(src, wblk[j].at[g, :, :, pl.ds(128 * a, 128), :],
                                     sem_w.at[j, a, g])

    def cp_wo(g):
        return pltpu.make_async_copy(wo_hbm.bitcast(U32).at[g], wo.at[g], sem_w.at[3, 0, g])

    def cp_ax(t):
        return pltpu.make_async_copy(ax_hbm.bitcast(U32).at[:, t], ax.at[t], sem_o.at[1, t])

    def cp_ao(t):
        return pltpu.make_async_copy(
            ostage.at[t], out_hbm.at[:, pl.ds(2 * t, 2), :, pl.ds(0, DM)], sem_o.at[0, t])

    def cp_f(j, k, half):
        src, dst = ((wr_hbm, wr), (wi_hbm, wi))[j]
        return pltpu.make_async_copy(
            src.at[pl.ds(256 * half, 256), pl.ds(pl.multiple_of(128 * k, 128), 128)].bitcast(U32),
            dst.at[k, pl.ds(128 * half, 128)], sem_m.at[half])

    def wait_f(half):
        for dst in (wr, wi):
            part = dst.at[:, pl.ds(128 * half, 128)]
            pltpu.make_async_copy(part, part, sem_m.at[half]).wait()

    for c in range(2):
        cp_bx(c).start()
        cp_s(c).start()

    rt = float(np.sqrt(0.5))
    row8 = lax.broadcasted_iota(jnp.int32, (8, 128), 0)

    def b_forward(c, carry):
        @pl.when(c < 6)
        def _():
            cp_bx(c + 2).start()
            cp_s(c + 2).start()

        for j in range(2):
            cp_f(j, 2 * c, 0).start()
            cp_f(j, 2 * c + 1, 0).start()

        @pl.when(c == 7)
        def _():
            cp_ax(T - 1).start()
            cp_ax(T - 2).start()

        cp_bx(c).wait()
        cp_s(c).wait()
        w = xw[c].reshape(128, DM)
        for half, xf in enumerate((_lo(w), _hi(w))):
            x = [xf[:, 128 * al:128 * (al + 1)] for al in range(8)]
            s = [x[i] + x[i + 4] for i in range(4)]
            d = [x[i] - x[i + 4] for i in range(4)]
            e, o = s[0] + s[2], s[1] + s[3]
            p, q = (d[1] - d[3]) * rt, (d[1] + d[3]) * rt
            u = [(e + o, e - o), (d[0] + p, d[2] + q), (s[0] - s[2], s[1] - s[3]),
                 (d[0] - p, d[2] - q)]
            tt = [lax.dot_general(d_ref[k], jnp.concatenate(u[k], axis=1).astype(BF16), NT,
                                  preferred_element_type=F32) for k in range(4)]
            dc, ny = tt[0][0:8], tt[0][128:136]
            re = [jnp.where(row8 == 0, dc * 0.5, dc), tt[0][8:128]]
            im = [jnp.where(row8 == 0, 0.0, ny), tt[0][136:256]]
            for k in range(1, 4):
                re.append(tt[k][0:128])
                im.append(tt[k][128:256])
            re += [jnp.where(row8 == 0, ny * 0.5, 0.0), jnp.zeros((8, 128), F32)]
            im.append(jnp.zeros((16, 128), F32))
            lhs = jnp.concatenate([jnp.concatenate(re, axis=0), jnp.concatenate(im, axis=0)],
                                  axis=1).astype(BF16)
            a = 2 * c + half
            yb[a] = jnp.dot(lhs, sm[a], preferred_element_type=F32)
        return carry

    lax.fori_loop(0, 8, b_forward, 0)
    for k in range(16):
        cp_f(0, k, 1).start()
        cp_f(1, k, 1).start()
    wait_f(0)

    def filt(row, wre, wim):
        y = [(yb[a, pl.ds(row, 8), 0:128], yb[a, pl.ds(row, 8), 128:256]) for a in range(16)]
        z = _fft16(y, -1)
        z = [(z[k][0] * wre(k) - z[k][1] * wim(k), z[k][0] * wim(k) + z[k][1] * wre(k))
             for k in range(16)]
        return _fft16(z, 1)

    def b_filter(i, carry):
        mg, j = i // 4, i % 4

        @pl.when(i == 8)
        def _():
            wait_f(1)

        @pl.when(i >= 16 - NG)
        def _():
            cp_wo(i - (16 - NG)).start()

        for half, un in enumerate((_lo, _hi)):
            off = [ROW_OFF[2 * jj + half] for jj in range(4)]
            base = jnp.where(j < 2, jnp.where(j == 0, off[0], off[1]),
                             jnp.where(j == 2, off[2], off[3])) + 16 * mg
            base = pl.multiple_of(base, 16)
            res = []
            for r8 in range(2):
                sl = pl.ds(64 * mg + 32 * r8 + j, 8, stride=4)
                res.append(filt(pl.multiple_of(base + 8 * r8, 8),
                                lambda k: un(wr[k, sl, :]),
                                lambda k: un(wi[k, sl, :])))
            for a in range(16):
                for ri in range(2):
                    vb[a, pl.ds(base, 16), 128 * ri:128 * (ri + 1)] = jnp.concatenate(
                        [res[0][a][ri], res[1][a][ri]], axis=0).astype(BF16)
        return carry

    lax.fori_loop(0, 16, b_filter, 0)
    res = filt(512, lambda k: wrn_ref[0:1, 128 * k:128 * (k + 1)].astype(F32),
               lambda k: win_ref[0:1, 128 * k:128 * (k + 1)].astype(F32))
    for a in range(16):
        for ri in range(2):
            vb[a, 512:KROWS, 128 * ri:128 * (ri + 1)] = jnp.concatenate(
                [res[a][ri], jnp.zeros((8, 128), F32)], axis=0).astype(BF16)
        vb[a, KROWS:640, :] = jnp.zeros((640 - KROWS, 256), BF16)

    lane0 = lax.broadcasted_iota(jnp.int32, (128, 128), 1) == 0

    def prep_wo(g):
        for c in range(NI):
            for r in range(0, 64, 8):
                w = [[wo[g, i, r:r + 8, 128 * (NB * c + j):128 * (NB * c + j + 1)]
                      for j in range(NB)] for i in range(NB)]
                ev, od = [_right([[un(v) for v in row] for row in w]) for un in (_lo, _hi)]
                for i in range(NB):
                    wo[g, i, r:r + 8, 128 * (NB * c + i):128 * (NB * c + i + 1)] = _words(
                        ev[0][i], od[0][i])
                for n in range(NX):
                    wox[g, 64 * n + r:64 * n + r + 8, 128 * c:128 * (c + 1)] = _words(
                        ev[1][n], od[1][n])

    def b_inverse(c, carry):
        for g in range(NG // 8):
            for a in range(NB // 2):
                cp_w(1, NG // 8 * c + g, a).start()
                cp_w(2, NG // 8 * c + g, a).start()
        for g in range(NG // 8):
            cp_wo(NG // 8 * c + g).wait()
        for g in range(NG // 8):
            prep_wo(NG // 8 * c + g)
        lhs = [[] for _ in range(4)]
        for half in range(2):
            a = 2 * c + half
            z = lax.dot_general(sm[a], vb[a, 0:512, :], NT, preferred_element_type=F32)
            ny = lax.dot_general(sm[a, 0:128, :], vb[a, 512:640, :], NT,
                                 preferred_element_type=F32)
            for k in range(4):
                zr, zi = z[0:128, 128 * k:128 * (k + 1)], z[128:256, 128 * k:128 * (k + 1)]
                if k == 0:
                    zi = jnp.where(lane0, ny, zi)
                lhs[k].append(jnp.concatenate([zr, zi], axis=1).astype(BF16))
        g = [jnp.dot(jnp.concatenate(lhs[k], axis=0), d_ref[k], preferred_element_type=F32)
             for k in range(4)]
        (g0, g4), (g1r, g1i), (g2r, g2i), (g3r, g3i) = [(v[:, :128], v[:, 128:]) for v in g]
        e, o = g0 + g4, g0 - g4
        s = [e + g2r, o + g2i, e - g2r, o - g2i]
        p, q = (g1r - g3r) * rt, (g1i - g3i) * rt
        d = [g1r + g3r, q + p, g1i + g3i, q - p]
        y = [s[i] + d[i] for i in range(4)] + [s[i] - d[i] for i in range(4)]
        for al in range(8):
            bits = _bf16_bits(y[al])
            xw[c, :, :, 128 * al:128 * (al + 1)] = (
                (bits[0:128] >> 16) | bits[128:256]).reshape(8, 16, 128)
        return carry

    lax.fori_loop(0, 8, b_inverse, 0)

    def blocks(v):
        n = v.shape[1] // (128 * NB)
        return [jnp.concatenate([v[:, 128 * (NB * c + i):128 * (NB * c + i + 1)]
                                 for c in range(n)], axis=1) for i in range(NB)]

    def x_pieces(t):
        def piece(g, c):
            cols = slice(128 * NB * c, 128 * NB * (c + 1))
            top, bot = ax[t, g, :, cols], ax[t, g + G // 2, :, cols]
            ev, od = [_left(blocks(un(top)), blocks(un(bot))) for un in (_lo, _hi)]
            for n in range(NL):
                hs[n, SEG // 2 * g:SEG // 2 * (g + 1), 128 * c:128 * (c + 1)] = _words(ev[n], od[n])

        return [functools.partial(piece, g, c) for g in range(G // 2) for c in range(NI)]

    def load_x(t):
        for fn in x_pieces(t):
            fn()

    def set_mem(m):
        for n, v in enumerate(_left(blocks(m[0:MH]), blocks(m[MH:2 * MH]))):
            hs[n, XH // 2:HH // 2, :] = pltpu.bitcast(v.astype(BF16), U32)

    def wait_w(j, g):
        for a in range(NB // 2):
            cp_w(j, g, a).wait()

    def prep_w(j, g):
        ref = wblk[j]

        def raw(c, i, r, n):
            w = [[ref[g, c, i, pl.ds(128 * a + 2 * r + d, n, stride=2), :]
                  for a in range(NB // 2)] for d in range(2)]
            return [[un(v) for v in w[d] for un in (_lo, _hi)] for d in range(2)]

        for c in range(NI):
            for r in range(0, 64, 8):
                b = [raw(c, i, r, 8) for i in range(NB)]
                ev, od = [_right([b[i][d] for i in range(NB)])[1] for d in range(2)]
                for n in range(NX):
                    wext[j][g, c, 64 * n + r:64 * n + r + 8, :] = _words(ev[n], od[n])
        for c in range(NI):
            for i in range(NB):
                ev, od = raw(c, i, 0, 64)
                for v in (ev, od):
                    v[i] = functools.reduce(lambda p, q: p + q, v)
                for e in range(NB):
                    ref[g, c, i, 64 * e:64 * (e + 1), :] = _words(ev[e], od[e])

    def right(blk, ext, b):
        w = ext(64 * b) if isinstance(b, int) else blk(*b)
        w = pltpu.bitcast(w, BF16)
        return w.reshape(w.shape[0] * 128, 128)

    def spread(extra):
        at = {NL * n // len(extra): fn for n, fn in enumerate(extra)}
        return lambda a: at[a]() if a in at else None

    def project(g, rows, extra=()):
        hook = spread(extra)

        def mm(a, b):
            hook(a)
            return jnp.concatenate([
                jnp.dot(pltpu.bitcast(hs[a, r0 // 2:r1 // 2, :], BF16),
                        right(lambda i, e: wblk[j][g, :, i, 64 * e:64 * (e + 1), :],
                              lambda o: wext[j][g, :, o:o + 64, :], b),
                        preferred_element_type=F32) for j, (r0, r1) in rows.items()], axis=0)

        res, out, r = _combine(mm), {}, 0
        for j, (r0, r1) in rows.items():
            out[j] = [[v[r:r + r1 - r0] for v in half] for half in res]
            r += r1 - r0
        return out

    def put_o(g, r0, o):
        for n, v in enumerate(_left([h[0] for h in o], [h[1] for h in o])):
            ob[n, g, r0:HH, :] = v.astype(BF16)

    def put_o_pieces(g, r0):
        def own(i):
            x, y = of[i, 0, r0:HH, :], of[i, 1, r0:HH, :]
            ob[i, g, r0:HH, :] = (x + KS[i] * y).astype(BF16)
            ob[NB + i, g, r0:HH, :] = y.astype(BF16)

        def cross(n, i, j):
            yi = of[i, 1, r0:HH, :]
            sx, sy = of[i, 0, r0:HH, :] + of[j, 0, r0:HH, :], yi + of[j, 1, r0:HH, :]
            p2, d = sx + KS[j] * sy, KS[j] - KS[i]
            for m, v in enumerate((p2 - (yi if d == 1.0 else d * yi), p2, sx + KS[i] * sy)):
                ob[2 * NB + 3 * n + m, g, r0:HH, :] = v.astype(BF16)

        return ([functools.partial(own, i) for i in range(NB)]
                + [functools.partial(cross, n, i, j) for n, (i, j) in enumerate(PAIRS)])

    def lanes(k, n=1):
        return pl.ds(pl.multiple_of(128 * k, 128), 128 * n)

    def out_mm(c, r0, a, b, g0, g1):
        o = jnp.concatenate([ob[a, g, r0:HH, :] for g in range(g0, g1)], axis=1)
        w = right(lambda i, e: wo[g0:g1, i, :, lanes(NB * c + e)],
                  lambda o: wox[g0:g1, o:o + 64, lanes(c)], b)
        return jnp.dot(o, w, preferred_element_type=F32)

    def out_mem(c, r0, keep, feed, early=(), extra=()):
        hook = spread(extra)

        def mm(a, b):
            hook(a)
            if a in early:
                return early[a] + out_mm(c, r0, a, b, NG - 1, NG)
            return out_mm(c, r0, a, b, 0, NG)

        top, bot = _combine(mm)
        x0 = XH - r0
        if keep:
            mend[0:MH, lanes(NB * c, NB)] = jnp.concatenate([v[x0:] for v in top], axis=1)
            mend[MH:2 * MH, lanes(NB * c, NB)] = jnp.concatenate([v[x0:] for v in bot], axis=1)
        if feed:
            for n, v in enumerate(_left([v[x0:] for v in top], [v[x0:] for v in bot])):
                hs[n, XH // 2:HH // 2, lanes(c)] = pltpu.bitcast(v.astype(BF16), U32)
        return [[v[:x0] for v in half] for half in (top, bot)]

    cp_ax(T - 1).wait()
    load_x(T - 1)

    def kv_loop(g, carry):
        for a in range(NB // 2):
            cp_w(0, g, a).start()
        for j, ret in ((1, kret), (2, vret)):
            wait_w(j, g)
        for j, ret in ((1, kret), (2, vret)):
            prep_w(j, g)
            top, bot = project(g, {j: (0, XH)})[j]
            for e in range(NB):
                ret[NB * g + e] = jnp.concatenate([top[e], bot[e]], axis=0).astype(BF16)
        return carry

    lax.fori_loop(0, NG, kv_loop, 0)

    cp_ax(T - 2).wait()
    xbar = jnp.sum(_lo(ax[T - 2]) + _hi(ax[T - 2]), axis=1, keepdims=True) * (1.0 / (SEG + MEM))
    set_mem(jnp.broadcast_to(xbar, (G, MEM, DM)).reshape(G * MEM, DM))

    def guess(g, carry):
        put_o(g, XH, list(zip(*project(g, {2: (XH, HH)})[2])))
        return carry

    lax.fori_loop(0, NG, guess, 0)
    lax.fori_loop(0, NI, lambda c, carry: (out_mem(c, XH, False, True), carry)[1], 0)

    TILES = ((0, 1, 2), (3, 4, 5), (6, 7))
    nx = [SEG * len(tl) for tl in TILES]
    nm = (32, 32, 16)

    def tile(v, g, with_x):
        m0 = XH if with_x else 0
        parts = [v[ch // 4][SEG * (ch % 4):SEG * (ch % 4 + 1)] for ch in TILES[g]] if with_x else []
        parts += [v[ch // 4][m0 + MEM * (ch % 4):m0 + MEM * (ch % 4 + 1)] for ch in TILES[g]]
        if len(TILES[g]) == 3:
            parts.append(jnp.zeros((MEM, DH), F32))
        return jnp.concatenate(parts, axis=0).astype(BF16)

    def step(mode):
        q_x, kv_x = mode != "pred", mode == "mid"
        q0, kv0 = (0 if q_x else XH), (0 if kv_x else XH)

        def put(ref, e, v, with_x):
            for g in range(3):
                ref[e, g, (0 if with_x else nx[g]):nx[g] + nm[g], :] = tile(v, g, with_x)

        def proj(hg, mats, extra=()):
            res = project(hg, {j: (kv0 if j else q0, HH) for j in mats}, extra)
            for j in mats:
                for e in range(NB):
                    v = [half[e] if j else half[e] * QSCALE for half in res[j]]
                    put((qt, kt, vt)[j], e, v, kv_x if j else q_x)

        def get(ref, ret, hg, e, g):
            if kv_x:
                return ref[e, g]
            return jnp.concatenate(
                [ret[NB * hg + e, 96 * g:96 * g + nx[g], :], ref[e, g, nx[g]:128, :]], axis=0)

        def scores(hg, e):
            out = []
            for g in range(3):
                r0 = 0 if q_x else nx[g]
                s = lax.dot_general(qt[e, g, r0:nx[g] + nm[g], :], get(kt, kret, hg, e, g), NT,
                                    preferred_element_type=F32)
                fill = mask_ref[g // 2, r0:nx[g] + nm[g], :]
                s = jnp.where(fill == 0.0, s, fill)
                pr = jnp.exp2(s - jnp.max(s, axis=1, keepdims=True))
                out.append((pr.astype(BF16), jnp.sum(pr, axis=1, keepdims=True)))
            return out

        def values(hg, e, sc):
            xs, ms = [], []
            for g in range(3):
                pr, den = sc[g]
                inv = pl.reciprocal(den, approx=True)
                inv = inv * (2.0 - den * inv)
                o = jnp.dot(pr, get(vt, vret, hg, e, g), preferred_element_type=F32) * inv
                m0 = nx[g] if q_x else 0
                for i in range(len(TILES[g])):
                    if q_x:
                        xs.append(o[SEG * i:SEG * (i + 1)])
                    ms.append(o[m0 + MEM * i:m0 + MEM * (i + 1)])
            return [jnp.concatenate(xs[4 * k:4 * k + 4] + ms[4 * k:4 * k + 4], axis=0)
                    for k in range(2)]

        def group(hg, fill=None):
            sc = [scores(hg, e) for e in range(NB)]
            if fill is not None:
                fill()
                put_o(hg, q0, [values(hg, e, sc[e]) for e in range(NB)])
                return

            def park(e):
                for k, v in enumerate(values(hg, e, sc[e])):
                    of[e, k, q0:HH, :] = v

            parks = [functools.partial(park, e) for e in range(NB)]
            if mode == "mid":
                proj(hg + 1, [0, 1, 2], [lambda: None] * 4 + parks + put_o_pieces(hg, q0))
            elif mode == "last":
                proj(hg + 1, [0], [lambda: None] * 2 + parks)
                proj(hg + 1, [1, 2], put_o_pieces(hg, q0))
            else:
                proj(hg + 1, [1, 2, 0], [lambda: None] * 4 + parks + put_o_pieces(hg, q0))

        def first():
            for mats in ([[0, 1, 2]] if mode == "mid" else [[1, 2, 0]]):
                proj(0, mats)

        return first, group

    kt[:, 2, 80:128, :] = jnp.zeros((NB, 48, DH), BF16)
    vt[:, 2, 80:128, :] = jnp.zeros((NB, 48, DH), BF16)

    first, group = step("pred")
    for t in range(T - 2):
        cp_ax(t).start()
    wait_w(0, 0)
    prep_w(0, 0)
    first()

    def pred_loop(hg, carry):
        wait_w(0, hg + 1)
        prep_w(0, hg + 1)
        group(hg)
        return carry

    lax.fori_loop(0, NG - 1, pred_loop, 0)
    group(NG - 1, lambda: None)
    lax.fori_loop(0, NI, lambda c, carry: (out_mem(c, XH, True, False), carry)[1], 0)
    for t in range(T - 2):
        cp_ax(t).wait()
    for c in range(8):
        cp_by(c).start()
    load_x(0)

    first, group = step("mid")
    group_last = step("last")[1]

    def segment(t, carry):
        first()

        @pl.when(t < T - 1)
        def _():
            lax.fori_loop(0, NG - 1, lambda hg, c: (group(hg), c)[1], 0)

        @pl.when(t == T - 1)
        def _():
            lax.fori_loop(0, NG - 1, lambda hg, c: (group_last(hg), c)[1], 0)
            for e in range(NB):
                for g in range(3):
                    kt[e, g, 0:nx[g], :] = kret[NH - NB + e, 96 * g:96 * g + nx[g], :]
                    vt[e, g, 0:nx[g], :] = vret[NH - NB + e, 96 * g:96 * g + nx[g], :]

        nxt = x_pieces((t + 1) % T)
        per = len(nxt) // NI
        early = {}
        group(NG - 1, lambda: early.update({i: out_mm(0, 0, i, i, 0, NG - 1) for i in range(3)}))
        for c in range(NI):
            for k, half in enumerate(out_mem(c, 0, True, True, early if c == 0 else {},
                                             nxt[per * c:per * (c + 1)])):
                for e, v in enumerate(half):
                    ostage[t, 4 * k:4 * k + 4, :, :, 128 * (NB * c + e):128 * (NB * c + e + 1)] = (
                        v.astype(BF16).reshape(G // 2, 2, 16, 128))
        cp_ao(t).start()
        return carry

    def one_pass(carry):
        it, _ = carry
        start = mend[0:(G - 1) * MEM, :]
        mstart[...] = start
        set_mem(jnp.concatenate([mem0_ref[...].astype(F32), start], axis=0))
        lax.fori_loop(0, T, segment, 0)
        real = mend[0:(G - 1) * MEM, :]
        lim = jnp.max(jnp.abs(real), axis=1, keepdims=True) * TOL
        good = jnp.abs(real - mstart[...]) <= lim
        bad = jnp.max(jnp.where(good, 0.0, 1.0))
        for t in range(T):
            cp_ao(t).wait()
        return it + 1, bad

    lax.while_loop(lambda c: jnp.logical_and(c[0] < G, c[1] > 0.0), one_pass,
                   (jnp.int32(0), jnp.float32(1.0)))
    for c in range(8):
        cp_by(c).wait()


@functools.partial(jax.jit, static_argnames=("A_seg_len",))
def pallas_concat_heads__memory_aug_recurrent_mem_tr__spectral_gfnet__prompt_kernel(
    A_x, A_mem0, A_Wq, A_Wk, A_Wv, A_Wo, A_seg_len, B_x, B_w_r, B_w_i,
):
    assert A_seg_len == SEG and A_x.shape == (1, G * T * SEG, DM) and A_Wq.shape == (DM, NH, DH)
    assert A_mem0.shape == (1, MEM, DM) and B_x.shape == (1, 2048, 1024)
    dmat, smat, mask = _constants()
    wr_t, wi_t = B_w_r.T, B_w_i.T
    hbm = pl.BlockSpec(memory_space=pl.ANY)
    nyq = pl.BlockSpec((16, 2048), lambda i: (32, 0))

    def full(shape):
        return pl.BlockSpec(shape, lambda i: (0,) * len(shape))

    out = pl.pallas_call(
        _kernel,
        grid=(1,),
        in_specs=[hbm] * 9 + [full((MEM, DM)), nyq, nyq, full(dmat.shape), full(mask.shape)],
        out_specs=hbm,
        out_shape=jax.ShapeDtypeStruct((G, 16, 16, 2 * DM), BF16),
        scratch_shapes=[
            pltpu.VMEM((T, G, SEG // 2, DM), U32),
            *[pltpu.VMEM((NG, NI, NB, NB * 64, DH), U32)] * 3,
            *[pltpu.VMEM((NG, NI, NX * 64, DH), U32)] * 3,
            pltpu.VMEM((NG, NB, 64, DM), U32),
            pltpu.VMEM((NG, NX * 64, NI * 128), U32),
            pltpu.VMEM((8, 8, 16, 1024), U32),
            pltpu.VMEM((16, 256, 128), U32),
            pltpu.VMEM((16, 256, 128), U32),
            pltpu.VMEM((16, 256, 256), BF16),
            pltpu.VMEM((16, KROWS, 256), F32),
            pltpu.VMEM((16, 640, 256), BF16),
            pltpu.VMEM((NH, G * SEG, DH), BF16),
            pltpu.VMEM((NH, G * SEG, DH), BF16),
            pltpu.VMEM((NL, HH // 2, NI * 128), U32),
            pltpu.VMEM((NB, 3, 128, DH), BF16),
            pltpu.VMEM((NB, 3, 128, DH), BF16),
            pltpu.VMEM((NB, 3, 128, DH), BF16),
            pltpu.VMEM((NL, NG, HH, DH), BF16),
            pltpu.VMEM((NB, 2, HH, DH), F32),
            pltpu.VMEM(((G - 1) * MEM, DM), F32),
            pltpu.VMEM((G * MEM, DM), F32),
            pltpu.VMEM((T, G, 2, 16, DM), BF16),
            pltpu.SemaphoreType.DMA((3, 8)),
            pltpu.SemaphoreType.DMA((4, NB // 2, NG)),
            pltpu.SemaphoreType.DMA((2,)),
            pltpu.SemaphoreType.DMA((2, T)),
        ],
        compiler_params=pltpu.CompilerParams(
            dimension_semantics=("arbitrary",), vmem_limit_bytes=120 * 1024 * 1024),
    )(
        A_x.reshape(G, T, SEG, DM),
        *[w.reshape(NI, NB, 128, NH, DH) for w in (A_Wq, A_Wk, A_Wv)],
        A_Wo.reshape(NG, NB, DH, DM), B_x.reshape(8, 16, 16, 1024), wr_t, wi_t, smat,
        A_mem0.reshape(MEM, DM), wr_t, wi_t, dmat, mask,
    )
    return out.reshape(1, 2048, 2 * DM)
```

```python
import functools

import jax
import jax.numpy as jnp
import numpy as np
from jax import lax
from jax.experimental import pallas as pl
from jax.experimental.pallas import tpu as pltpu

F32 = jnp.float32
BF16 = jnp.bfloat16
U32 = jnp.uint32

G = 8
T = 8
SEG = 32
MEM = 8
DM = 1024
NH = 32
DH = 128
KS = (-4.0 / 3, -1.0 / 3, 1.0 / 3, 4.0 / 3)
NB = len(KS)
PAIRS = [(i, j) for i in range(NB) for j in range(i + 1, NB)]
NL = 2 * NB + 3 * len(PAIRS)
NX = NB + len(PAIRS)
NG = NH // NB
NI = DM // 128 // NB
XH = G // 2 * SEG
MH = G // 2 * MEM
HH = XH + MH
LOG2E = 1.4426950408889634
QSCALE = float(DH ** -0.5 * LOG2E)
MASKED = float(-1e9 * LOG2E)
TOL = 2.0 ** -9
NT = (((1,), (1,)), ((), ()))
KROWS = 528
ROW_OFF = {0: 0, 4: 64, 1: 128, 7: 192, 2: 256, 6: 320, 3: 384, 5: 448}


def _constants():
    beta = np.arange(128)[None, :]
    m = np.arange(64)[:, None]
    d = np.zeros((4, 256, 256))
    for blk, r in enumerate((0, 4)):
        th = 2 * np.pi * (8 * m + r) * beta / 1024
        d[0, 64 * blk:64 * blk + 64, 128 * blk:128 * blk + 128] = np.cos(th)
        d[0, 128 + 64 * blk:192 + 64 * blk, 128 * blk:128 * blk + 128] = -np.sin(th)
    d[0, 128, 0:128] = np.cos(np.pi * np.arange(128))
    for r, sg in ((1, -1.0), (2, -1.0), (3, 1.0)):
        for blk, (res, cj) in enumerate(((r, 1.0), (8 - r, -1.0))):
            th = 2 * np.pi * (8 * m + res) * beta / 1024
            re, im = slice(64 * blk, 64 * blk + 64), slice(128 + 64 * blk, 192 + 64 * blk)
            d[r, re, 0:128] = np.cos(th)
            d[r, im, 0:128] = -np.sin(th)
            d[r, re, 128:256] = sg * cj * np.sin(th)
            d[r, im, 128:256] = sg * cj * np.cos(th)
    d *= 2.0 ** -10
    b = np.arange(128)[:, None]
    kb = np.arange(128)[None, :]
    s = np.zeros((16, 256, 256))
    for a in range(16):
        th = 2 * np.pi * ((kb * (16 * b + a)) % 2048) / 2048
        s[a, :128, :128] = np.cos(th)
        s[a, 128:, :128] = np.sin(th)
        s[a, :128, 128:] = -np.sin(th)
        s[a, 128:, 128:] = np.cos(th)
    mask = np.zeros((2, 128, 128), np.float32)
    for i, ns in enumerate((3, 2)):
        idx = np.arange(128)
        isx = idx < SEG * ns
        pad = idx >= (SEG + MEM) * ns
        seg = np.where(isx, idx // SEG, (idx - SEG * ns) // MEM)
        same = (seg[:, None] == seg[None, :]) & ~pad[None, :]
        future = isx[:, None] & isx[None, :] & (idx[None, :] > idx[:, None])
        mk = np.where(same, np.where(future, MASKED, 0.0), -np.inf)
        mask[i] = np.where(pad[:, None], 0.0, mk)
    return d.astype(BF16), s.astype(BF16), mask


def _lo(w):
    return lax.bitcast_convert_type(w << 16, F32)


def _hi(w):
    return lax.bitcast_convert_type(w & np.uint32(0xFFFF0000), F32)


def _bf16_bits(y):
    return lax.bitcast_convert_type(y.astype(BF16).astype(F32), U32)


def _r4(x, sg):
    (ar, ai), (br, bi), (cr, ci), (dr, di) = x
    s0r, s0i, d0r, d0i = ar + cr, ai + ci, ar - cr, ai - ci
    s1r, s1i, d1r, d1i = br + dr, bi + di, br - dr, bi - di
    p = (d0r - d1i, d0i + d1r)
    q = (d0r + d1i, d0i - d1r)
    y1, y3 = (p, q) if sg > 0 else (q, p)
    return [(s0r + s1r, s0i + s1i), y1, (s0r - s1r, s0i - s1i), y3]


def _tw(z, e, sg):
    r, i = z
    if e == 0:
        return z
    if e == 4:
        return (-i, r) if sg > 0 else (i, -r)
    h = float(np.sqrt(0.5))
    if e == 2:
        return ((r - i) * h, (r + i) * h) if sg > 0 else ((r + i) * h, (i - r) * h)
    if e == 6:
        return ((r + i) * -h, (r - i) * h) if sg > 0 else ((i - r) * h, (r + i) * -h)
    c = float(np.cos(2 * np.pi * e / 16))
    s = float(sg * np.sin(2 * np.pi * e / 16))
    return (r * c - i * s, r * s + i * c)


def _fft16(x, sg):
    t = [_r4([x[4 * a1 + a0] for a1 in range(4)], sg) for a0 in range(4)]
    out = [None] * 16
    for k0 in range(4):
        u = _r4([_tw(t[a0][k0], a0 * k0, sg) for a0 in range(4)], sg)
        for k1 in range(4):
            out[k0 + 4 * k1] = u[k1]
    return out


def _words(even, odd):
    return pltpu.pack_elementwise([even, odd], packed_dtype=BF16)


def _left(x, y):
    z = [x[i] + KS[i] * y[i] for i in range(NB)]
    out = z + list(y)
    for i, j in PAIRS:
        sx, sy = x[i] + x[j], y[i] + y[j]
        out += [z[i] + z[j], sx + KS[j] * sy, sx + KS[i] * sy]
    return out


def _right(b):
    rows = [functools.reduce(lambda u, v: u + v, b[i]) for i in range(NB)]
    extra = [functools.reduce(lambda u, v: u - v, [b[j][i] for j in range(NB) if j != i], b[i][i])
             for i in range(NB)]
    extra += [(b[i][j] + b[j][i]) * (1.0 / (KS[j] - KS[i])) for i, j in PAIRS]
    return rows, extra


def _combine(mm):
    s = [mm(i, i) for i in range(NB)]
    r = [mm(NB + i, (i, i)) for i in range(NB)]
    for n, (i, j) in enumerate(PAIRS):
        p1 = mm(2 * NB + 3 * n, NB + n)
        p2 = mm(2 * NB + 3 * n + 1, (i, j))
        p3 = mm(2 * NB + 3 * n + 2, (j, i))
        d = 1.0 / (KS[j] - KS[i])
        e = (p2 + p3 if d == 1.0 else (p2 + p3) * d) - p1
        r[j], r[i], s[j], s[i] = r[j] + e, r[i] - e, s[j] + p2, s[i] + p3
    return [s[i] - KS[i] * r[i] for i in range(NB)], r


def _kernel(ax_hbm, wq_hbm, wk_hbm, wv_hbm, wo_hbm, bx_hbm, wr_hbm, wi_hbm, s_hbm,
            mem0_ref, wrn_ref, win_ref, d_ref, mask_ref,
            out_hbm,
            ax, wq, wk, wv, wqx, wkx, wvx, wo, wox, xw, wr, wi, sm, yb, vb, kret, vret, hs,
            qt, kt, vt, ob, of, mstart, mend, ostage, sem_b, sem_w, sem_m, sem_o):
    wblk, wext = (wq, wk, wv), (wqx, wkx, wvx)

    def cp_bx(c):
        return pltpu.make_async_copy(bx_hbm.bitcast(U32).at[:, :, c, :], xw.at[c], sem_b.at[0, c])

    def cp_s(c):
        sl = pl.ds(2 * c, 2)
        return pltpu.make_async_copy(s_hbm.at[sl], sm.at[sl], sem_b.at[1, c])

    def cp_by(c):
        return pltpu.make_async_copy(
            xw.at[c], out_hbm.bitcast(U32).at[:, :, c, pl.ds(DM, DM)], sem_b.at[2, c])

    def cp_w(j, g, a):
        src = (wq_hbm, wk_hbm, wv_hbm)[j].bitcast(U32).at[:, :, :, NB // 2 * g + a, :]
        return pltpu.make_async_copy(src, wblk[j].at[g, :, :, pl.ds(128 * a, 128), :],
                                     sem_w.at[j, a, g])

    def start_w(j, g):
        for a in range(NB // 2):
            cp_w(j, g, a).start()

    def cp_wo(g):
        return pltpu.make_async_copy(wo_hbm.bitcast(U32).at[g], wo.at[g], sem_w.at[3, 0, g])

    def cp_ax(t):
        return pltpu.make_async_copy(ax_hbm.bitcast(U32).at[:, t], ax.at[t], sem_o.at[1, t])

    def cp_ao(t):
        return pltpu.make_async_copy(
            ostage.at[t], out_hbm.at[:, pl.ds(2 * t, 2), :, pl.ds(0, DM)], sem_o.at[0, t])

    def cp_f(j, k, half):
        src, dst = ((wr_hbm, wr), (wi_hbm, wi))[j]
        return pltpu.make_async_copy(
            src.at[pl.ds(256 * half, 256), pl.ds(pl.multiple_of(128 * k, 128), 128)].bitcast(U32),
            dst.at[k, pl.ds(128 * half, 128)], sem_m.at[half])

    def wait_f(half):
        for dst in (wr, wi):
            part = dst.at[:, pl.ds(128 * half, 128)]
            pltpu.make_async_copy(part, part, sem_m.at[half]).wait()

    for c in range(2):
        cp_bx(c).start()
        cp_s(c).start()

    rt = float(np.sqrt(0.5))
    row8 = lax.broadcasted_iota(jnp.int32, (8, 128), 0)

    def b_forward(c, carry):
        @pl.when(c < 6)
        def _():
            cp_bx(c + 2).start()
            cp_s(c + 2).start()

        for j in range(2):
            cp_f(j, 2 * c, 0).start()
            cp_f(j, 2 * c + 1, 0).start()

        @pl.when(c == 7)
        def _():
            cp_ax(T - 1).start()
            cp_ax(T - 2).start()

        cp_bx(c).wait()
        cp_s(c).wait()
        w = xw[c].reshape(128, DM)
        for half, xf in enumerate((_lo(w), _hi(w))):
            x = [xf[:, 128 * al:128 * (al + 1)] for al in range(8)]
            s = [x[i] + x[i + 4] for i in range(4)]
            d = [x[i] - x[i + 4] for i in range(4)]
            e, o = s[0] + s[2], s[1] + s[3]
            p, q = (d[1] - d[3]) * rt, (d[1] + d[3]) * rt
            u = [(e + o, e - o), (d[0] + p, d[2] + q), (s[0] - s[2], s[1] - s[3]),
                 (d[0] - p, d[2] - q)]
            tt = [lax.dot_general(d_ref[k], jnp.concatenate(u[k], axis=1).astype(BF16), NT,
                                  preferred_element_type=F32) for k in range(4)]
            dc, ny = tt[0][0:8], tt[0][128:136]
            re = [jnp.where(row8 == 0, dc * 0.5, dc), tt[0][8:128]]
            im = [jnp.where(row8 == 0, 0.0, ny), tt[0][136:256]]
            for k in range(1, 4):
                re.append(tt[k][0:128])
                im.append(tt[k][128:256])
            re += [jnp.where(row8 == 0, ny * 0.5, 0.0), jnp.zeros((8, 128), F32)]
            im.append(jnp.zeros((16, 128), F32))
            lhs = jnp.concatenate([jnp.concatenate(re, axis=0), jnp.concatenate(im, axis=0)],
                                  axis=1).astype(BF16)
            a = 2 * c + half
            yb[a] = jnp.dot(lhs, sm[a], preferred_element_type=F32)
        return carry

    lax.fori_loop(0, 8, b_forward, 0)
    for k in range(16):
        cp_f(0, k, 1).start()
        cp_f(1, k, 1).start()
    wait_f(0)

    def filt(row, wre, wim):
        y = [(yb[a, pl.ds(row, 8), 0:128], yb[a, pl.ds(row, 8), 128:256]) for a in range(16)]
        z = _fft16(y, -1)
        z = [(z[k][0] * wre(k) - z[k][1] * wim(k), z[k][0] * wim(k) + z[k][1] * wre(k))
             for k in range(16)]
        return _fft16(z, 1)

    def b_filter(i, carry):
        mg, j = i // 4, i % 4

        @pl.when(i == 8)
        def _():
            wait_f(1)

        @pl.when(jnp.logical_and(i >= 8, i % 4 == 0))
        def _():
            start_w(1, i // 4 - 2)
            start_w(2, i // 4 - 2)

        for half, un in enumerate((_lo, _hi)):
            off = [ROW_OFF[2 * jj + half] for jj in range(4)]
            base = jnp.where(j < 2, jnp.where(j == 0, off[0], off[1]),
                             jnp.where(j == 2, off[2], off[3])) + 16 * mg
            base = pl.multiple_of(base, 16)
            res = []
            for r8 in range(2):
                sl = pl.ds(64 * mg + 32 * r8 + j, 8, stride=4)
                res.append(filt(pl.multiple_of(base + 8 * r8, 8),
                                lambda k: un(wr[k, sl, :]),
                                lambda k: un(wi[k, sl, :])))
            for a in range(16):
                for ri in range(2):
                    vb[a, pl.ds(base, 16), 128 * ri:128 * (ri + 1)] = jnp.concatenate(
                        [res[0][a][ri], res[1][a][ri]], axis=0).astype(BF16)
        return carry

    lax.fori_loop(0, 16, b_filter, 0)
    res = filt(512, lambda k: wrn_ref[0:1, 128 * k:128 * (k + 1)].astype(F32),
               lambda k: win_ref[0:1, 128 * k:128 * (k + 1)].astype(F32))
    for a in range(16):
        for ri in range(2):
            vb[a, 512:KROWS, 128 * ri:128 * (ri + 1)] = jnp.concatenate(
                [res[a][ri], jnp.zeros((8, 128), F32)], axis=0).astype(BF16)
        vb[a, KROWS:640, :] = jnp.zeros((640 - KROWS, 256), BF16)

    lane0 = lax.broadcasted_iota(jnp.int32, (128, 128), 1) == 0

    def prep_wo(g, c, r):
        w = [[wo[g, i, r:r + 8, 128 * (NB * c + j):128 * (NB * c + j + 1)]
              for j in range(NB)] for i in range(NB)]
        ev, od = [_right([[un(v) for v in row] for row in w]) for un in (_lo, _hi)]
        for n, (u, v) in enumerate(zip(ev[1] + ev[0], od[1] + od[0])):
            wox[g, 64 * n + r:64 * n + r + 8, 128 * c:128 * (c + 1)] = _words(u, v)

    def b_inverse(c, carry):
        @pl.when(c < NG - 2)
        def _():
            start_w(1, c + 2)
            start_w(2, c + 2)

        lhs = [[] for _ in range(4)]
        for half in range(2):
            a = 2 * c + half
            ny = lax.dot_general(sm[a, 0:128, :], vb[a, 512:640, :], NT,
                                 preferred_element_type=F32)
            z = lax.dot_general(sm[a], vb[a, 0:512, :], NT, preferred_element_type=F32)
            for k in range(4):
                zr, zi = z[0:128, 128 * k:128 * (k + 1)], z[128:256, 128 * k:128 * (k + 1)]
                if k == 0:
                    zi = jnp.where(lane0, ny, zi)
                lhs[k].append(jnp.concatenate([zr, zi], axis=1).astype(BF16))
        g = [jnp.dot(jnp.concatenate(lhs[k], axis=0), d_ref[k], preferred_element_type=F32)
             for k in range(4)]
        (g0, g4), (g1r, g1i), (g2r, g2i), (g3r, g3i) = [(v[:, :128], v[:, 128:]) for v in g]
        e, o = g0 + g4, g0 - g4
        s = [e + g2r, o + g2i, e - g2r, o - g2i]
        p, q = (g1r - g3r) * rt, (g1i - g3i) * rt
        d = [g1r + g3r, q + p, g1i + g3i, q - p]
        y = [s[i] + d[i] for i in range(4)] + [s[i] - d[i] for i in range(4)]
        for al in range(8):
            bits = _bf16_bits(y[al])
            xw[c, :, :, 128 * al:128 * (al + 1)] = (
                (bits[0:128] >> 16) | bits[128:256]).reshape(8, 16, 128)
        return carry

    lax.fori_loop(0, 8, b_inverse, 0)

    def blocks(v):
        n = v.shape[1] // (128 * NB)
        return [jnp.concatenate([v[:, 128 * (NB * c + i):128 * (NB * c + i + 1)]
                                 for c in range(n)], axis=1) for i in range(NB)]

    def x_pieces(t):
        def piece(g, c):
            cols = slice(128 * NB * c, 128 * NB * (c + 1))
            top, bot = ax[t, g, :, cols], ax[t, g + G // 2, :, cols]
            ev, od = [_left(blocks(un(top)), blocks(un(bot))) for un in (_lo, _hi)]
            for n in range(NL):
                hs[n, SEG // 2 * g:SEG // 2 * (g + 1), 128 * c:128 * (c + 1)] = _words(ev[n], od[n])

        return [functools.partial(piece, g, c) for g in range(G // 2) for c in range(NI)]

    def load_x(t):
        for fn in x_pieces(t):
            fn()

    def set_mem(m):
        for n, v in enumerate(_left(blocks(m[0:MH]), blocks(m[MH:2 * MH]))):
            hs[n, XH // 2:HH // 2, :] = pltpu.bitcast(v.astype(BF16), U32)

    def wait_w(j, g):
        for a in range(NB // 2):
            cp_w(j, g, a).wait()

    def prep_w(j, g):
        ref = wblk[j]

        def raw(c, i, r, n):
            w = [[ref[g, c, i, pl.ds(128 * a + 2 * r + d, n, stride=2), :]
                  for a in range(NB // 2)] for d in range(2)]
            return [[un(v) for v in w[d] for un in (_lo, _hi)] for d in range(2)]

        for c in range(NI):
            for r in range(0, 64, 8):
                b = [raw(c, i, r, 8) for i in range(NB)]
                ev, od = [_right([b[i][d] for i in range(NB)])[1] for d in range(2)]
                for n in range(NX):
                    wext[j][g, c, 64 * n + r:64 * n + r + 8, :] = _words(ev[n], od[n])
        for c in range(NI):
            for i in range(NB):
                ev, od = raw(c, i, 0, 64)
                for v in (ev, od):
                    v[i] = functools.reduce(lambda p, q: p + q, v)
                for e in range(NB):
                    ref[g, c, i, 64 * e:64 * (e + 1), :] = _words(ev[e], od[e])

    def right(blk, ext, b):
        w = ext(64 * b) if isinstance(b, int) else blk(*b)
        w = pltpu.bitcast(w, BF16)
        return w.reshape(w.shape[0] * 128, 128)

    def spread(extra):
        at = {NL * n // len(extra): fn for n, fn in enumerate(extra)}
        return lambda a: at[a]() if a in at else None

    def project(g, rows, extra=()):
        hook = spread(extra)

        def mm(a, b):
            hook(a)
            return jnp.concatenate([
                jnp.dot(pltpu.bitcast(hs[a, r0 // 2:r1 // 2, :], BF16),
                        right(lambda i, e: wblk[j][g, :, i, 64 * e:64 * (e + 1), :],
                              lambda o: wext[j][g, :, o:o + 64, :], b),
                        preferred_element_type=F32) for j, (r0, r1) in rows.items()], axis=0)

        res, out, r = _combine(mm), {}, 0
        for j, (r0, r1) in rows.items():
            out[j] = [[v[r:r + r1 - r0] for v in half] for half in res]
            r += r1 - r0
        return out

    def put_o(g, r0, o):
        for n, v in enumerate(_left([h[0] for h in o], [h[1] for h in o])):
            ob[n, g, r0:HH, :] = v.astype(BF16)

    def put_o_pieces(g, r0):
        def own(i):
            x, y = of[i, 0, r0:HH, :], of[i, 1, r0:HH, :]
            ob[i, g, r0:HH, :] = (x + KS[i] * y).astype(BF16)
            ob[NB + i, g, r0:HH, :] = y.astype(BF16)

        def cross(n, i, j):
            yi = of[i, 1, r0:HH, :]
            sx, sy = of[i, 0, r0:HH, :] + of[j, 0, r0:HH, :], yi + of[j, 1, r0:HH, :]
            p2, d = sx + KS[j] * sy, KS[j] - KS[i]
            for m, v in enumerate((p2 - (yi if d == 1.0 else d * yi), p2, sx + KS[i] * sy)):
                ob[2 * NB + 3 * n + m, g, r0:HH, :] = v.astype(BF16)

        return ([functools.partial(own, i) for i in range(NB)]
                + [functools.partial(cross, n, i, j) for n, (i, j) in enumerate(PAIRS)])

    def lanes(k, n=1):
        return pl.ds(pl.multiple_of(128 * k, 128), 128 * n)

    def out_mm(c, r0, a, b, g0, g1):
        o = jnp.concatenate([ob[a, g, r0:HH, :] for g in range(g0, g1)], axis=1)
        if not isinstance(b, int) and b[0] == b[1]:
            b = NX + b[0]
        w = right(lambda i, e: wo[g0:g1, i, :, lanes(NB * c + e)],
                  lambda o: wox[g0:g1, o:o + 64, lanes(c)], b)
        return jnp.dot(o, w, preferred_element_type=F32)

    def out_mem(c, r0, keep, feed, early=(), extra=()):
        hook = spread(extra)

        def mm(a, b):
            hook(a)
            if a in early:
                return early[a] + out_mm(c, r0, a, b, NG - 1, NG)
            return out_mm(c, r0, a, b, 0, NG)

        top, bot = _combine(mm)
        x0 = XH - r0
        if keep:
            mend[0:MH, lanes(NB * c, NB)] = jnp.concatenate([v[x0:] for v in top], axis=1)
            mend[MH:2 * MH, lanes(NB * c, NB)] = jnp.concatenate([v[x0:] for v in bot], axis=1)
        if feed:
            for n, v in enumerate(_left([v[x0:] for v in top], [v[x0:] for v in bot])):
                hs[n, XH // 2:HH // 2, lanes(c)] = pltpu.bitcast(v.astype(BF16), U32)
        return [[v[:x0] for v in half] for half in (top, bot)]

    cp_ax(T - 1).wait()
    load_x(T - 1)

    def kv_loop(g, carry):
        @pl.when(g < NG // 2)
        def _():
            cp_wo(2 * g).start()
            cp_wo(2 * g + 1).start()

        @pl.when(g >= NG // 2)
        def _():
            start_w(0, 2 * g - NG)
            start_w(0, 2 * g - NG + 1)

        for j, ret in ((1, kret), (2, vret)):
            wait_w(j, g)
        for j, ret in ((1, kret), (2, vret)):
            prep_w(j, g)
            top, bot = project(g, {j: (0, XH)})[j]
            for e in range(NB):
                ret[NB * g + e] = jnp.concatenate([top[e], bot[e]], axis=0).astype(BF16)
        return carry

    lax.fori_loop(0, NG, kv_loop, 0)

    cp_ax(T - 2).wait()
    xbar = jnp.sum(_lo(ax[T - 2]) + _hi(ax[T - 2]), axis=1, keepdims=True) * (1.0 / (SEG + MEM))
    set_mem(jnp.broadcast_to(xbar, (G, MEM, DM)).reshape(G * MEM, DM))

    def guess(g, carry):
        cp_wo(g).wait()
        side = [functools.partial(prep_wo, g, c, r) for c in range(NI) for r in range(0, 64, 8)]
        put_o(g, XH, list(zip(*project(g, {2: (XH, HH)}, side)[2])))
        return carry

    lax.fori_loop(0, NG, guess, 0)
    lax.fori_loop(0, NI, lambda c, carry: (out_mem(c, XH, False, True), carry)[1], 0)

    TILES = ((0, 1, 2), (3, 4, 5), (6, 7))
    nx = [SEG * len(tl) for tl in TILES]
    nm = (32, 32, 16)

    def tile(v, g, with_x):
        m0 = XH if with_x else 0
        parts = [v[ch // 4][SEG * (ch % 4):SEG * (ch % 4 + 1)] for ch in TILES[g]] if with_x else []
        parts += [v[ch // 4][m0 + MEM * (ch % 4):m0 + MEM * (ch % 4 + 1)] for ch in TILES[g]]
        if len(TILES[g]) == 3:
            parts.append(jnp.zeros((MEM, DH), F32))
        return jnp.concatenate(parts, axis=0).astype(BF16)

    def step(mode):
        q_x, kv_x = mode != "pred", mode == "mid"
        q0, kv0 = (0 if q_x else XH), (0 if kv_x else XH)

        def put(ref, e, v, with_x):
            for g in range(3):
                ref[e, g, (0 if with_x else nx[g]):nx[g] + nm[g], :] = tile(v, g, with_x)

        def proj(hg, mats, extra=()):
            res = project(hg, {j: (kv0 if j else q0, HH) for j in mats}, extra)
            for j in mats:
                for e in range(NB):
                    v = [half[e] if j else half[e] * QSCALE for half in res[j]]
                    put((qt, kt, vt)[j], e, v, kv_x if j else q_x)

        def get(ref, ret, hg, e, g):
            if kv_x:
                return ref[e, g]
            return jnp.concatenate(
                [ret[NB * hg + e, 96 * g:96 * g + nx[g], :], ref[e, g, nx[g]:128, :]], axis=0)

        def scores(hg, e):
            out = []
            for g in range(3):
                r0 = 0 if q_x else nx[g]
                s = lax.dot_general(qt[e, g, r0:nx[g] + nm[g], :], get(kt, kret, hg, e, g), NT,
                                    preferred_element_type=F32)
                fill = mask_ref[g // 2, r0:nx[g] + nm[g], :]
                s = jnp.where(fill == 0.0, s, fill)
                pr = jnp.exp2(s - jnp.max(s, axis=1, keepdims=True))
                out.append((pr.astype(BF16), jnp.sum(pr, axis=1, keepdims=True)))
            return out

        def values(hg, e, sc):
            xs, ms = [], []
            for g in range(3):
                pr, den = sc[g]
                inv = pl.reciprocal(den, approx=True)
                inv = inv * (2.0 - den * inv)
                o = jnp.dot(pr, get(vt, vret, hg, e, g), preferred_element_type=F32) * inv
                m0 = nx[g] if q_x else 0
                for i in range(len(TILES[g])):
                    if q_x:
                        xs.append(o[SEG * i:SEG * (i + 1)])
                    ms.append(o[m0 + MEM * i:m0 + MEM * (i + 1)])
            return [jnp.concatenate(xs[4 * k:4 * k + 4] + ms[4 * k:4 * k + 4], axis=0)
                    for k in range(2)]

        def group(hg, fill=None):
            sc = [scores(hg, e) for e in range(NB)]
            if fill is not None:
                fill()
                put_o(hg, q0, [values(hg, e, sc[e]) for e in range(NB)])
                return

            def park(e):
                for k, v in enumerate(values(hg, e, sc[e])):
                    of[e, k, q0:HH, :] = v

            parks = [functools.partial(park, e) for e in range(NB)]
            if mode == "mid":
                proj(hg + 1, [0, 1, 2], [lambda: None] * 4 + parks + put_o_pieces(hg, q0))
            elif mode == "last":
                proj(hg + 1, [0], [lambda: None] * 2 + parks)
                proj(hg + 1, [1, 2], put_o_pieces(hg, q0))
            else:
                proj(hg + 1, [1, 2, 0], [lambda: None] * 4 + parks + put_o_pieces(hg, q0))

        def first():
            for mats in ([[0, 1, 2]] if mode == "mid" else [[1, 2, 0]]):
                proj(0, mats)

        return first, group

    kt[:, 2, 80:128, :] = jnp.zeros((NB, 48, DH), BF16)
    vt[:, 2, 80:128, :] = jnp.zeros((NB, 48, DH), BF16)

    first, group = step("pred")
    for t in range(T - 2):
        cp_ax(t).start()
    wait_w(0, 0)
    prep_w(0, 0)
    first()

    def pred_loop(hg, carry):
        wait_w(0, hg + 1)
        prep_w(0, hg + 1)
        group(hg)
        return carry

    lax.fori_loop(0, NG - 1, pred_loop, 0)
    group(NG - 1, lambda: None)
    lax.fori_loop(0, NI, lambda c, carry: (out_mem(c, XH, True, False), carry)[1], 0)
    for t in range(T - 2):
        cp_ax(t).wait()
    for c in range(8):
        cp_by(c).start()
    load_x(0)

    first, group = step("mid")
    group_last = step("last")[1]

    def segment(t, carry):
        first()

        @pl.when(t < T - 1)
        def _():
            lax.fori_loop(0, NG - 1, lambda hg, c: (group(hg), c)[1], 0)

        @pl.when(t == T - 1)
        def _():
            lax.fori_loop(0, NG - 1, lambda hg, c: (group_last(hg), c)[1], 0)
            for e in range(NB):
                for g in range(3):
                    kt[e, g, 0:nx[g], :] = kret[NH - NB + e, 96 * g:96 * g + nx[g], :]
                    vt[e, g, 0:nx[g], :] = vret[NH - NB + e, 96 * g:96 * g + nx[g], :]

        nxt = x_pieces((t + 1) % T)
        per = len(nxt) // NI
        early = {}
        group(NG - 1, lambda: early.update({i: out_mm(0, 0, i, i, 0, NG - 1) for i in range(3)}))
        for c in range(NI):
            for k, half in enumerate(out_mem(c, 0, True, True, early if c == 0 else {},
                                             nxt[per * c:per * (c + 1)])):
                for e, v in enumerate(half):
                    ostage[t, 4 * k:4 * k + 4, :, :, 128 * (NB * c + e):128 * (NB * c + e + 1)] = (
                        v.astype(BF16).reshape(G // 2, 2, 16, 128))
        cp_ao(t).start()
        return carry

    def one_pass(carry):
        it, _ = carry
        start = mend[0:(G - 1) * MEM, :]
        mstart[...] = start
        set_mem(jnp.concatenate([mem0_ref[...].astype(F32), start], axis=0))
        lax.fori_loop(0, T, segment, 0)
        real = mend[0:(G - 1) * MEM, :]
        lim = jnp.max(jnp.abs(real), axis=1, keepdims=True) * TOL
        good = jnp.abs(real - mstart[...]) <= lim
        bad = jnp.max(jnp.where(good, 0.0, 1.0))
        for t in range(T):
            cp_ao(t).wait()
        return it + 1, bad

    lax.while_loop(lambda c: jnp.logical_and(c[0] < G, c[1] > 0.0), one_pass,
                   (jnp.int32(0), jnp.float32(1.0)))
    for c in range(8):
        cp_by(c).wait()


@functools.partial(jax.jit, static_argnames=("A_seg_len",))
def pallas_concat_heads__memory_aug_recurrent_mem_tr__spectral_gfnet__prompt_kernel(
    A_x, A_mem0, A_Wq, A_Wk, A_Wv, A_Wo, A_seg_len, B_x, B_w_r, B_w_i,
):
    assert A_seg_len == SEG and A_x.shape == (1, G * T * SEG, DM) and A_Wq.shape == (DM, NH, DH)
    assert A_mem0.shape == (1, MEM, DM) and B_x.shape == (1, 2048, 1024)
    dmat, smat, mask = _constants()
    wr_t, wi_t = B_w_r.T, B_w_i.T
    hbm = pl.BlockSpec(memory_space=pl.ANY)
    nyq = pl.BlockSpec((16, 2048), lambda i: (32, 0))

    def full(shape):
        return pl.BlockSpec(shape, lambda i: (0,) * len(shape))

    out = pl.pallas_call(
        _kernel,
        grid=(1,),
        in_specs=[hbm] * 9 + [full((MEM, DM)), nyq, nyq, full(dmat.shape), full(mask.shape)],
        out_specs=hbm,
        out_shape=jax.ShapeDtypeStruct((G, 16, 16, 2 * DM), BF16),
        scratch_shapes=[
            pltpu.VMEM((T, G, SEG // 2, DM), U32),
            *[pltpu.VMEM((NG, NI, NB, NB * 64, DH), U32)] * 3,
            *[pltpu.VMEM((NG, NI, NX * 64, DH), U32)] * 3,
            pltpu.VMEM((NG, NB, 64, DM), U32),
            pltpu.VMEM((NG, (NX + NB) * 64, NI * 128), U32),
            pltpu.VMEM((8, 8, 16, 1024), U32),
            pltpu.VMEM((16, 256, 128), U32),
            pltpu.VMEM((16, 256, 128), U32),
            pltpu.VMEM((16, 256, 256), BF16),
            pltpu.VMEM((16, KROWS, 256), F32),
            pltpu.VMEM((16, 640, 256), BF16),
            pltpu.VMEM((NH, G * SEG, DH), BF16),
            pltpu.VMEM((NH, G * SEG, DH), BF16),
            pltpu.VMEM((NL, HH // 2, NI * 128), U32),
            pltpu.VMEM((NB, 3, 128, DH), BF16),
            pltpu.VMEM((NB, 3, 128, DH), BF16),
            pltpu.VMEM((NB, 3, 128, DH), BF16),
            pltpu.VMEM((NL, NG, HH, DH), BF16),
            pltpu.VMEM((NB, 2, HH, DH), F32),
            pltpu.VMEM(((G - 1) * MEM, DM), F32),
            pltpu.VMEM((G * MEM, DM), F32),
            pltpu.VMEM((T, G, 2, 16, DM), BF16),
            pltpu.SemaphoreType.DMA((3, 8)),
            pltpu.SemaphoreType.DMA((4, NB // 2, NG)),
            pltpu.SemaphoreType.DMA((2,)),
            pltpu.SemaphoreType.DMA((2, T)),
        ],
        compiler_params=pltpu.CompilerParams(
            dimension_semantics=("arbitrary",), vmem_limit_bytes=120 * 1024 * 1024),
    )(
        A_x.reshape(G, T, SEG, DM),
        *[w.reshape(NI, NB, 128, NH, DH) for w in (A_Wq, A_Wk, A_Wv)],
        A_Wo.reshape(NG, NB, DH, DM), B_x.reshape(8, 16, 16, 1024), wr_t, wi_t, smat,
        A_mem0.reshape(MEM, DM), wr_t, wi_t, dmat, mask,
    )
    return out.reshape(1, 2048, 2 * DM)
```

```python
import functools

import jax
import jax.numpy as jnp
import numpy as np
from jax import lax
from jax.experimental import pallas as pl
from jax.experimental.pallas import tpu as pltpu

F32 = jnp.float32
BF16 = jnp.bfloat16
U32 = jnp.uint32

G = 8
T = 8
SEG = 32
MEM = 8
DM = 1024
NH = 32
DH = 128
KS = (-4.0 / 3, -1.0 / 3, 1.0 / 3, 4.0 / 3)
NB = len(KS)
PAIRS = [(i, j) for i in range(NB) for j in range(i + 1, NB)]
NL = 2 * NB + 3 * len(PAIRS)
NX = NB + len(PAIRS)
NG = NH // NB
NI = DM // 128 // NB
XH = G // 2 * SEG
MH = G // 2 * MEM
HH = XH + MH
LOG2E = 1.4426950408889634
QSCALE = float(DH ** -0.5 * LOG2E)
MASKED = float(-1e9 * LOG2E)
TOL = 2.0 ** -9
NT = (((1,), (1,)), ((), ()))
KROWS = 528
ROW_OFF = {0: 0, 4: 64, 1: 128, 7: 192, 2: 256, 6: 320, 3: 384, 5: 448}


def _constants():
    beta = np.arange(128)[None, :]
    m = np.arange(64)[:, None]
    d = np.zeros((4, 256, 256))
    for blk, r in enumerate((0, 4)):
        th = 2 * np.pi * (8 * m + r) * beta / 1024
        d[0, 64 * blk:64 * blk + 64, 128 * blk:128 * blk + 128] = np.cos(th)
        d[0, 128 + 64 * blk:192 + 64 * blk, 128 * blk:128 * blk + 128] = -np.sin(th)
    d[0, 128, 0:128] = np.cos(np.pi * np.arange(128))
    for r, sg in ((1, -1.0), (2, -1.0), (3, 1.0)):
        for blk, (res, cj) in enumerate(((r, 1.0), (8 - r, -1.0))):
            th = 2 * np.pi * (8 * m + res) * beta / 1024
            re, im = slice(64 * blk, 64 * blk + 64), slice(128 + 64 * blk, 192 + 64 * blk)
            d[r, re, 0:128] = np.cos(th)
            d[r, im, 0:128] = -np.sin(th)
            d[r, re, 128:256] = sg * cj * np.sin(th)
            d[r, im, 128:256] = sg * cj * np.cos(th)
    d *= 2.0 ** -10
    b = np.arange(128)[:, None]
    kb = np.arange(128)[None, :]
    s = np.zeros((16, 256, 256))
    for a in range(16):
        th = 2 * np.pi * ((kb * (16 * b + a)) % 2048) / 2048
        s[a, :128, :128] = np.cos(th)
        s[a, 128:, :128] = np.sin(th)
        s[a, :128, 128:] = -np.sin(th)
        s[a, 128:, 128:] = np.cos(th)
    mask = np.zeros((2, 128, 128), np.float32)
    for i, ns in enumerate((3, 2)):
        idx = np.arange(128)
        isx = idx < SEG * ns
        pad = idx >= (SEG + MEM) * ns
        seg = np.where(isx, idx // SEG, (idx - SEG * ns) // MEM)
        same = (seg[:, None] == seg[None, :]) & ~pad[None, :]
        future = isx[:, None] & isx[None, :] & (idx[None, :] > idx[:, None])
        mk = np.where(same, np.where(future, MASKED, 0.0), -np.inf)
        mask[i] = np.where(pad[:, None], 0.0, mk)
    return d.astype(BF16), s.astype(BF16), mask


def _lo(w):
    return lax.bitcast_convert_type(w << 16, F32)


def _hi(w):
    return lax.bitcast_convert_type(w & np.uint32(0xFFFF0000), F32)


def _bf16_bits(y):
    return lax.bitcast_convert_type(y.astype(BF16).astype(F32), U32)


def _r4(x, sg):
    (ar, ai), (br, bi), (cr, ci), (dr, di) = x
    s0r, s0i, d0r, d0i = ar + cr, ai + ci, ar - cr, ai - ci
    s1r, s1i, d1r, d1i = br + dr, bi + di, br - dr, bi - di
    p = (d0r - d1i, d0i + d1r)
    q = (d0r + d1i, d0i - d1r)
    y1, y3 = (p, q) if sg > 0 else (q, p)
    return [(s0r + s1r, s0i + s1i), y1, (s0r - s1r, s0i - s1i), y3]


def _tw(z, e, sg):
    r, i = z
    if e == 0:
        return z
    if e == 4:
        return (-i, r) if sg > 0 else (i, -r)
    h = float(np.sqrt(0.5))
    if e == 2:
        return ((r - i) * h, (r + i) * h) if sg > 0 else ((r + i) * h, (i - r) * h)
    if e == 6:
        return ((r + i) * -h, (r - i) * h) if sg > 0 else ((i - r) * h, (r + i) * -h)
    c = float(np.cos(2 * np.pi * e / 16))
    s = float(sg * np.sin(2 * np.pi * e / 16))
    return (r * c - i * s, r * s + i * c)


def _fft16(x, sg):
    t = [_r4([x[4 * a1 + a0] for a1 in range(4)], sg) for a0 in range(4)]
    out = [None] * 16
    for k0 in range(4):
        u = _r4([_tw(t[a0][k0], a0 * k0, sg) for a0 in range(4)], sg)
        for k1 in range(4):
            out[k0 + 4 * k1] = u[k1]
    return out


def _words(even, odd):
    return pltpu.pack_elementwise([even, odd], packed_dtype=BF16)


def _left(x, y):
    z = [x[i] + KS[i] * y[i] for i in range(NB)]
    out = z + list(y)
    for i, j in PAIRS:
        sx, sy = x[i] + x[j], y[i] + y[j]
        out += [z[i] + z[j], sx + KS[j] * sy, sx + KS[i] * sy]
    return out


def _right(b):
    rows = [functools.reduce(lambda u, v: u + v, b[i]) for i in range(NB)]
    extra = [functools.reduce(lambda u, v: u - v, [b[j][i] for j in range(NB) if j != i], b[i][i])
             for i in range(NB)]
    extra += [(b[i][j] + b[j][i]) * (1.0 / (KS[j] - KS[i])) for i, j in PAIRS]
    return rows, extra


def _combine(mm):
    s = [mm(i, i) for i in range(NB)]
    r = [mm(NB + i, (i, i)) for i in range(NB)]
    for n, (i, j) in enumerate(PAIRS):
        p1 = mm(2 * NB + 3 * n, NB + n)
        p2 = mm(2 * NB + 3 * n + 1, (i, j))
        p3 = mm(2 * NB + 3 * n + 2, (j, i))
        d = 1.0 / (KS[j] - KS[i])
        e = (p2 + p3 if d == 1.0 else (p2 + p3) * d) - p1
        r[j], r[i], s[j], s[i] = r[j] + e, r[i] - e, s[j] + p2, s[i] + p3
    return [s[i] - KS[i] * r[i] for i in range(NB)], r


def _kernel(ax_hbm, wq_hbm, wk_hbm, wv_hbm, wo_hbm, bx_hbm, wr_hbm, wi_hbm, s_hbm,
            mem0_ref, wrn_ref, win_ref, d_ref, mask_ref,
            out_hbm,
            ax, wq, wk, wv, wqx, wkx, wvx, wo, wox, xw, wr, wi, sm, yb, vb, kret, vret, hs,
            qt, kt, vt, ob, of, mstart, mend, ostage, sem_b, sem_w, sem_m, sem_o):
    wblk, wext = (wq, wk, wv), (wqx, wkx, wvx)

    def cp_bx(c):
        return pltpu.make_async_copy(bx_hbm.bitcast(U32).at[:, :, c, :], xw.at[c], sem_b.at[0, c])

    def cp_s(c):
        sl = pl.ds(2 * c, 2)
        return pltpu.make_async_copy(s_hbm.at[sl], sm.at[sl], sem_b.at[1, c])

    def cp_by(c):
        return pltpu.make_async_copy(
            xw.at[c], out_hbm.bitcast(U32).at[:, :, c, pl.ds(DM, DM)], sem_b.at[2, c])

    def cp_w(j, g, a):
        src = (wq_hbm, wk_hbm, wv_hbm)[j].bitcast(U32).at[:, :, :, NB // 2 * g + a, :]
        return pltpu.make_async_copy(src, wblk[j].at[g, :, :, pl.ds(128 * a, 128), :],
                                     sem_w.at[j, a, g])

    def start_w(j, g):
        for a in range(NB // 2):
            cp_w(j, g, a).start()

    def cp_wo(g):
        return pltpu.make_async_copy(wo_hbm.bitcast(U32).at[g], wo.at[g], sem_w.at[3, 0, g])

    def cp_ax(t):
        return pltpu.make_async_copy(ax_hbm.bitcast(U32).at[:, t], ax.at[t], sem_o.at[1, t])

    def cp_ao(t):
        return pltpu.make_async_copy(
            ostage.at[t], out_hbm.at[:, pl.ds(2 * t, 2), :, pl.ds(0, DM)], sem_o.at[0, t])

    def cp_f(j, k, half):
        src, dst = ((wr_hbm, wr), (wi_hbm, wi))[j]
        return pltpu.make_async_copy(
            src.at[pl.ds(256 * half, 256), pl.ds(pl.multiple_of(128 * k, 128), 128)].bitcast(U32),
            dst.at[k, pl.ds(128 * half, 128)], sem_m.at[j, half])

    def wait_f(half):
        for j, dst in enumerate((wr, wi)):
            part = dst.at[:, pl.ds(128 * half, 128)]
            pltpu.make_async_copy(part, part, sem_m.at[j, half]).wait()

    for c in range(2):
        cp_bx(c).start()
        cp_s(c).start()

    kt[:, 2, 80:128, :] = jnp.zeros((NB, 48, DH), BF16)
    vt[:, 2, 80:128, :] = jnp.zeros((NB, 48, DH), BF16)

    vb[:, KROWS:640, :] = jnp.zeros((16, 640 - KROWS, 256), BF16)

    rt = float(np.sqrt(0.5))
    row8 = lax.broadcasted_iota(jnp.int32, (8, 128), 0)

    def b_forward(c, carry):
        @pl.when(c < 6)
        def _():
            cp_bx(c + 2).start()
            cp_s(c + 2).start()

        for j in range(2):
            cp_f(j, 2 * c, 0).start()
            cp_f(j, 2 * c + 1, 0).start()

        @pl.when(c == 7)
        def _():
            cp_ax(T - 1).start()
            cp_ax(T - 2).start()

        cp_bx(c).wait()
        cp_s(c).wait()
        w = xw[c].reshape(128, DM)
        for half, xf in enumerate((_lo(w), _hi(w))):
            x = [xf[:, 128 * al:128 * (al + 1)] for al in range(8)]
            s = [x[i] + x[i + 4] for i in range(4)]
            d = [x[i] - x[i + 4] for i in range(4)]
            e, o = s[0] + s[2], s[1] + s[3]
            p, q = (d[1] - d[3]) * rt, (d[1] + d[3]) * rt
            u = [(e + o, e - o), (d[0] + p, d[2] + q), (s[0] - s[2], s[1] - s[3]),
                 (d[0] - p, d[2] - q)]
            tt = [lax.dot_general(d_ref[k], jnp.concatenate(u[k], axis=1).astype(BF16), NT,
                                  preferred_element_type=F32) for k in range(4)]
            dc, ny = tt[0][0:8], tt[0][128:136]
            re = [jnp.where(row8 == 0, dc * 0.5, dc), tt[0][8:128]]
            im = [jnp.where(row8 == 0, 0.0, ny), tt[0][136:256]]
            for k in range(1, 4):
                re.append(tt[k][0:128])
                im.append(tt[k][128:256])
            re += [jnp.where(row8 == 0, ny * 0.5, 0.0), jnp.zeros((8, 128), F32)]
            im.append(jnp.zeros((16, 128), F32))
            lhs = jnp.concatenate([jnp.concatenate(re, axis=0), jnp.concatenate(im, axis=0)],
                                  axis=1).astype(BF16)
            a = 2 * c + half
            yb[a] = jnp.dot(lhs, sm[a], preferred_element_type=F32)
        return carry

    lax.fori_loop(0, 8, b_forward, 0)
    for k in range(16):
        cp_f(0, k, 1).start()
        cp_f(1, k, 1).start()
    wait_f(0)

    def filt(row, wre, wim):
        y = [(yb[a, pl.ds(row, 8), 0:128], yb[a, pl.ds(row, 8), 128:256]) for a in range(16)]
        z = _fft16(y, -1)
        z = [(z[k][0] * wre(k) - z[k][1] * wim(k), z[k][0] * wim(k) + z[k][1] * wre(k))
             for k in range(16)]
        return _fft16(z, 1)

    def b_filter(i, carry):
        mg, j = i // 4, i % 4

        @pl.when(i == 8)
        def _():
            wait_f(1)

        @pl.when(jnp.logical_and(i >= 8, i % 4 == 0))
        def _():
            start_w(1, i // 4 - 2)
            start_w(2, i // 4 - 2)

        for half, un in enumerate((_lo, _hi)):
            off = [ROW_OFF[2 * jj + half] for jj in range(4)]
            base = jnp.where(j < 2, jnp.where(j == 0, off[0], off[1]),
                             jnp.where(j == 2, off[2], off[3])) + 16 * mg
            base = pl.multiple_of(base, 16)
            for r8 in range(2):
                sl = pl.ds(64 * mg + 32 * r8 + j, 8, stride=4)
                row = pl.multiple_of(base + 8 * r8, 8)
                res = filt(row, lambda k: un(wr[k, sl, :]), lambda k: un(wi[k, sl, :]))
                for a in range(16):
                    for ri in range(2):
                        vb[a, pl.ds(row, 8), 128 * ri:128 * (ri + 1)] = res[a][ri].astype(BF16)
        return carry

    lax.fori_loop(0, 16, b_filter, 0)
    res = filt(512, lambda k: wrn_ref[0:1, 128 * k:128 * (k + 1)].astype(F32),
               lambda k: win_ref[0:1, 128 * k:128 * (k + 1)].astype(F32))
    for a in range(16):
        for ri in range(2):
            vb[a, 512:KROWS, 128 * ri:128 * (ri + 1)] = jnp.concatenate(
                [res[a][ri], jnp.zeros((8, 128), F32)], axis=0).astype(BF16)

    lane0 = lax.broadcasted_iota(jnp.int32, (128, 128), 1) == 0

    def prep_wo(g, c, r):
        w = [[wo[g, i, r:r + 8, 128 * (NB * c + j):128 * (NB * c + j + 1)]
              for j in range(NB)] for i in range(NB)]
        ev, od = [_right([[un(v) for v in row] for row in w]) for un in (_lo, _hi)]
        for n, (u, v) in enumerate(zip(ev[1] + ev[0], od[1] + od[0])):
            wox[g, 64 * n + r:64 * n + r + 8, 128 * c:128 * (c + 1)] = _words(u, v)

    def b_inverse(c, carry):
        @pl.when(c < NG - 2)
        def _():
            start_w(1, c + 2)
            start_w(2, c + 2)

        lhs = [[] for _ in range(4)]
        for half in range(2):
            a = 2 * c + half
            ny = lax.dot_general(sm[a, 0:128, :], vb[a, 512:640, :], NT,
                                 preferred_element_type=F32)
            z = lax.dot_general(sm[a], vb[a, 0:512, :], NT, preferred_element_type=F32)
            for k in range(4):
                zr, zi = z[0:128, 128 * k:128 * (k + 1)], z[128:256, 128 * k:128 * (k + 1)]
                if k == 0:
                    zi = jnp.where(lane0, ny, zi)
                lhs[k].append(jnp.concatenate([zr, zi], axis=1).astype(BF16))
        g = [jnp.dot(jnp.concatenate(lhs[k], axis=0), d_ref[k], preferred_element_type=F32)
             for k in range(4)]
        (g0, g4), (g1r, g1i), (g2r, g2i), (g3r, g3i) = [(v[:, :128], v[:, 128:]) for v in g]
        e, o = g0 + g4, g0 - g4
        s = [e + g2r, o + g2i, e - g2r, o - g2i]
        p, q = (g1r - g3r) * rt, (g1i - g3i) * rt
        d = [g1r + g3r, q + p, g1i + g3i, q - p]
        y = [s[i] + d[i] for i in range(4)] + [s[i] - d[i] for i in range(4)]
        for al in range(8):
            bits = _bf16_bits(y[al])
            xw[c, :, :, 128 * al:128 * (al + 1)] = (
                (bits[0:128] >> 16) | bits[128:256]).reshape(8, 16, 128)
        return carry

    lax.fori_loop(0, 8, b_inverse, 0)

    def blocks(v):
        n = v.shape[1] // (128 * NB)
        return [jnp.concatenate([v[:, 128 * (NB * c + i):128 * (NB * c + i + 1)]
                                 for c in range(n)], axis=1) for i in range(NB)]

    def x_pieces(t):
        def piece(g, c):
            cols = slice(128 * NB * c, 128 * NB * (c + 1))
            top, bot = ax[t, g, :, cols], ax[t, g + G // 2, :, cols]
            ev, od = [_left(blocks(un(top)), blocks(un(bot))) for un in (_lo, _hi)]
            for n in range(NL):
                hs[n, SEG // 2 * g:SEG // 2 * (g + 1), 128 * c:128 * (c + 1)] = _words(ev[n], od[n])

        return [functools.partial(piece, g, c) for g in range(G // 2) for c in range(NI)]

    def load_x(t):
        for fn in x_pieces(t):
            fn()

    def set_mem(m):
        for n, v in enumerate(_left(blocks(m[0:MH]), blocks(m[MH:2 * MH]))):
            hs[n, XH // 2:HH // 2, :] = pltpu.bitcast(v.astype(BF16), U32)

    def wait_w(j, g):
        for a in range(NB // 2):
            cp_w(j, g, a).wait()

    def prep_w(j, g):
        ref = wblk[j]

        def raw(c, i, r, n):
            w = [[ref[g, c, i, pl.ds(128 * a + 2 * r + d, n, stride=2), :]
                  for a in range(NB // 2)] for d in range(2)]
            return [[un(v) for v in w[d] for un in (_lo, _hi)] for d in range(2)]

        for c in range(NI):
            for r in range(0, 64, 8):
                b = [raw(c, i, r, 8) for i in range(NB)]
                ev, od = [_right([b[i][d] for i in range(NB)])[1] for d in range(2)]
                for n in range(NX):
                    wext[j][g, c, 64 * n + r:64 * n + r + 8, :] = _words(ev[n], od[n])
        for c in range(NI):
            for i in range(NB):
                ev, od = raw(c, i, 0, 64)
                for v in (ev, od):
                    v[i] = functools.reduce(lambda p, q: p + q, v)
                for e in range(NB):
                    ref[g, c, i, 64 * e:64 * (e + 1), :] = _words(ev[e], od[e])

    def right(blk, ext, b):
        w = ext(64 * b) if isinstance(b, int) else blk(*b)
        w = pltpu.bitcast(w, BF16)
        return w.reshape(w.shape[0] * 128, 128)

    def spread(extra):
        at = {NL * n // len(extra): fn for n, fn in enumerate(extra)}
        return lambda a: at[a]() if a in at else None

    def project(g, rows, extra=()):
        hook = spread(extra)

        def mm(a, b):
            hook(a)
            return jnp.concatenate([
                jnp.dot(pltpu.bitcast(hs[a, r0 // 2:r1 // 2, :], BF16),
                        right(lambda i, e: wblk[j][g, :, i, 64 * e:64 * (e + 1), :],
                              lambda o: wext[j][g, :, o:o + 64, :], b),
                        preferred_element_type=F32) for j, (r0, r1) in rows.items()], axis=0)

        res, out, r = _combine(mm), {}, 0
        for j, (r0, r1) in rows.items():
            out[j] = [[v[r:r + r1 - r0] for v in half] for half in res]
            r += r1 - r0
        return out

    def put_o(g, r0, o):
        for n, v in enumerate(_left([h[0] for h in o], [h[1] for h in o])):
            ob[n, g, r0:HH, :] = v.astype(BF16)

    def put_o_pieces(g, r0):
        def own(i):
            x, y = of[i, 0, r0:HH, :], of[i, 1, r0:HH, :]
            ob[i, g, r0:HH, :] = (x + KS[i] * y).astype(BF16)
            ob[NB + i, g, r0:HH, :] = y.astype(BF16)

        def cross(n, i, j):
            yi = of[i, 1, r0:HH, :]
            sx, sy = of[i, 0, r0:HH, :] + of[j, 0, r0:HH, :], yi + of[j, 1, r0:HH, :]
            p2, d = sx + KS[j] * sy, KS[j] - KS[i]
            for m, v in enumerate((p2 - (yi if d == 1.0 else d * yi), p2, sx + KS[i] * sy)):
                ob[2 * NB + 3 * n + m, g, r0:HH, :] = v.astype(BF16)

        return ([functools.partial(own, i) for i in range(NB)]
                + [functools.partial(cross, n, i, j) for n, (i, j) in enumerate(PAIRS)])

    def lanes(k, n=1):
        return pl.ds(pl.multiple_of(128 * k, 128), 128 * n)

    def out_mm(c, r0, a, b, g0, g1):
        o = jnp.concatenate([ob[a, g, r0:HH, :] for g in range(g0, g1)], axis=1)
        if not isinstance(b, int) and b[0] == b[1]:
            b = NX + b[0]
        w = right(lambda i, e: wo[g0:g1, i, :, lanes(NB * c + e)],
                  lambda o: wox[g0:g1, o:o + 64, lanes(c)], b)
        return jnp.dot(o, w, preferred_element_type=F32)

    def out_mem(c, r0, keep, feed, early=(), extra=()):
        hook = spread(extra)

        def mm(a, b):
            hook(a)
            if a in early:
                return early[a] + out_mm(c, r0, a, b, NG - 1, NG)
            return out_mm(c, r0, a, b, 0, NG)

        top, bot = _combine(mm)
        x0 = XH - r0
        if keep:
            mend[0:MH, lanes(NB * c, NB)] = jnp.concatenate([v[x0:] for v in top], axis=1)
            mend[MH:2 * MH, lanes(NB * c, NB)] = jnp.concatenate([v[x0:] for v in bot], axis=1)
        if feed:
            for n, v in enumerate(_left([v[x0:] for v in top], [v[x0:] for v in bot])):
                hs[n, XH // 2:HH // 2, lanes(c)] = pltpu.bitcast(v.astype(BF16), U32)
        return [[v[:x0] for v in half] for half in (top, bot)]

    cp_ax(T - 1).wait()
    load_x(T - 1)

    def kv_loop(g, carry):
        @pl.when(g < NG // 2)
        def _():
            cp_wo(2 * g).start()
            cp_wo(2 * g + 1).start()

        @pl.when(g >= NG // 2)
        def _():
            start_w(0, 2 * g - NG)
            start_w(0, 2 * g - NG + 1)

        for j, ret in ((1, kret), (2, vret)):
            wait_w(j, g)
        for j, ret in ((1, kret), (2, vret)):
            prep_w(j, g)
            top, bot = project(g, {j: (0, XH)})[j]
            for e in range(NB):
                ret[NB * g + e] = jnp.concatenate([top[e], bot[e]], axis=0).astype(BF16)
        return carry

    lax.fori_loop(0, NG, kv_loop, 0)

    cp_ax(T - 2).wait()
    xbar = jnp.sum(_lo(ax[T - 2]) + _hi(ax[T - 2]), axis=1, keepdims=True) * (1.0 / (SEG + MEM))
    set_mem(jnp.broadcast_to(xbar, (G, MEM, DM)).reshape(G * MEM, DM))

    def guess(g, carry):
        cp_wo(g).wait()
        side = [functools.partial(prep_wo, g, c, r) for c in range(NI) for r in range(0, 64, 8)]
        put_o(g, XH, list(zip(*project(g, {2: (XH, HH)}, side)[2])))
        return carry

    lax.fori_loop(0, NG, guess, 0)
    lax.fori_loop(0, NI, lambda c, carry: (out_mem(c, XH, False, True), carry)[1], 0)

    TILES = ((0, 1, 2), (3, 4, 5), (6, 7))
    nx = [SEG * len(tl) for tl in TILES]
    nm = (32, 32, 16)

    def tile(v, g, with_x):
        m0 = XH if with_x else 0
        parts = [v[ch // 4][SEG * (ch % 4):SEG * (ch % 4 + 1)] for ch in TILES[g]] if with_x else []
        parts += [v[ch // 4][m0 + MEM * (ch % 4):m0 + MEM * (ch % 4 + 1)] for ch in TILES[g]]
        if len(TILES[g]) == 3:
            parts.append(jnp.zeros((MEM, DH), F32))
        return jnp.concatenate(parts, axis=0).astype(BF16)

    def step(mode):
        q_x, kv_x = mode != "pred", mode == "mid"
        q0, kv0 = (0 if q_x else XH), (0 if kv_x else XH)

        def put(ref, e, v, with_x):
            for g in range(3):
                ref[e, g, (0 if with_x else nx[g]):nx[g] + nm[g], :] = tile(v, g, with_x)

        def proj(hg, mats, extra=()):
            res = project(hg, {j: (kv0 if j else q0, HH) for j in mats}, extra)
            for j in mats:
                for e in range(NB):
                    v = [half[e] if j else half[e] * QSCALE for half in res[j]]
                    put((qt, kt, vt)[j], e, v, kv_x if j else q_x)

        def get(ref, ret, hg, e, g):
            if kv_x:
                return ref[e, g]
            return jnp.concatenate(
                [ret[NB * hg + e, 96 * g:96 * g + nx[g], :], ref[e, g, nx[g]:128, :]], axis=0)

        def scores(hg, e):
            out = []
            for g in range(3):
                r0 = 0 if q_x else nx[g]
                s = lax.dot_general(qt[e, g, r0:nx[g] + nm[g], :], get(kt, kret, hg, e, g), NT,
                                    preferred_element_type=F32)
                fill = mask_ref[g // 2, r0:nx[g] + nm[g], :]
                s = jnp.where(fill == 0.0, s, fill)
                pr = jnp.exp2(s - jnp.max(s, axis=1, keepdims=True))
                out.append((pr.astype(BF16), jnp.sum(pr, axis=1, keepdims=True)))
            return out

        def values(hg, e, sc):
            xs, ms = [], []
            for g in range(3):
                pr, den = sc[g]
                inv = pl.reciprocal(den, approx=True)
                inv = inv * (2.0 - den * inv)
                o = jnp.dot(pr, get(vt, vret, hg, e, g), preferred_element_type=F32) * inv
                m0 = nx[g] if q_x else 0
                for i in range(len(TILES[g])):
                    if q_x:
                        xs.append(o[SEG * i:SEG * (i + 1)])
                    ms.append(o[m0 + MEM * i:m0 + MEM * (i + 1)])
            return [jnp.concatenate(xs[4 * k:4 * k + 4] + ms[4 * k:4 * k + 4], axis=0)
                    for k in range(2)]

        def group(hg, fill=None):
            sc = [scores(hg, e) for e in range(NB)]
            if fill is not None:
                fill()
                put_o(hg, q0, [values(hg, e, sc[e]) for e in range(NB)])
                return

            def park(e):
                for k, v in enumerate(values(hg, e, sc[e])):
                    of[e, k, q0:HH, :] = v

            parks = [functools.partial(park, e) for e in range(NB)]
            if mode == "mid":
                proj(hg + 1, [0, 1, 2], [lambda: None] * 4 + parks + put_o_pieces(hg, q0))
            elif mode == "last":
                proj(hg + 1, [0], [lambda: None] * 2 + parks)
                proj(hg + 1, [1, 2], put_o_pieces(hg, q0))
            else:
                proj(hg + 1, [1, 2, 0], [lambda: None] * 4 + parks + put_o_pieces(hg, q0))

        def first():
            for mats in ([[0, 1, 2]] if mode == "mid" else [[1, 2, 0]]):
                proj(0, mats)

        return first, group

    first, group = step("pred")
    for t in range(T - 2):
        cp_ax(t).start()
    wait_w(0, 0)
    prep_w(0, 0)
    first()

    def pred_loop(hg, carry):
        wait_w(0, hg + 1)
        prep_w(0, hg + 1)
        group(hg)
        return carry

    lax.fori_loop(0, NG - 1, pred_loop, 0)
    group(NG - 1, lambda: None)
    lax.fori_loop(0, NI, lambda c, carry: (out_mem(c, XH, True, False), carry)[1], 0)
    for t in range(T - 2):
        cp_ax(t).wait()
    for c in range(8):
        cp_by(c).start()
    load_x(0)

    first, group = step("mid")
    group_last = step("last")[1]

    def segment(t, it):
        first()

        @pl.when(t < T - 1)
        def _():
            lax.fori_loop(0, NG - 1, lambda hg, c: (group(hg), c)[1], 0)

        @pl.when(t == T - 1)
        def _():
            lax.fori_loop(0, NG - 1, lambda hg, c: (group_last(hg), c)[1], 0)
            for e in range(NB):
                for g in range(3):
                    kt[e, g, 0:nx[g], :] = kret[NH - NB + e, 96 * g:96 * g + nx[g], :]
                    vt[e, g, 0:nx[g], :] = vret[NH - NB + e, 96 * g:96 * g + nx[g], :]

        nxt = x_pieces((t + 1) % T)
        per = len(nxt) // NI
        early = {}
        group(NG - 1, lambda: early.update({i: out_mm(0, 0, i, i, 0, NG - 1) for i in range(3)}))
        for c in range(NI):
            for k, half in enumerate(out_mem(c, 0, True, True, early if c == 0 else {},
                                             nxt[per * c:per * (c + 1)])):
                for e, v in enumerate(half):
                    ostage[t, 4 * k:4 * k + 4, :, :, 128 * (NB * c + e):128 * (NB * c + e + 1)] = (
                        v.astype(BF16).reshape(G // 2, 2, 16, 128))

        @pl.when(jnp.logical_and(it == 0, t == 0))
        def _():
            for c in range(8):
                cp_by(c).wait()

        cp_ao(t).start()
        return it

    def one_pass(carry):
        it, _ = carry
        start = mend[0:(G - 1) * MEM, :]
        mstart[...] = start
        set_mem(jnp.concatenate([mem0_ref[...].astype(F32), start], axis=0))
        lax.fori_loop(0, T, segment, it)
        real = mend[0:(G - 1) * MEM, :]
        lim = jnp.max(jnp.abs(real), axis=1, keepdims=True) * TOL
        good = jnp.abs(real - mstart[...]) <= lim
        bad = jnp.max(jnp.where(good, 0.0, 1.0))
        for t in range(T):
            cp_ao(t).wait()
        return it + 1, bad

    lax.while_loop(lambda c: jnp.logical_and(c[0] < G, c[1] > 0.0), one_pass,
                   (jnp.int32(0), jnp.float32(1.0)))


@functools.partial(jax.jit, static_argnames=("A_seg_len",))
def pallas_concat_heads__memory_aug_recurrent_mem_tr__spectral_gfnet__prompt_kernel(
    A_x, A_mem0, A_Wq, A_Wk, A_Wv, A_Wo, A_seg_len, B_x, B_w_r, B_w_i,
):
    assert A_seg_len == SEG and A_x.shape == (1, G * T * SEG, DM) and A_Wq.shape == (DM, NH, DH)
    assert A_mem0.shape == (1, MEM, DM) and B_x.shape == (1, 2048, 1024)
    dmat, smat, mask = _constants()
    wr_t, wi_t = B_w_r.T, B_w_i.T
    hbm = pl.BlockSpec(memory_space=pl.ANY)
    nyq = pl.BlockSpec((16, 2048), lambda i: (32, 0))

    def full(shape):
        return pl.BlockSpec(shape, lambda i: (0,) * len(shape))

    out = pl.pallas_call(
        _kernel,
        grid=(1,),
        in_specs=[hbm] * 9 + [full((MEM, DM)), nyq, nyq, full(dmat.shape), full(mask.shape)],
        out_specs=hbm,
        out_shape=jax.ShapeDtypeStruct((G, 16, 16, 2 * DM), BF16),
        scratch_shapes=[
            pltpu.VMEM((T, G, SEG // 2, DM), U32),
            *[pltpu.VMEM((NG, NI, NB, NB * 64, DH), U32)] * 3,
            *[pltpu.VMEM((NG, NI, NX * 64, DH), U32)] * 3,
            pltpu.VMEM((NG, NB, 64, DM), U32),
            pltpu.VMEM((NG, (NX + NB) * 64, NI * 128), U32),
            pltpu.VMEM((8, 8, 16, 1024), U32),
            pltpu.VMEM((16, 256, 128), U32),
            pltpu.VMEM((16, 256, 128), U32),
            pltpu.VMEM((16, 256, 256), BF16),
            pltpu.VMEM((16, KROWS, 256), F32),
            pltpu.VMEM((16, 640, 256), BF16),
            pltpu.VMEM((NH, G * SEG, DH), BF16),
            pltpu.VMEM((NH, G * SEG, DH), BF16),
            pltpu.VMEM((NL, HH // 2, NI * 128), U32),
            pltpu.VMEM((NB, 3, 128, DH), BF16),
            pltpu.VMEM((NB, 3, 128, DH), BF16),
            pltpu.VMEM((NB, 3, 128, DH), BF16),
            pltpu.VMEM((NL, NG, HH, DH), BF16),
            pltpu.VMEM((NB, 2, HH, DH), F32),
            pltpu.VMEM(((G - 1) * MEM, DM), F32),
            pltpu.VMEM((G * MEM, DM), F32),
            pltpu.VMEM((T, G, 2, 16, DM), BF16),
            pltpu.SemaphoreType.DMA((3, 8)),
            pltpu.SemaphoreType.DMA((4, NB // 2, NG)),
            pltpu.SemaphoreType.DMA((2, 2)),
            pltpu.SemaphoreType.DMA((2, T)),
        ],
        compiler_params=pltpu.CompilerParams(
            dimension_semantics=("arbitrary",), vmem_limit_bytes=120 * 1024 * 1024),
    )(
        A_x.reshape(G, T, SEG, DM),
        *[w.reshape(NI, NB, 128, NH, DH) for w in (A_Wq, A_Wk, A_Wv)],
        A_Wo.reshape(NG, NB, DH, DM), B_x.reshape(8, 16, 16, 1024), wr_t, wi_t, smat,
        A_mem0.reshape(MEM, DM), wr_t, wi_t, dmat, mask,
    )
    return out.reshape(1, 2048, 2 * DM)
```

```python
import functools

import jax
import jax.numpy as jnp
import numpy as np
from jax import lax
from jax.experimental import pallas as pl
from jax.experimental.pallas import tpu as pltpu

F32 = jnp.float32
BF16 = jnp.bfloat16
U32 = jnp.uint32

G = 8
T = 8
SEG = 32
MEM = 8
DM = 1024
NH = 32
DH = 128
KS = (-4.0 / 3, -1.0 / 3, 1.0 / 3, 4.0 / 3)
NB = len(KS)
PAIRS = [(i, j) for i in range(NB) for j in range(i + 1, NB)]
NL = 2 * NB + 3 * len(PAIRS)
NX = NB + len(PAIRS)
NG = NH // NB
NI = DM // 128 // NB
assert NG == 8
XH = G // 2 * SEG
MH = G // 2 * MEM
HH = XH + MH
LOG2E = 1.4426950408889634
QSCALE = float(DH ** -0.5 * LOG2E)
MASKED = float(-1e9 * LOG2E)
TOL = 2.0 ** -9
NT = (((1,), (1,)), ((), ()))
KROWS = 528
ROW_OFF = {0: 0, 4: 64, 1: 128, 7: 192, 2: 256, 6: 320, 3: 384, 5: 448}


def _constants():
    beta = np.arange(128)[None, :]
    m = np.arange(64)[:, None]
    d = np.zeros((4, 256, 256))
    for blk, r in enumerate((0, 4)):
        th = 2 * np.pi * (8 * m + r) * beta / 1024
        d[0, 64 * blk:64 * blk + 64, 128 * blk:128 * blk + 128] = np.cos(th)
        d[0, 128 + 64 * blk:192 + 64 * blk, 128 * blk:128 * blk + 128] = -np.sin(th)
    d[0, 128, 0:128] = np.cos(np.pi * np.arange(128))
    for r, sg in ((1, -1.0), (2, -1.0), (3, 1.0)):
        for blk, (res, cj) in enumerate(((r, 1.0), (8 - r, -1.0))):
            th = 2 * np.pi * (8 * m + res) * beta / 1024
            re, im = slice(64 * blk, 64 * blk + 64), slice(128 + 64 * blk, 192 + 64 * blk)
            d[r, re, 0:128] = np.cos(th)
            d[r, im, 0:128] = -np.sin(th)
            d[r, re, 128:256] = sg * cj * np.sin(th)
            d[r, im, 128:256] = sg * cj * np.cos(th)
    d *= 2.0 ** -10
    b = np.arange(128)[:, None]
    kb = np.arange(128)[None, :]
    s = np.zeros((16, 256, 256))
    for a in range(16):
        th = 2 * np.pi * ((kb * (16 * b + a)) % 2048) / 2048
        s[a, :128, :128] = np.cos(th)
        s[a, 128:, :128] = np.sin(th)
        s[a, :128, 128:] = -np.sin(th)
        s[a, 128:, 128:] = np.cos(th)
    mask = np.zeros((2, 128, 128), np.float32)
    for i, ns in enumerate((3, 2)):
        idx = np.arange(128)
        isx = idx < SEG * ns
        pad = idx >= (SEG + MEM) * ns
        seg = np.where(isx, idx // SEG, (idx - SEG * ns) // MEM)
        same = (seg[:, None] == seg[None, :]) & ~pad[None, :]
        future = isx[:, None] & isx[None, :] & (idx[None, :] > idx[:, None])
        mk = np.where(same, np.where(future, MASKED, 0.0), -np.inf)
        mask[i] = np.where(pad[:, None], 0.0, mk)
    return d.astype(BF16), s.astype(BF16), mask


def _lo(w):
    return lax.bitcast_convert_type(w << 16, F32)


def _hi(w):
    return lax.bitcast_convert_type(w & np.uint32(0xFFFF0000), F32)


def _r4(x, sg):
    (ar, ai), (br, bi), (cr, ci), (dr, di) = x
    s0r, s0i, d0r, d0i = ar + cr, ai + ci, ar - cr, ai - ci
    s1r, s1i, d1r, d1i = br + dr, bi + di, br - dr, bi - di
    p = (d0r - d1i, d0i + d1r)
    q = (d0r + d1i, d0i - d1r)
    y1, y3 = (p, q) if sg > 0 else (q, p)
    return [(s0r + s1r, s0i + s1i), y1, (s0r - s1r, s0i - s1i), y3]


def _tw(z, e, sg):
    r, i = z
    if e == 0:
        return z
    if e == 4:
        return (-i, r) if sg > 0 else (i, -r)
    h = float(np.sqrt(0.5))
    if e == 2:
        return ((r - i) * h, (r + i) * h) if sg > 0 else ((r + i) * h, (i - r) * h)
    if e == 6:
        return ((r + i) * -h, (r - i) * h) if sg > 0 else ((i - r) * h, (r + i) * -h)
    c = float(np.cos(2 * np.pi * e / 16))
    s = float(sg * np.sin(2 * np.pi * e / 16))
    return (r * c - i * s, r * s + i * c)


def _fft16(x, sg):
    t = [_r4([x[4 * a1 + a0] for a1 in range(4)], sg) for a0 in range(4)]
    out = [None] * 16
    for k0 in range(4):
        u = _r4([_tw(t[a0][k0], a0 * k0, sg) for a0 in range(4)], sg)
        for k1 in range(4):
            out[k0 + 4 * k1] = u[k1]
    return out


def _words(even, odd):
    return pltpu.pack_elementwise([even, odd], packed_dtype=BF16)


def _left(x, y):
    z = [x[i] + KS[i] * y[i] for i in range(NB)]
    out = z + list(y)
    for i, j in PAIRS:
        sx, sy = x[i] + x[j], y[i] + y[j]
        out += [z[i] + z[j], sx + KS[j] * sy, sx + KS[i] * sy]
    return out


def _right(b):
    rows = [functools.reduce(lambda u, v: u + v, b[i]) for i in range(NB)]
    extra = [functools.reduce(lambda u, v: u - v, [b[j][i] for j in range(NB) if j != i], b[i][i])
             for i in range(NB)]
    extra += [(b[i][j] + b[j][i]) * (1.0 / (KS[j] - KS[i])) for i, j in PAIRS]
    return rows, extra


def _combine(mm):
    s = [mm(i, i) for i in range(NB)]
    r = [mm(NB + i, (i, i)) for i in range(NB)]
    for n, (i, j) in enumerate(PAIRS):
        p1 = mm(2 * NB + 3 * n, NB + n)
        p2 = mm(2 * NB + 3 * n + 1, (i, j))
        p3 = mm(2 * NB + 3 * n + 2, (j, i))
        d = 1.0 / (KS[j] - KS[i])
        e = (p2 + p3 if d == 1.0 else (p2 + p3) * d) - p1
        r[j], r[i], s[j], s[i] = r[j] + e, r[i] - e, s[j] + p2, s[i] + p3
    return [s[i] - KS[i] * r[i] for i in range(NB)], r


def _kernel(ax_hbm, wq_hbm, wk_hbm, wv_hbm, wo_hbm, bx_hbm, wr_hbm, wi_hbm, s_hbm,
            mem0_ref, wrn_ref, win_ref, d_ref, mask_ref,
            out_hbm,
            ax, wq, wk, wv, wqx, wkx, wvx, wo, wox, xw, wr, wi, sm, yb, vb, kret, vret, hs,
            qt, kt, vt, ob, of, mstart, mend, ostage, sem_b, sem_w, sem_m, sem_o):
    wblk, wext = (wq, wk, wv), (wqx, wkx, wvx)

    def cp_bx(c):
        return pltpu.make_async_copy(bx_hbm.bitcast(U32).at[:, :, c, :], xw.at[c], sem_b.at[0, c])

    def cp_s(c):
        sl = pl.ds(2 * c, 2)
        return pltpu.make_async_copy(s_hbm.at[sl], sm.at[sl], sem_b.at[1, c])

    def cp_by(c):
        return pltpu.make_async_copy(
            xw.at[c], out_hbm.bitcast(U32).at[:, :, c, pl.ds(DM, DM)], sem_b.at[2, c])

    def cp_w(j, g, a):
        src = (wq_hbm, wk_hbm, wv_hbm)[j].bitcast(U32).at[:, :, :, NB // 2 * g + a, :]
        return pltpu.make_async_copy(src, wblk[j].at[g, :, :, pl.ds(128 * a, 128), :],
                                     sem_w.at[j, a, g])

    def start_w(j, g):
        for a in range(NB // 2):
            cp_w(j, g, a).start()

    def cp_wo(g):
        return pltpu.make_async_copy(wo_hbm.bitcast(U32).at[g], wo.at[g], sem_w.at[3, 0, g])

    def cp_ax(t):
        return pltpu.make_async_copy(ax_hbm.bitcast(U32).at[:, t], ax.at[t], sem_o.at[1, t])

    def cp_ao(t):
        return pltpu.make_async_copy(
            ostage.at[t], out_hbm.at[:, pl.ds(2 * t, 2), :, pl.ds(0, DM)], sem_o.at[0, t])

    def cp_f(j, k, half):
        src, dst = ((wr_hbm, wr), (wi_hbm, wi))[j]
        return pltpu.make_async_copy(
            src.at[pl.ds(256 * half, 256), pl.ds(pl.multiple_of(128 * k, 128), 128)].bitcast(U32),
            dst.at[k, pl.ds(128 * half, 128)], sem_m.at[j, half])

    def wait_f(half):
        for j, dst in enumerate((wr, wi)):
            part = dst.at[:, pl.ds(128 * half, 128)]
            pltpu.make_async_copy(part, part, sem_m.at[j, half]).wait()

    for c in range(2):
        cp_bx(c).start()
        cp_s(c).start()

    kt[:, 2, 80:128, :] = jnp.zeros((NB, 48, DH), BF16)
    vt[:, 2, 80:128, :] = jnp.zeros((NB, 48, DH), BF16)
    vb[:, KROWS:640, :] = jnp.zeros((16, 640 - KROWS, 256), BF16)

    rt = float(np.sqrt(0.5))
    row8 = lax.broadcasted_iota(jnp.int32, (8, 128), 0)

    def b_forward(c, carry):
        @pl.when(c < 6)
        def _():
            cp_bx(c + 2).start()
            cp_s(c + 2).start()

        for j in range(2):
            cp_f(j, 2 * c, 0).start()
            cp_f(j, 2 * c + 1, 0).start()

        @pl.when(c == 7)
        def _():
            cp_ax(T - 1).start()
            cp_ax(T - 2).start()

        cp_bx(c).wait()
        cp_s(c).wait()
        w = xw[c].reshape(128, DM)
        for half, xf in enumerate((_lo(w), _hi(w))):
            x = [xf[:, 128 * al:128 * (al + 1)] for al in range(8)]
            s = [x[i] + x[i + 4] for i in range(4)]
            d = [x[i] - x[i + 4] for i in range(4)]
            e, o = s[0] + s[2], s[1] + s[3]
            p, q = (d[1] - d[3]) * rt, (d[1] + d[3]) * rt
            u = [(e + o, e - o), (d[0] + p, d[2] + q), (s[0] - s[2], s[1] - s[3]),
                 (d[0] - p, d[2] - q)]
            tt = [lax.dot_general(d_ref[k], jnp.concatenate(u[k], axis=1).astype(BF16), NT,
                                  preferred_element_type=F32) for k in range(4)]
            dc, ny = tt[0][0:8], tt[0][128:136]
            re = [jnp.where(row8 == 0, dc * 0.5, dc), tt[0][8:128]]
            im = [jnp.where(row8 == 0, 0.0, ny), tt[0][136:256]]
            for k in range(1, 4):
                re.append(tt[k][0:128])
                im.append(tt[k][128:256])
            re += [jnp.where(row8 == 0, ny * 0.5, 0.0), jnp.zeros((8, 128), F32)]
            im.append(jnp.zeros((16, 128), F32))
            lhs = jnp.concatenate([jnp.concatenate(re, axis=0), jnp.concatenate(im, axis=0)],
                                  axis=1).astype(BF16)
            a = 2 * c + half
            yb[a] = jnp.dot(lhs, sm[a], preferred_element_type=F32)
        return carry

    lax.fori_loop(0, 8, b_forward, 0)
    for k in range(16):
        cp_f(0, k, 1).start()
        cp_f(1, k, 1).start()
    wait_f(0)

    def filt(row, wre, wim):
        y = [(yb[a, pl.ds(row, 8), 0:128], yb[a, pl.ds(row, 8), 128:256]) for a in range(16)]
        z = _fft16(y, -1)
        z = [(z[k][0] * wre(k) - z[k][1] * wim(k), z[k][0] * wim(k) + z[k][1] * wre(k))
             for k in range(16)]
        return _fft16(z, 1)

    def b_filter(i, carry):
        mg, j = i // 4, i % 4

        @pl.when(i == 8)
        def _():
            wait_f(1)

        @pl.when(jnp.logical_and(i >= 8, i % 4 == 0))
        def _():
            start_w(1, i // 4 - 2)
            start_w(2, i // 4 - 2)

        for half, un in enumerate((_lo, _hi)):
            off = [ROW_OFF[2 * jj + half] for jj in range(4)]
            base = jnp.where(j < 2, jnp.where(j == 0, off[0], off[1]),
                             jnp.where(j == 2, off[2], off[3])) + 16 * mg
            base = pl.multiple_of(base, 16)
            for r8 in range(2):
                sl = pl.ds(64 * mg + 32 * r8 + j, 8, stride=4)
                row = pl.multiple_of(base + 8 * r8, 8)
                res = filt(row, lambda k: un(wr[k, sl, :]), lambda k: un(wi[k, sl, :]))
                for a in range(16):
                    for ri in range(2):
                        vb[a, pl.ds(row, 8), 128 * ri:128 * (ri + 1)] = res[a][ri].astype(BF16)
        return carry

    lax.fori_loop(0, 16, b_filter, 0)
    res = filt(512, lambda k: wrn_ref[0:1, 128 * k:128 * (k + 1)].astype(F32),
               lambda k: win_ref[0:1, 128 * k:128 * (k + 1)].astype(F32))
    for a in range(16):
        for ri in range(2):
            vb[a, 512:KROWS, 128 * ri:128 * (ri + 1)] = jnp.concatenate(
                [res[a][ri], jnp.zeros((8, 128), F32)], axis=0).astype(BF16)

    lane0 = lax.broadcasted_iota(jnp.int32, (128, 128), 1) == 0

    def b_inverse(c, carry):
        @pl.when(c < NG - 2)
        def _():
            start_w(1, c + 2)
            start_w(2, c + 2)

        lhs = [[] for _ in range(4)]
        for half in range(2):
            a = 2 * c + half
            ny = lax.dot_general(sm[a, 0:128, :], vb[a, 512:640, :], NT,
                                 preferred_element_type=F32)
            z = lax.dot_general(sm[a], vb[a, 0:512, :], NT, preferred_element_type=F32)
            for k in range(4):
                zr, zi = z[0:128, 128 * k:128 * (k + 1)], z[128:256, 128 * k:128 * (k + 1)]
                if k == 0:
                    zi = jnp.where(lane0, ny, zi)
                lhs[k].append(jnp.concatenate([zr, zi], axis=1).astype(BF16))
        g = [jnp.dot(jnp.concatenate(lhs[k], axis=0), d_ref[k], preferred_element_type=F32)
             for k in range(4)]
        (g0, g4), (g1r, g1i), (g2r, g2i), (g3r, g3i) = [(v[:, :128], v[:, 128:]) for v in g]
        e, o = g0 + g4, g0 - g4
        s = [e + g2r, o + g2i, e - g2r, o - g2i]
        p, q = (g1r - g3r) * rt, (g1i - g3i) * rt
        d = [g1r + g3r, q + p, g1i + g3i, q - p]
        y = [s[i] + d[i] for i in range(4)] + [s[i] - d[i] for i in range(4)]
        for al in range(8):
            xw[c, :, :, 128 * al:128 * (al + 1)] = _words(
                y[al][0:128], y[al][128:256]).reshape(8, 16, 128)
        return carry

    lax.fori_loop(0, 8, b_inverse, 0)

    def blocks(v):
        n = v.shape[1] // (128 * NB)
        return [jnp.concatenate([v[:, 128 * (NB * c + i):128 * (NB * c + i + 1)]
                                 for c in range(n)], axis=1) for i in range(NB)]

    def x_pieces(t):
        def piece(g, c):
            cols = slice(128 * NB * c, 128 * NB * (c + 1))
            top, bot = ax[t, g, :, cols], ax[t, g + G // 2, :, cols]
            ev, od = [_left(blocks(un(top)), blocks(un(bot))) for un in (_lo, _hi)]
            for n in range(NL):
                hs[n, SEG // 2 * g:SEG // 2 * (g + 1), 128 * c:128 * (c + 1)] = _words(ev[n], od[n])

        return [functools.partial(piece, g, c) for g in range(G // 2) for c in range(NI)]

    def set_mem(m):
        for n, v in enumerate(_left(blocks(m[0:MH]), blocks(m[MH:2 * MH]))):
            hs[n, XH // 2:HH // 2, :] = pltpu.bitcast(v.astype(BF16), U32)

    def wait_w(j, g):
        for a in range(NB // 2):
            cp_w(j, g, a).wait()

    def prep_w(j, g):
        ref = wblk[j]

        def raw(c, i, r, n):
            w = [[ref[g, c, i, pl.ds(128 * a + 2 * r + d, n, stride=2), :]
                  for a in range(NB // 2)] for d in range(2)]
            return [[un(v) for v in w[d] for un in (_lo, _hi)] for d in range(2)]

        for c in range(NI):
            for r in range(0, 64, 8):
                b = [raw(c, i, r, 8) for i in range(NB)]
                ev, od = [_right([b[i][d] for i in range(NB)])[1] for d in range(2)]
                for n in range(NX):
                    wext[j][g, c, 64 * n + r:64 * n + r + 8, :] = _words(ev[n], od[n])
        for c in range(NI):
            for i in range(NB):
                ev, od = raw(c, i, 0, 64)
                for v in (ev, od):
                    v[i] = functools.reduce(lambda p, q: p + q, v)
                for e in range(NB):
                    ref[g, c, i, 64 * e:64 * (e + 1), :] = _words(ev[e], od[e])

    def prep_wo(g, c, r):
        w = [[wo[g, i, r:r + 8, 128 * (NB * c + j):128 * (NB * c + j + 1)]
              for j in range(NB)] for i in range(NB)]
        ev, od = [_right([[un(v) for v in row] for row in w]) for un in (_lo, _hi)]
        for n, (u, v) in enumerate(zip(ev[1] + ev[0], od[1] + od[0])):
            wox[g, 64 * n + r:64 * n + r + 8, 128 * c:128 * (c + 1)] = _words(u, v)

    def run(pieces):
        for fn in pieces:
            fn()

    def right(blk, ext, b):
        w = ext(64 * b) if isinstance(b, int) else blk(*b)
        w = pltpu.bitcast(w, BF16)
        return w.reshape(w.shape[0] * 128, 128)

    def spread(extra):
        at = {NL * n // len(extra): fn for n, fn in enumerate(extra)}
        return lambda a: at[a]() if a in at else None

    def project(g, rows, extra=()):
        hook = spread(extra)

        def mm(a, b):
            hook(a)
            return jnp.concatenate([
                jnp.dot(pltpu.bitcast(hs[a, r0 // 2:r1 // 2, :], BF16),
                        right(lambda i, e: wblk[j][g, :, i, 64 * e:64 * (e + 1), :],
                              lambda o: wext[j][g, :, o:o + 64, :], b),
                        preferred_element_type=F32) for j, (r0, r1) in rows.items()], axis=0)

        res, out, r = _combine(mm), {}, 0
        for j, (r0, r1) in rows.items():
            out[j] = [[v[r:r + r1 - r0] for v in half] for half in res]
            r += r1 - r0
        return out

    def put_o(g, r0, o):
        for n, v in enumerate(_left([h[0] for h in o], [h[1] for h in o])):
            ob[n, g, r0:HH, :] = v.astype(BF16)

    def put_o_pieces(g, r0):
        def own(i):
            x, y = of[i, 0, r0:HH, :], of[i, 1, r0:HH, :]
            ob[i, g, r0:HH, :] = (x + KS[i] * y).astype(BF16)
            ob[NB + i, g, r0:HH, :] = y.astype(BF16)

        def cross(n, i, j):
            yi = of[i, 1, r0:HH, :]
            sx, sy = of[i, 0, r0:HH, :] + of[j, 0, r0:HH, :], yi + of[j, 1, r0:HH, :]
            p2, d = sx + KS[j] * sy, KS[j] - KS[i]
            for m, v in enumerate((p2 - (yi if d == 1.0 else d * yi), p2, sx + KS[i] * sy)):
                ob[2 * NB + 3 * n + m, g, r0:HH, :] = v.astype(BF16)

        return ([functools.partial(own, i) for i in range(NB)]
                + [functools.partial(cross, n, i, j) for n, (i, j) in enumerate(PAIRS)])

    def lanes(k, n=1):
        return pl.ds(pl.multiple_of(128 * k, 128), 128 * n)

    def out_mm(c, r0, a, b, g0, g1):
        o = jnp.concatenate([ob[a, g, r0:HH, :] for g in range(g0, g1)], axis=1)
        if not isinstance(b, int) and b[0] == b[1]:
            b = NX + b[0]
        w = right(lambda i, e: wo[g0:g1, i, :, lanes(NB * c + e)],
                  lambda o: wox[g0:g1, o:o + 64, lanes(c)], b)
        return jnp.dot(o, w, preferred_element_type=F32)

    def out_mem(c, r0, keep, feed, early=(), extra=()):
        hook = spread(extra)

        def mm(a, b):
            hook(a)
            if a in early:
                return early[a] + out_mm(c, r0, a, b, NG - 1, NG)
            return out_mm(c, r0, a, b, 0, NG)

        top, bot = _combine(mm)
        x0 = XH - r0
        if keep:
            mend[0:MH, lanes(NB * c, NB)] = jnp.concatenate([v[x0:] for v in top], axis=1)
            mend[MH:2 * MH, lanes(NB * c, NB)] = jnp.concatenate([v[x0:] for v in bot], axis=1)
        if feed:
            for n, v in enumerate(_left([v[x0:] for v in top], [v[x0:] for v in bot])):
                hs[n, XH // 2:HH // 2, lanes(c)] = pltpu.bitcast(v.astype(BF16), U32)
        return [[v[:x0] for v in half] for half in (top, bot)]

    cp_ax(T - 1).wait()
    run(x_pieces(T - 1))

    def kv_loop(g, carry):
        @pl.when(g < NG // 2)
        def _():
            cp_wo(2 * g).start()
            cp_wo(2 * g + 1).start()

        @pl.when(g >= NG // 2)
        def _():
            start_w(0, 2 * g - NG)
            start_w(0, 2 * g - NG + 1)

        for j, ret in ((1, kret), (2, vret)):
            wait_w(j, g)
        for j, ret in ((1, kret), (2, vret)):
            prep_w(j, g)
            top, bot = project(g, {j: (0, XH)})[j]
            for e in range(NB):
                ret[NB * g + e] = jnp.concatenate([top[e], bot[e]], axis=0).astype(BF16)
        return carry

    lax.fori_loop(0, NG, kv_loop, 0)

    cp_ax(T - 2).wait()
    xbar = jnp.sum(_lo(ax[T - 2]) + _hi(ax[T - 2]), axis=1, keepdims=True) * (1.0 / (SEG + MEM))
    set_mem(jnp.broadcast_to(xbar, (G, MEM, DM)).reshape(G * MEM, DM))

    def guess(g, carry):
        cp_wo(g).wait()
        side = [functools.partial(prep_wo, g, c, r) for c in range(NI) for r in range(0, 64, 8)]
        put_o(g, XH, list(zip(*project(g, {2: (XH, HH)}, side)[2])))
        return carry

    lax.fori_loop(0, NG, guess, 0)
    lax.fori_loop(0, NI, lambda c, carry: (out_mem(c, XH, False, True), carry)[1], 0)

    TILES = ((0, 1, 2), (3, 4, 5), (6, 7))
    nx = [SEG * len(tl) for tl in TILES]
    nm = (32, 32, 16)

    def tile(v, g, with_x):
        m0 = XH if with_x else 0
        parts = [v[ch // 4][SEG * (ch % 4):SEG * (ch % 4 + 1)] for ch in TILES[g]] if with_x else []
        parts += [v[ch // 4][m0 + MEM * (ch % 4):m0 + MEM * (ch % 4 + 1)] for ch in TILES[g]]
        if len(TILES[g]) == 3:
            parts.append(jnp.zeros((MEM, DH), F32))
        return jnp.concatenate(parts, axis=0).astype(BF16)

    def step(mode):
        q_x, kv_x = mode != "pred", mode == "mid"
        q0, kv0 = (0 if q_x else XH), (0 if kv_x else XH)

        def put(ref, e, v, with_x):
            for g in range(3):
                ref[e, g, (0 if with_x else nx[g]):nx[g] + nm[g], :] = tile(v, g, with_x)

        def proj(hg, mats, extra=()):
            res = project(hg, {j: (kv0 if j else q0, HH) for j in mats}, extra)
            for j in mats:
                for e in range(NB):
                    v = [half[e] if j else half[e] * QSCALE for half in res[j]]
                    put((qt, kt, vt)[j], e, v, kv_x if j else q_x)

        def get(ref, ret, hg, e, g):
            if kv_x:
                return ref[e, g]
            return jnp.concatenate(
                [ret[NB * hg + e, 96 * g:96 * g + nx[g], :], ref[e, g, nx[g]:128, :]], axis=0)

        def scores(hg, e):
            out = []
            for g in range(3):
                r0 = 0 if q_x else nx[g]
                s = lax.dot_general(qt[e, g, r0:nx[g] + nm[g], :], get(kt, kret, hg, e, g), NT,
                                    preferred_element_type=F32)
                fill = mask_ref[g // 2, r0:nx[g] + nm[g], :]
                s = jnp.where(fill == 0.0, s, fill)
                pr = jnp.exp2(s - jnp.max(s, axis=1, keepdims=True))
                out.append((pr.astype(BF16), jnp.sum(pr, axis=1, keepdims=True)))
            return out

        def values(hg, e, sc):
            xs, ms = [], []
            for g in range(3):
                pr, den = sc[g]
                inv = pl.reciprocal(den, approx=True)
                inv = inv * (2.0 - den * inv)
                o = jnp.dot(pr, get(vt, vret, hg, e, g), preferred_element_type=F32) * inv
                m0 = nx[g] if q_x else 0
                for i in range(len(TILES[g])):
                    if q_x:
                        xs.append(o[SEG * i:SEG * (i + 1)])
                    ms.append(o[m0 + MEM * i:m0 + MEM * (i + 1)])
            return [jnp.concatenate(xs[4 * k:4 * k + 4] + ms[4 * k:4 * k + 4], axis=0)
                    for k in range(2)]

        def group(hg, fill=None):
            sc = [scores(hg, e) for e in range(NB)]
            if fill is not None:
                fill()
                put_o(hg, q0, [values(hg, e, sc[e]) for e in range(NB)])
                return

            def park(e):
                for k, v in enumerate(values(hg, e, sc[e])):
                    of[e, k, q0:HH, :] = v

            parks = [functools.partial(park, e) for e in range(NB)]
            if mode == "mid":
                gap = [lambda: None] * 3
                proj(hg + 1, [0, 1, 2], gap + parks + put_o_pieces(hg, q0) + gap)
            elif mode == "last":
                proj(hg + 1, [0], [lambda: None] * 2 + parks)
                proj(hg + 1, [1, 2], put_o_pieces(hg, q0))
            else:
                proj(hg + 1, [1, 2, 0], [lambda: None] * 4 + parks + put_o_pieces(hg, q0))

        def first():
            for mats in ([[0, 1, 2]] if mode == "mid" else [[1, 2, 0]]):
                proj(0, mats)

        return first, group

    first, group = step("pred")
    for t in range(T - 2):
        cp_ax(t).start()
    wait_w(0, 0)
    prep_w(0, 0)
    first()

    def pred_loop(hg, carry):
        wait_w(0, hg + 1)
        prep_w(0, hg + 1)
        group(hg)
        return carry

    lax.fori_loop(0, NG - 1, pred_loop, 0)
    group(NG - 1, lambda: None)
    lax.fori_loop(0, NI, lambda c, carry: (out_mem(c, XH, True, False), carry)[1], 0)
    for t in range(T - 2):
        cp_ax(t).wait()
    for c in range(8):
        cp_by(c).start()
    run(x_pieces(0))

    first, group = step("mid")
    group_last = step("last")[1]

    def segment(t, it):
        first()

        @pl.when(t < T - 1)
        def _():
            lax.fori_loop(0, NG - 1, lambda hg, c: (group(hg), c)[1], 0)

        @pl.when(t == T - 1)
        def _():
            lax.fori_loop(0, NG - 1, lambda hg, c: (group_last(hg), c)[1], 0)
            for e in range(NB):
                for g in range(3):
                    kt[e, g, 0:nx[g], :] = kret[NH - NB + e, 96 * g:96 * g + nx[g], :]
                    vt[e, g, 0:nx[g], :] = vret[NH - NB + e, 96 * g:96 * g + nx[g], :]

        nxt = x_pieces((t + 1) % T)
        per = len(nxt) // NI
        early = {}
        group(NG - 1, lambda: early.update({i: out_mm(0, 0, i, i, 0, NG - 1) for i in range(3)}))
        for c in range(NI):
            for k, half in enumerate(out_mem(c, 0, True, True, early if c == 0 else {},
                                             nxt[per * c:per * (c + 1)])):
                for e, v in enumerate(half):
                    ostage[t, 4 * k:4 * k + 4, :, :, 128 * (NB * c + e):128 * (NB * c + e + 1)] = (
                        v.astype(BF16).reshape(G // 2, 2, 16, 128))

        @pl.when(jnp.logical_and(it == 0, t == 0))
        def _():
            for c in range(8):
                cp_by(c).wait()

        cp_ao(t).start()
        return it

    def one_pass(carry):
        it, _ = carry
        start = mend[0:(G - 1) * MEM, :]
        mstart[...] = start
        set_mem(jnp.concatenate([mem0_ref[...].astype(F32), start], axis=0))
        lax.fori_loop(0, T, segment, it)
        real = mend[0:(G - 1) * MEM, :]
        lim = jnp.max(jnp.abs(real), axis=1, keepdims=True) * TOL
        good = jnp.abs(real - mstart[...]) <= lim
        bad = jnp.max(jnp.where(good, 0.0, 1.0))
        for t in range(T):
            cp_ao(t).wait()
        return it + 1, bad

    lax.while_loop(lambda c: jnp.logical_and(c[0] < G, c[1] > 0.0), one_pass,
                   (jnp.int32(0), jnp.float32(1.0)))


@functools.partial(jax.jit, static_argnames=("A_seg_len",))
def pallas_concat_heads__memory_aug_recurrent_mem_tr__spectral_gfnet__prompt_kernel(
    A_x, A_mem0, A_Wq, A_Wk, A_Wv, A_Wo, A_seg_len, B_x, B_w_r, B_w_i,
):
    assert A_seg_len == SEG and A_x.shape == (1, G * T * SEG, DM) and A_Wq.shape == (DM, NH, DH)
    assert A_mem0.shape == (1, MEM, DM) and B_x.shape == (1, 2048, 1024)
    dmat, smat, mask = _constants()
    wr_t, wi_t = B_w_r.T, B_w_i.T
    hbm = pl.BlockSpec(memory_space=pl.ANY)
    nyq = pl.BlockSpec((16, 2048), lambda i: (32, 0))

    def full(shape):
        return pl.BlockSpec(shape, lambda i: (0,) * len(shape))

    out = pl.pallas_call(
        _kernel,
        grid=(1,),
        in_specs=[hbm] * 9 + [full((MEM, DM)), nyq, nyq, full(dmat.shape), full(mask.shape)],
        out_specs=hbm,
        out_shape=jax.ShapeDtypeStruct((G, 16, 16, 2 * DM), BF16),
        scratch_shapes=[
            pltpu.VMEM((T, G, SEG // 2, DM), U32),
            *[pltpu.VMEM((NG, NI, NB, NB * 64 + 8, DH), U32)] * 3,
            *[pltpu.VMEM((NG, NI, NX * 64, DH), U32)] * 3,
            pltpu.VMEM((NG, NB, 64, DM), U32),
            pltpu.VMEM((NG, (NX + NB) * 64, NI * 128), U32),
            pltpu.VMEM((8, 8, 16, 1024), U32),
            pltpu.VMEM((16, 264, 128), U32),
            pltpu.VMEM((16, 264, 128), U32),
            pltpu.VMEM((16, 256, 256), BF16),
            pltpu.VMEM((16, KROWS, 256), F32),
            pltpu.VMEM((16, 640, 256), BF16),
            pltpu.VMEM((NH, G * SEG, DH), BF16),
            pltpu.VMEM((NH, G * SEG, DH), BF16),
            pltpu.VMEM((NL, HH // 2, NI * 128), U32),
            pltpu.VMEM((NB, 3, 128, DH), BF16),
            pltpu.VMEM((NB, 3, 128, DH), BF16),
            pltpu.VMEM((NB, 3, 128, DH), BF16),
            pltpu.VMEM((NL, NG, HH, DH), BF16),
            pltpu.VMEM((NB, 2, HH, DH), F32),
            pltpu.VMEM(((G - 1) * MEM, DM), F32),
            pltpu.VMEM((G * MEM, DM), F32),
            pltpu.VMEM((T, G, 2, 16, DM), BF16),
            pltpu.SemaphoreType.DMA((3, 8)),
            pltpu.SemaphoreType.DMA((4, NB // 2, NG)),
            pltpu.SemaphoreType.DMA((2, 2)),
            pltpu.SemaphoreType.DMA((2, T)),
        ],
        compiler_params=pltpu.CompilerParams(
            dimension_semantics=("arbitrary",), vmem_limit_bytes=120 * 1024 * 1024),
    )(
        A_x.reshape(G, T, SEG, DM),
        *[w.reshape(NI, NB, 128, NH, DH) for w in (A_Wq, A_Wk, A_Wv)],
        A_Wo.reshape(NG, NB, DH, DM), B_x.reshape(8, 16, 16, 1024), wr_t, wi_t, smat,
        A_mem0.reshape(MEM, DM), wr_t, wi_t, dmat, mask,
    )
    return out.reshape(1, 2048, 2 * DM)
```
